```python
import jax
import jax.numpy as jnp

def _softmax(x, axis=-1):
    return jax.nn.softmax(x, axis=axis)
def _gelu(x):
    return jax.nn.gelu(x, approximate=True)
def _silu(x):
    return jax.nn.silu(x)
def _sigmoid(x):
    return jax.nn.sigmoid(x)
def _layernorm(x, axis=-1, eps=1e-5):
    m = jnp.mean(x, axis=axis, keepdims=True)
    v = jnp.var(x, axis=axis, keepdims=True)
    return (x - m) / jnp.sqrt(v + eps)
def _scatter_add(tgt, idx, src, axis=0):
    return tgt.at[idx].add(src)
def _segment_sum(src, seg, n):
    return jax.ops.segment_sum(src, seg, n)
class _Rng:
    def __init__(self, key):
        self._k = key
    def _next(self):
        self._k, sub = jax.random.split(self._k)
        return sub
    def normal(self, shape):
        return jax.random.normal(self._next(), shape, dtype=jnp.bfloat16)
    def randint(self, lo, hi, shape):
        return jax.random.randint(self._next(), shape, lo, hi, dtype=jnp.int32)
    def uniform(self, shape, lo=0.0, hi=1.0):
        return jax.random.uniform(self._next(), shape, jnp.bfloat16, lo, hi)
    def permutation(self, n):
        return jax.random.permutation(self._next(), n)


kernel_name = 'concat_heads__linear_attn_block__ssm_conv_h3__prompt'

def setup_inputs():
    _rng = _Rng(jax.random.key(int.from_bytes(__import__("os").urandom(4), "little")))
    _w = (lambda a: (lambda t: t.astype(jnp.bfloat16) if jnp.issubdtype(t.dtype, jnp.floating) else t)(jnp.asarray(a)))
    def _A_setup():
        B, S, D = 1, 2048, 1024
        return {
            "x": _w((lambda *s: _rng.normal(s) * 0.05)(B, S, D)),
            "wqkv": _w((lambda *s: _rng.normal(s) * 0.05)(D, 3 * D)),
            "wo": _w((lambda *s: _rng.normal(s) * 0.05)(D, D)),
        }
    _A_in = _A_setup()

    def _B_setup():
        B, S, D = 1, 2048, 1024
        ks = 4
        return {
            "q": _w((lambda *s: _rng.normal(s) * 0.05)(B, S, D)),
            "k": _w((lambda *s: _rng.normal(s) * 0.05)(B, S, D)),
            "v": _w((lambda *s: _rng.normal(s) * 0.05)(B, S, D)),
            "shift_k": _w((lambda *s: _rng.normal(s) * 0.05)(D, ks) * 0.5),
            "ssm_k": _w((lambda *s: _rng.normal(s) * 0.05)(D, S) * (1.0 / S ** 0.5)),
            "ssm_D": _w((lambda *s: _rng.normal(s) * 0.05)(D)),
        }
    _B_in = _B_setup()

    return {
        "A_x": _A_in["x"],
        "A_wqkv": _A_in["wqkv"],
        "A_wo": _A_in["wo"],
        "B_q": _B_in["q"],
        "B_k": _B_in["k"],
        "B_v": _B_in["v"],
        "B_shift_k": _B_in["shift_k"],
        "B_ssm_k": _B_in["ssm_k"],
        "B_ssm_D": _B_in["ssm_D"],
    }

def reference(A_x, A_wqkv, A_wo, B_q, B_k, B_v, B_shift_k, B_ssm_k, B_ssm_D):
    def _A_ref(x, wqkv, wo):
        B, S, D = x.shape
        H = 32; Dh = D // H
        qkv = (lambda x, *d: x.transpose(*d))((x @ wqkv).reshape(B, S, 3, H, Dh), 2, 0, 3, 1, 4)
        q, k, v = qkv[0], qkv[1], qkv[2]
        phi = lambda t: jnp.where(t > 0, t + 1, jnp.exp(t)) + 1e-6
        pq, pk = phi(q), phi(k)
        kv = jnp.einsum("bhsd,bhse->bhde", pk, v)
        z = jnp.einsum("bhsd->bhd", pk)
        num = jnp.einsum("bhqd,bhde->bhqe", pq, kv)
        den = jnp.einsum("bhqd,bhd->bhq", pq, z)[..., None] + 1e-6
        o = num / den
        return (lambda x, *d: x.transpose(*d))(o, 0, 2, 1, 3).reshape(B, S, D) @ wo

    def _B_ref(q, k, v, shift_k, ssm_k, ssm_D):
        B, S, D = q.shape
        ks = shift_k.shape[-1]
        k_pad = jnp.pad(k, ((0, 0), (ks - 1, 0), (0, 0)))
        k_shift = jnp.zeros_like(k)
        for t in range(ks):
            k_shift = k_shift + k_pad[:, t:t + S, :] * shift_k[:, ks - 1 - t][None, None, :]
        kv = k_shift * v
        L = 2 * S
        kv_pad = jnp.pad(kv, ((0, 0), (0, S), (0, 0)))
        kf_pad = jnp.pad(ssm_k, ((0, 0), (0, S)))
        kv_f = (lambda x, axes=(-2,-1): jnp.fft.rfft2(x.astype(jnp.float32), axes=axes))(kv_pad[:, None, :, :], axes=(1, 2))
        kf_f = (lambda x, axes=(-2,-1): jnp.fft.rfft2(x.astype(jnp.float32), axes=axes))(kf_pad[:, None, :], axes=(1, 2))
        kf_f = (lambda x, *d: x.transpose(*d))(kf_f, 1, 2, 0)
        y_f = kv_f * kf_f[None, :, :, :]
        y = (lambda x, s, axes=(-2,-1): jnp.fft.irfft2(x, s=s, axes=axes).astype(jnp.bfloat16))(y_f, (1, L), axes=(1, 2))[:, 0, :S, :]
        y = y + kv * ssm_D[None, None, :]
        return q * y

    a = _A_ref(A_x, A_wqkv, A_wo)
    b = _B_ref(B_q, B_k, B_v, B_shift_k, B_ssm_k, B_ssm_D)
    return jnp.concatenate([a, b], axis=-1)
```

```python
import numpy as np
import jax
import jax.numpy as jnp
import jax.experimental.pallas as pl
import jax.experimental.pallas.tpu as pltpu

S = 2048
D = 1024
DH = 32
N1, N2 = 64, 32
CB = 128
NB = D // CB
KB = 256
TC = 256
HALO = 8
BF = jnp.bfloat16
F32 = jnp.float32


def _dft_matrices():
    n1 = np.arange(N1)
    k1 = np.arange(N1)
    col = 16 * (n1 // 8) + (n1 % 8)
    fwd = np.zeros((N2, 2 * N1, 2 * N1), np.float64)
    for k2 in range(N2):
        e = np.exp(-2j * np.pi * np.outer(N2 * k1 + k2 + 0.25, n1) / S)
        fwd[k2][:N1, col] = e.real
        fwd[k2][:N1, col + 8] = -e.imag
        fwd[k2][N1:, col] = e.imag
        fwd[k2][N1:, col + 8] = e.real
    inv = np.transpose(fwd, (0, 2, 1)) / S
    return fwd.astype(np.float32).astype(BF), inv.astype(np.float32).astype(BF)


_FWD, _INV = _dft_matrices()


def _add(a, b):
    (sa, xa), (sb, xb) = a, b
    if sa == sb:
        return (sa, xa + xb)
    return (1, xa - xb) if sa > 0 else (1, xb - xa)


def _neg(a):
    return (-a[0], a[1])


def _sub(a, b):
    return _add(a, _neg(b))


def _scale(a, c):
    return (1, a[1] * np.float32(a[0] * c))


def _val(a):
    return a[1] if a[0] > 0 else -a[1]


def _cadd(a, b):
    return (_add(a[0], b[0]), _add(a[1], b[1]))


def _csub(a, b):
    return (_sub(a[0], b[0]), _sub(a[1], b[1]))


def _cmul_i(a, s):
    return (_neg(a[1]), a[0]) if s > 0 else (a[1], _neg(a[0]))


def _cmul_const(a, w):
    c, s = float(np.real(w)), float(np.imag(w))
    return (_add(_scale(a[0], c), _scale(a[1], -s)), _add(_scale(a[0], s), _scale(a[1], c)))


def _fft4(x, s):
    a0, a1 = _cadd(x[0], x[2]), _cadd(x[1], x[3])
    b0, b1 = _csub(x[0], x[2]), _cmul_i(_csub(x[1], x[3]), s)
    return [_cadd(a0, a1), _cadd(b0, b1), _csub(a0, a1), _csub(b0, b1)]


def _fft8(x, s):
    r = np.sqrt(0.5)
    a = [_cadd(x[n], x[n + 4]) for n in range(4)]
    b = [_csub(x[n], x[n + 4]) for n in range(4)]
    t = _cadd(b[1], _cmul_i(b[1], s))
    b[1] = (_scale(t[0], r), _scale(t[1], r))
    b[2] = _cmul_i(b[2], s)
    t = _csub(_cmul_i(b[3], s), b[3])
    b[3] = (_scale(t[0], r), _scale(t[1], r))
    ev, od = _fft4(a, s), _fft4(b, s)
    return [ev[0], od[0], ev[1], od[1], ev[2], od[2], ev[3], od[3]]


_C1, _S1, _R2 = np.cos(np.pi / 8), np.sin(np.pi / 8), np.sqrt(0.5)


def _dft32_fwd(load, emit):
    tw = [[None] * 8 for _ in range(4)]
    for n in range(8):
        u0, u1, u2, u3 = [(1, load(n + 8 * m)) for m in range(4)]
        t = _scale(u2, _R2)
        p, m_ = _add(u0, t), _sub(u0, t)
        c1u1, s1u1, c1u3, s1u3 = _scale(u1, _C1), _scale(u1, _S1), _scale(u3, _C1), _scale(u3, _S1)
        a, b = _add(c1u1, s1u3), _add(s1u1, c1u3)
        d, e = _sub(c1u1, s1u3), _sub(s1u1, c1u3)
        sj = [(_add(p, a), _neg(_add(t, b))), (_sub(m_, e), _sub(t, d)),
              (_sub(p, a), _sub(b, t)), (_add(m_, e), _add(t, d))]
        for j in range(4):
            tw[j][n] = sj[j] if n == 0 else _cmul_const(sj[j], np.exp(-2j * np.pi * n * (4 * j + 1) / 128))
    for j in range(4):
        out = _fft8(tw[j], -1)
        for l in range(8):
            emit(j + 4 * l, _val(out[l][0]), _val(out[l][1]))


def _dft32_inv(load, emit):
    tw = []
    for j in range(4):
        x = []
        for l in range(8):
            re, im = load(j + 4 * l)
            x.append(((1, re), (1, im)))
        out = _fft8(x, 1)
        tw.append([out[n] if n == 0 else _cmul_const(out[n], np.exp(2j * np.pi * n * (4 * j + 1) / 128))
                   for n in range(8)])
    for n in range(8):
        (x0, y0), (x1, y1), (x2, y2), (x3, y3) = [tw[j][n] for j in range(4)]
        p, a, b = _add(x0, x2), _sub(x0, x2), _sub(y2, y0)
        m_, e, d = _add(x1, x3), _sub(x3, x1), _sub(y3, y1)
        t = _add(_sub(_add(y1, y3), _add(y0, y2)), _sub(p, m_))
        emit(n, _val(_add(p, m_)))
        emit(n + 8, _val(_add(_scale(_add(a, d), _C1), _scale(_add(b, e), _S1))))
        emit(n + 16, _val(_scale(t, _R2)))
        emit(n + 24, _val(_add(_scale(_sub(a, d), _S1), _scale(_sub(b, e), _C1))))


def _phi(t):
    return jnp.where(t > 0, t + 1.0, jnp.exp(t)) + 1e-6


def _dot(a, b):
    return jnp.dot(a, b, preferred_element_type=F32)


def _dot_nt(a, b):
    return lax_dot_general(a, b, (((1,), (1,)), ((), ())), preferred_element_type=F32)


lax_dot_general = jax.lax.dot_general


def _interleave(main, side):
    done = 0
    for i, task in enumerate(main):
        task()
        upto = (len(side) * (i + 1)) // len(main)
        for t in side[done:upto]:
            t()
        done = upto


def _kernel(x_hbm, wqkv_hbm, wo_hbm, q_hbm, k_hbm, v_hbm, sk_ref, h_hbm, d_ref, fwd_hbm, inv_hbm,
            out_hbm,
            x_v, wq_v, wk_v, wv_v, wo_v, q_v, k_v, v_v, h_v, fwd_v, inv_v,
            wkt_s, pkt_s, g_s, m_s, zb_s, r_s, oa_s, ob_s,
            kf_s, u_s, ht_s, y_s, a_s, b_s, sems):
    sem_count = [0]

    def copy(src, dst):
        c = pltpu.make_async_copy(src, dst, sems.at[sem_count[0]])
        sem_count[0] += 1
        return c

    def cols(ref, start, size):
        return ref.at[:, pl.ds(start, size)]

    def rows(ref, start, size):
        return ref.at[pl.ds(start, size), :]

    n_tc = S // TC
    n_p1 = D // KB
    cp_x = [copy(rows(x_hbm, c * TC, TC), rows(x_v, c * TC, TC)) for c in range(n_tc)]
    cp_wq = copy(cols(wqkv_hbm, 0, D), wq_v)
    cp_wk = [copy(cols(wqkv_hbm, D + i * KB, KB), wk_v.at[i]) for i in range(n_p1)]
    cp_wv = [copy(cols(wqkv_hbm, 2 * D + i * KB, KB), wv_v.at[i]) for i in range(n_p1)]
    cp_wo = [copy(rows(wo_hbm, i * KB, KB), rows(wo_v, i * KB, KB)) for i in range(n_p1)]
    cp_q = [copy(cols(q_hbm, i * CB, CB), q_v.at[i]) for i in range(NB)]
    cp_k = [copy(cols(k_hbm, i * CB, CB), k_v.at[i]) for i in range(NB)]
    cp_v = [copy(cols(v_hbm, i * CB, CB), v_v.at[i]) for i in range(NB)]
    cp_h = [copy(rows(h_hbm, i * CB, CB), h_v.at[i]) for i in range(NB)]
    cp_fwd = copy(fwd_hbm, fwd_v)
    cp_inv = copy(inv_hbm, inv_v)
    cp_oa = [copy(rows(oa_s, c * TC, TC), out_hbm.at[pl.ds(c * TC, TC), pl.ds(0, D)]) for c in range(n_tc)]
    cp_ob = [copy(ob_s.at[i], cols(out_hbm, D + i * CB, CB)) for i in range(NB)]

    RP = 256

    def b_prep(i):
        def widen(p):
            def run():
                if p == 0:
                    cp_k[i].wait()
                    cp_v[i].wait()
                kf_s[pl.ds(HALO + p * RP, RP), :] = k_v[i, pl.ds(p * RP, RP), :].astype(F32)
            return run

        def gate(p):
            def run():
                taps = sk_ref[:, pl.ds(i * CB, CB)].astype(F32)
                acc = kf_s[pl.ds(HALO + p * RP, RP), :] * taps[0:1, :]
                for j in range(1, 4):
                    acc = acc + kf_s[pl.ds(HALO + p * RP - j, RP), :] * taps[j:j + 1, :]
                u_s[pl.ds(p * RP, RP), :] = acc * v_v[i, pl.ds(p * RP, RP), :].astype(F32)
            return run

        def transpose(p):
            def run():
                if p == 0:
                    cp_h[i].wait()
                ht_s[pl.ds(p * RP, RP), :] = h_v[i, :, pl.ds(p * RP, RP)].T.astype(F32)
            return run

        tasks = []
        for p in range(S // RP):
            tasks += [widen(p), gate(p), transpose(p)]
        return tasks

    def b_fwd(i):
        def column(src, lane0, j):
            def run():
                def emit(k2, re, im):
                    a_s[k2, pl.ds(16 * j, 16), pl.ds(lane0, CB)] = jnp.concatenate([re, im], axis=0).astype(BF)
                _dft32_fwd(lambda n2: src[pl.ds(N1 * n2 + 8 * j, 8), :], emit)
            return run
        return [column(src, lane0, j) for j in range(N1 // 8) for src, lane0 in ((u_s, 0), (ht_s, CB))]

    def b_mid(i):
        def one(k2):
            def run():
                if i == 0 and k2 == 0:
                    cp_fwd.wait()
                    cp_inv.wait()
                xf = _dot(fwd_v[k2], a_s[k2])
                ur, ui, hr, hi = xf[:N1, :CB], xf[N1:, :CB], xf[:N1, CB:], xf[N1:, CB:]
                y = jnp.concatenate([ur * hr - ui * hi, ur * hi + ui * hr], axis=0).astype(BF)
                b_s[k2] = _dot(inv_v[k2], y)
            return run
        return [one(k2) for k2 in range(N2)]

    def b_inv(i):
        def column(j):
            def run():
                def emit(n2, val):
                    y_s[pl.ds(N1 * n2 + 8 * j, 8), :] = val
                _dft32_inv(lambda k2: (b_s[k2, pl.ds(16 * j, 8), :], b_s[k2, pl.ds(16 * j + 8, 8), :]), emit)
            return run

        def post(p):
            def run():
                if p == 0:
                    cp_q[i].wait()
                r = pl.ds(p * RP, RP)
                skip = d_ref[:, pl.ds(i * CB, CB)].astype(F32)
                ob_s[i, r, :] = (q_v[i, r, :].astype(F32) * (y_s[r, :] + u_s[r, :] * skip)).astype(BF)
                if p == S // RP - 1:
                    cp_ob[i].start()
            return run
        return [column(j) for j in range(N1 // 8)] + [post(p) for p in range(S // RP)]

    def head_mask():
        r = jax.lax.broadcasted_iota(jnp.int32, (128, 128), 0) // DH
        c = jax.lax.broadcasted_iota(jnp.int32, (128, 128), 1) // DH
        return r == c

    def a1_keys(i):
        zacc = [None]

        def chunk(c):
            def run():
                if c == 0:
                    cp_wk[i].wait()
                    wkt_s[...] = wk_v[i].T
                if i == 0:
                    cp_x[c].wait()
                pk = _phi(_dot_nt(wkt_s[...], x_v[pl.ds(c * TC, TC), :]))
                pkt_s[:, pl.ds(c * TC, TC)] = pk.astype(BF)
                part = pk[:, :128]
                for t in range(1, TC // 128):
                    part = part + pk[:, t * 128:(t + 1) * 128]
                zacc[0] = part if c == 0 else zacc[0] + part
                if c == n_tc - 1:
                    z = jnp.sum(zacc[0], axis=1, keepdims=True)
                    for g in range(KB // 128):
                        zg = jnp.broadcast_to(z[g * 128:(g + 1) * 128], (128, 128))
                        zb_s[i * (KB // 128) + g] = jnp.where(head_mask(), zg, 0.0).astype(BF)
            return run
        return [chunk(c) for c in range(n_tc)]

    def a1_gram(i):
        def chunk(c):
            def run():
                g_s[:, pl.ds(c * 256, 256)] = _dot(pkt_s[...], x_v[:, pl.ds(c * 256, 256)]).astype(BF)
            return run
        return [chunk(c) for c in range(D // 256)]

    def a1_mix(i):
        def group(g):
            def run():
                if g == 0:
                    cp_wv[i].wait()
                    cp_wo[i].wait()
                kv = _dot(g_s[pl.ds(g * 128, 128), :], wv_v[i, :, pl.ds(g * 128, 128)])
                kv = jnp.where(head_mask(), kv, 0.0).astype(BF)
                r = pl.ds(i * KB + g * 128, 128)
                m_s[r, :] = _dot(kv, wo_v[r, :]).astype(BF)
            return run
        return [group(g) for g in range(KB // 128)]

    def a2_query(c):
        def chunk(n):
            def run():
                if c == 0 and n == 0:
                    cp_wq.wait()
                pq = _phi(_dot(x_v[pl.ds(c * TC, TC), :], wq_v[:, pl.ds(n * 256, 256)]))
                pqb = pq.astype(BF)
                den = jnp.concatenate(
                    [_dot(pqb[:, g * 128:(g + 1) * 128], zb_s[2 * n + g]) for g in range(2)], axis=1) + 1e-6
                r_s[c % 2, :, pl.ds(n * 256, 256)] = (pq / den).astype(BF)
            return run
        return [chunk(n) for n in range(D // 256)]

    def a2_out(c):
        def chunk(n):
            def run():
                oa_s[pl.ds(c * TC, TC), pl.ds(n * 256, 256)] = _dot(
                    r_s[c % 2], m_s[:, pl.ds(n * 256, 256)]).astype(BF)
                if n == D // 256 - 1:
                    cp_oa[c].start()
            return run
        return [chunk(n) for n in range(D // 256)]

    def start_block_inputs(i):
        for c in (cp_k[i], cp_v[i], cp_h[i], cp_q[i]):
            c.start()

    for c in [cp_wk[0], cp_x[0], cp_k[0], cp_v[0], cp_x[1], cp_h[0]] + cp_x[2:] + [cp_fwd, cp_inv, cp_q[0]]:
        c.start()
    kf_s[pl.ds(0, HALO), :] = jnp.zeros((HALO, CB), F32)

    for i in range(NB):
        if i + 1 < NB:
            start_block_inputs(i + 1)
        if i < n_p1:
            cp_wv[i].start()
            cp_wo[i].start()
            if i + 1 < n_p1:
                cp_wk[i + 1].start()
            if i == 1:
                cp_wq.start()
            first = a1_keys(i)
            if i > 0:
                first = first[:1] + a1_mix(i - 1) + first[1:]
            second = a1_gram(i)
        else:
            c0 = 2 * (i - n_p1)
            first = a2_query(c0) + a2_query(c0 + 1)
            if i == n_p1:
                first = a1_mix(n_p1 - 1) + first
            second = a2_out(c0) + a2_out(c0 + 1)
        _interleave(first, (b_prep(0) if i == 0 else []) + b_fwd(i))
        for t in b_mid(i):
            t()
        _interleave(second, b_inv(i) + (b_prep(i + 1) if i + 1 < NB else []))

    for c in cp_oa + cp_ob:
        c.wait()


@jax.jit
def pallas_concat_heads__linear_attn_block__ssm_conv_h3__prompt_kernel(
    A_x: jax.Array,
    A_wqkv: jax.Array,
    A_wo: jax.Array,
    B_q: jax.Array,
    B_k: jax.Array,
    B_v: jax.Array,
    B_shift_k: jax.Array,
    B_ssm_k: jax.Array,
    B_ssm_D: jax.Array,
):
    hbm = pl.BlockSpec(memory_space=pl.ANY)
    vmem = pl.BlockSpec(memory_space=pltpu.VMEM)
    n_p1 = D // KB
    scratch = [
        pltpu.VMEM((S, D), BF),
        pltpu.VMEM((D, D), BF),
        pltpu.VMEM((n_p1, D, KB), BF),
        pltpu.VMEM((n_p1, D, KB), BF),
        pltpu.VMEM((D, D), BF),
        pltpu.VMEM((NB, S, CB), BF),
        pltpu.VMEM((NB, S, CB), BF),
        pltpu.VMEM((NB, S, CB), BF),
        pltpu.VMEM((NB, CB, S), BF),
        pltpu.VMEM((N2, 128, 128), BF),
        pltpu.VMEM((N2, 128, 128), BF),
        pltpu.VMEM((KB, D), BF),
        pltpu.VMEM((KB, S), BF),
        pltpu.VMEM((KB, D), BF),
        pltpu.VMEM((D, D), BF),
        pltpu.VMEM((D // 128, 128, 128), BF),
        pltpu.VMEM((2, TC, D), BF),
        pltpu.VMEM((S, D), BF),
        pltpu.VMEM((NB, S, CB), BF),
        pltpu.VMEM((HALO + S, CB), F32),
        pltpu.VMEM((S, CB), F32),
        pltpu.VMEM((S, CB), F32),
        pltpu.VMEM((S, CB), F32),
        pltpu.VMEM((N2, 128, 2 * CB), BF),
        pltpu.VMEM((N2, 128, CB), F32),
        pltpu.SemaphoreType.DMA((80,)),
    ]
    out = pl.pallas_call(
        _kernel,
        out_shape=jax.ShapeDtypeStruct((S, 2 * D), BF),
        in_specs=[hbm, hbm, hbm, hbm, hbm, hbm, vmem, hbm, vmem, hbm, hbm],
        out_specs=hbm,
        scratch_shapes=scratch,
        compiler_params=pltpu.CompilerParams(vmem_limit_bytes=100 * 1024 * 1024),
    )(A_x.reshape(S, D), A_wqkv, A_wo, B_q.reshape(S, D), B_k.reshape(S, D), B_v.reshape(S, D),
      B_shift_k.T, B_ssm_k, B_ssm_D.reshape(1, D), _FWD, _INV)
    return out.reshape(1, S, 2 * D)
```

```python
import numpy as np
import jax
import jax.numpy as jnp
import jax.experimental.pallas as pl
import jax.experimental.pallas.tpu as pltpu

S = 2048
D = 1024
DH = 32
N1, N2 = 64, 32
CB = 128
NB = D // CB
NT = D // 128
OC = 256
HALO = 8
NZ = 32
V_LEAD, V_TRAIL, M_TRAIL = {0: 600}, {NB + 1: 1500}, 300
REGION_BIAS = [0] * (NB + 2)
REGIONS = range(NB + 2)
DBG = ''
FENCE, FROW = 1, 0
BF = jnp.bfloat16
F32 = jnp.float32


def _dft_matrices():
    n1 = np.arange(N1)
    k1 = np.arange(N1)
    col = 16 * (n1 // 8) + (n1 % 8)
    fwd = np.zeros((N2, 2 * N1, 2 * N1), np.float64)
    for k2 in range(N2):
        e = np.exp(-2j * np.pi * np.outer(N2 * k1 + k2 + 0.25, n1) / S)
        fwd[k2][:N1, col] = e.real
        fwd[k2][:N1, col + 8] = -e.imag
        fwd[k2][N1:, col] = e.imag
        fwd[k2][N1:, col + 8] = e.real
    inv = np.transpose(fwd, (0, 2, 1)) / S
    return fwd.astype(np.float32).astype(BF), inv.astype(np.float32).astype(BF)


_FWD, _INV = _dft_matrices()


def _add(a, b):
    (sa, xa), (sb, xb) = a, b
    if sa == sb:
        return (sa, xa + xb)
    return (1, xa - xb) if sa > 0 else (1, xb - xa)


def _neg(a):
    return (-a[0], a[1])


def _sub(a, b):
    return _add(a, _neg(b))


def _scale(a, c):
    return (1, a[1] * np.float32(a[0] * c))


def _val(a):
    return a[1] if a[0] > 0 else -a[1]


def _cadd(a, b):
    return (_add(a[0], b[0]), _add(a[1], b[1]))


def _csub(a, b):
    return (_sub(a[0], b[0]), _sub(a[1], b[1]))


def _cmul_i(a, s):
    return (_neg(a[1]), a[0]) if s > 0 else (a[1], _neg(a[0]))


def _cmul_const(a, w):
    c, s = float(np.real(w)), float(np.imag(w))
    return (_add(_scale(a[0], c), _scale(a[1], -s)), _add(_scale(a[0], s), _scale(a[1], c)))


def _fft4(x, s):
    a0, a1 = _cadd(x[0], x[2]), _cadd(x[1], x[3])
    b0, b1 = _csub(x[0], x[2]), _cmul_i(_csub(x[1], x[3]), s)
    return [_cadd(a0, a1), _cadd(b0, b1), _csub(a0, a1), _csub(b0, b1)]


def _fft8(x, s):
    r = np.sqrt(0.5)
    a = [_cadd(x[n], x[n + 4]) for n in range(4)]
    b = [_csub(x[n], x[n + 4]) for n in range(4)]
    t = _cadd(b[1], _cmul_i(b[1], s))
    b[1] = (_scale(t[0], r), _scale(t[1], r))
    b[2] = _cmul_i(b[2], s)
    t = _csub(_cmul_i(b[3], s), b[3])
    b[3] = (_scale(t[0], r), _scale(t[1], r))
    ev, od = _fft4(a, s), _fft4(b, s)
    return [ev[0], od[0], ev[1], od[1], ev[2], od[2], ev[3], od[3]]


_C1, _S1, _R2 = np.cos(np.pi / 8), np.sin(np.pi / 8), np.sqrt(0.5)


def _tw(n, j, s):
    return np.exp(s * 2j * np.pi * n * (4 * j + 1) / 128)


def _fwd_stage1(n, u0, u1, u2, u3):
    u0, u1, u2, u3 = (1, u0), (1, u1), (1, u2), (1, u3)
    t = _scale(u2, _R2)
    p, m_ = _add(u0, t), _sub(u0, t)
    c1u1, s1u1, c1u3, s1u3 = _scale(u1, _C1), _scale(u1, _S1), _scale(u3, _C1), _scale(u3, _S1)
    a, b = _add(c1u1, s1u3), _add(s1u1, c1u3)
    d, e = _sub(c1u1, s1u3), _sub(s1u1, c1u3)
    sj = [(_add(p, a), _neg(_add(t, b))), (_sub(m_, e), _sub(t, d)),
          (_sub(p, a), _sub(b, t)), (_add(m_, e), _add(t, d))]
    out = [sj[j] if n == 0 else _cmul_const(sj[j], _tw(n, j, -1)) for j in range(4)]
    return [(_val(re), _val(im)) for re, im in out]


def _fwd_stage2(t):
    out = _fft8([((1, re), (1, im)) for re, im in t], -1)
    return [(_val(re), _val(im)) for re, im in out]


def _inv_stage1(j, b):
    out = _fft8([((1, re), (1, im)) for re, im in b], 1)
    out = [out[n] if n == 0 else _cmul_const(out[n], _tw(n, j, 1)) for n in range(8)]
    return [(_val(re), _val(im)) for re, im in out]


def _inv_stage2(s):
    (x0, y0), (x1, y1), (x2, y2), (x3, y3) = [((1, re), (1, im)) for re, im in s]
    p, a, b = _add(x0, x2), _sub(x0, x2), _sub(y2, y0)
    m_, e, d = _add(x1, x3), _sub(x3, x1), _sub(y3, y1)
    t = _add(_sub(_add(y1, y3), _add(y0, y2)), _sub(p, m_))
    return [_val(_add(p, m_)),
            _val(_add(_scale(_add(a, d), _C1), _scale(_add(b, e), _S1))),
            _val(_scale(t, _R2)),
            _val(_add(_scale(_sub(a, d), _S1), _scale(_sub(b, e), _C1)))]


def _phi(t):
    return jnp.where(t > 0, t + 1.0, jnp.exp(t)) + 1e-6


def _dot(a, b):
    return jnp.dot(a, b, preferred_element_type=F32)


def _dot_nt(a, b):
    return jax.lax.dot_general(a, b, (((1,), (1,)), ((), ())), preferred_element_type=F32)


def _ld(ref, lead, r0, n):
    lead = lead if isinstance(lead, tuple) else (lead,)
    return pltpu.bitcast(ref.bitcast(jnp.uint32)[(*lead, pl.ds(r0 // 2, n // 2), slice(None))], BF)


def _cat(parts, axis):
    return parts[0] if len(parts) == 1 else jnp.concatenate(parts, axis=axis)


def _spread(stream, extra):
    out = []
    extra = sorted(extra, key=lambda e: e[0])
    e = 0
    for pos, item in enumerate(stream):
        while e < len(extra) and extra[e][0] <= pos:
            out.append(extra[e][1])
            e += 1
        out.append(item)
    return out + [t for _, t in extra[e:]]


def _kernel(zero_ref, x_hbm, wqkv_hbm, wo_hbm, q_hbm, k_hbm, v_hbm, sk_ref, h_hbm, d_ref, fwd_hbm, inv_hbm,
            out_hbm,
            x_v, wq_v, wk_v, wv_v, wo_v, q_v, k_v, v_v, h_v, fwd_v, inv_v,
            wkt_s, pkt_s, g_s, kv_s, m_s, zb_s, pq_s, r_s, oa_s, ob_s,
            kf_s, u_s, ht_s, tf_s, a_s, yf_s, b_s, ti_s, z_s, sems):
    n_sem = [0]

    def zero(i):
        return zero_ref[i % NZ]

    def group(pairs):
        sem = sems.at[n_sem[0]]
        n_sem[0] += 1
        return [pltpu.make_async_copy(src, dst, sem) for src, dst in pairs]

    def start(g):
        for c in g:
            c.start()

    def wait(g):
        for c in (g if 'nodma' not in DBG else []):
            c.wait()

    def col(ref, j):
        return ref.at[:, pl.ds(j * 128, 128)]

    x_edges = [0, 256, 512, 1024, S]
    cp_x = {r0: group([(x_hbm.at[pl.ds(r0, r1 - r0), pl.ds(j * 128, 128)], x_v.at[j, pl.ds(r0, r1 - r0), :])
                       for j in range(NT)]) for r0, r1 in zip(x_edges[:-1], x_edges[1:])}
    cp_wq = group([(col(wqkv_hbm, j), wq_v.at[j]) for j in range(NT)])
    cp_wk = [group([(col(wqkv_hbm, NT + g), wk_v.at[g])]) for g in range(NT)]
    cp_wv = group([(col(wqkv_hbm, 2 * NT + g), wv_v.at[g]) for g in range(NT)])
    cp_wo = group([(col(wo_hbm, j), wo_v.at[j]) for j in range(NT)])
    cp_q = [group([(col(q_hbm, i), q_v.at[i])]) for i in range(NB)]
    cp_kv = [group([(col(k_hbm, i), k_v.at[i]), (col(v_hbm, i), v_v.at[i])]) for i in range(NB)]
    cp_h = [group([(h_hbm.at[pl.ds(i * CB, CB), :], h_v.at[i])]) for i in range(NB)]
    cp_dft = group([(fwd_hbm, fwd_v), (inv_hbm, inv_v)])
    cp_oa = [group([(oa_s.at[pl.ds(c * OC, OC), :], out_hbm.at[pl.ds(c * OC, OC), pl.ds(0, D)])])
             for c in range(S // OC)]
    cp_ob = [group([(ob_s.at[i], col(out_hbm, NT + i))]) for i in range(NB)]

    RP = 128

    def b_forward(i):
        def widen(p):
            def run():
                if p == 0:
                    wait(cp_kv[i])
                kf_s[pl.ds(HALO + p * RP, RP), :] = _ld(k_v, i, p * RP, RP).astype(F32)
            return 16, run

        def gate(p):
            def run():
                taps = sk_ref[:, pl.ds(i * CB, CB)].astype(F32)
                acc = kf_s[pl.ds(HALO + p * RP, RP), :] * taps[0:1, :]
                for j in range(1, 4):
                    acc = acc + kf_s[pl.ds(HALO + p * RP - j, RP), :] * taps[j:j + 1, :]
                u_s[pl.ds(p * RP, RP), :] = acc * _ld(v_v, i, p * RP, RP).astype(F32)
            return 150, run

        def transpose(p):
            def run():
                if p == 0:
                    wait(cp_h[i])
                ht = h_v[i, :, pl.ds(p * RP, RP)].astype(F32).T
                if p == 0:
                    skip = d_ref[:, pl.ds(i * CB, CB)].astype(F32)
                    lag = jax.lax.broadcasted_iota(jnp.int32, (RP, CB), 0)
                    ht = ht + jnp.where(lag == 0, skip, 0.0)
                ht_s[pl.ds(p * RP, RP), :] = ht
            return 40, run

        def stage1(src, h, j, n):
            def run():
                out = _fwd_stage1(n, *[src[pl.ds(N1 * (n + 8 * m) + 8 * j, 8), :] for m in range(4)])
                for r in range(4):
                    tf_s[h, j, pl.ds(16 * (8 * r + n), 8), :] = out[r][0]
                    tf_s[h, j, pl.ds(16 * (8 * r + n) + 8, 8), :] = out[r][1]
            return (43 if n else 21), run

        def stage2(h, j, r):
            def run():
                out = _fwd_stage2([(tf_s[h, j, pl.ds(16 * (8 * r + n), 8), :],
                                    tf_s[h, j, pl.ds(16 * (8 * r + n) + 8, 8), :]) for n in range(8)])
                for l in range(8):
                    a_s[i % 2, h, r + 4 * l, pl.ds(16 * j, 16), :] = _cat(out[l], 0).astype(BF)
            return 64, run

        tasks = [transpose(p) for p in range(S // RP)] if 'notr' not in DBG else []
        prep = [widen(0)]
        for p in range(S // RP):
            prep += ([widen(p + 1)] if p + 1 < S // RP else []) + [gate(p)]
        cols = [(ht_s, 1, j) for j in range(N1 // 8)] + [(u_s, 0, j) for j in range(N1 // 8)]
        for c, (src, h, j) in enumerate(cols):
            tasks += [stage1(src, h, j, n) for n in range(8)]
            if c < 8 and 'noprep' not in DBG:
                tasks += prep[4 * c:4 * c + 4]
            if c > 0:
                tasks += [stage2(cols[c - 1][1], cols[c - 1][2], r) for r in range(4)]
        return tasks + [stage2(cols[-1][1], cols[-1][2], r) for r in range(4)]

    def b_inverse(i):
        def stage1(j, r):
            def run():
                out = _inv_stage1(r, [(b_s[i % 2, r + 4 * l, pl.ds(16 * j, 8), :],
                                       b_s[i % 2, r + 4 * l, pl.ds(16 * j + 8, 8), :]) for l in range(8)])
                for n in range(8):
                    ti_s[j, pl.ds(16 * (4 * n + r), 8), :] = out[n][0]
                    ti_s[j, pl.ds(16 * (4 * n + r) + 8, 8), :] = out[n][1]
            return 98, run

        def stage2(jp, n, last):
            def run():
                if jp == 0 and n == 0:
                    wait(cp_q[i])
                ys = [_inv_stage2([(ti_s[j, pl.ds(16 * (4 * n + r), 8), :],
                                    ti_s[j, pl.ds(16 * (4 * n + r) + 8, 8), :]) for r in range(4)])
                      for j in (2 * jp, 2 * jp + 1)]
                for m in range(4):
                    r0 = N1 * (n + 8 * m) + 16 * jp
                    y = _cat([ys[0][m], ys[1][m]], 0)
                    ob_s[i, pl.ds(r0, 16), :] = (_ld(q_v, i, r0, 16).astype(F32) * y).astype(BF)
                if last:
                    start(cp_ob[i])
            return 66, run

        tasks = []
        for jp in range(N1 // 16 + 1):
            if jp < N1 // 16:
                tasks += [stage1(j, r) for j in (2 * jp, 2 * jp + 1) for r in range(4)]
            if jp > 0:
                tasks += [stage2(jp - 1, n, jp == N1 // 16 and n == 7) for n in range(8)]
        return tasks

    def b_middle(i):
        def forward(k2):
            def run():
                if i == 0 and k2 == 0:
                    wait(cp_dft)
                rhs = _cat([_ld(a_s, (i % 2, h, k2), 0, 128) for h in range(2)], 1)
                xf = _dot(_ld(fwd_v, k2 + zero(i), 0, 128), rhs)
                ur, ui, hr, hi = xf[:N1, :CB], xf[N1:, :CB], xf[:N1, CB:], xf[N1:, CB:]
                yf_s[k2] = _cat([ur * hr - ui * hi, ur * hi + ui * hr], 0).astype(BF)
            return 64, run

        def inverse(k2):
            def run():
                b_s[i % 2, k2] = _dot(_ld(inv_v, k2 + zero(i), 0, 128), _ld(yf_s, k2, 0, 128))
            return 32, run

        tasks = []
        for k4 in range(N2 // 4 + 1):
            if k4 < N2 // 4:
                tasks += [[forward(4 * k4), forward(4 * k4 + 1)], [forward(4 * k4 + 2), forward(4 * k4 + 3)]]
            if k4 > 0:
                tasks += [[inverse(4 * k4 - 4 + r) for r in range(4)]]
        return tasks

    def head_mask():
        r = jax.lax.broadcasted_iota(jnp.int32, (128, 128), 0) // DH
        c = jax.lax.broadcasted_iota(jnp.int32, (128, 128), 1) // DH
        return r == c

    mid_chain = set()

    n_piece = [0]

    def fence(value):
        for ref in (kf_s, u_s, ht_s):
            ref[pl.ds(pl.multiple_of(zero(0) + (ref.shape[0] - 8), 8), 8), :] = value
        for ref in (tf_s, b_s, ti_s):
            lead = (zero(0) + (ref.shape[0] - 1),) + (0,) * (len(ref.shape) - 3)
            ref[(*lead, pl.ds(0, 8), slice(None))] = value
        yf_s.bitcast(jnp.uint32)[zero(0) + N2, pl.ds(0, 8), :] = pltpu.bitcast(value, jnp.uint32)

    def chain(n_k, operands, dot, finish, before=None):
        acc = [None]

        def piece(kk):
            def run():
                if before is not None:
                    before(kk)
                d = dot(*operands(kk))
                acc[0] = d if kk == 0 else acc[0] + d
                n_piece[0] += 1
                if n_piece[0] % FENCE == 0:
                    fence(d[FROW:FROW + 8, :128])
                if kk == n_k - 1:
                    finish(acc[0])
            if kk > 0:
                mid_chain.add(run)
            return 128, run
        return [piece(kk) for kk in range(n_k)]

    def a_transpose_wk(g):
        def run():
            wait(cp_wk[g])
            for j in range(NT):
                wkt_s[g, j] = wk_v[g, pl.ds(j * 128, 128), :].astype(F32).T.astype(BF)
        return 0, run

    def a_keys(g):
        def block(c):
            def before(kk):
                if g == 0 and kk == 0 and c * 256 in cp_x:
                    wait(cp_x[c * 256])

            def operands(kk):
                js = (2 * kk, 2 * kk + 1)
                return (_cat([_ld(wkt_s, (g + zero(c), j), 0, 128) for j in js], 1),
                        _cat([_ld(x_v, j + zero(g), c * 256, 256) for j in js], 1))

            def finish(acc):
                pk = _phi(acc)
                pkt_s[g, 2 * c] = pk[:, :128].astype(BF)
                pkt_s[g, 2 * c + 1] = pk[:, 128:].astype(BF)
                part = pk[:, :128] + pk[:, 128:]
                if c < S // 256 - 1:
                    z_s[g, c] = part
                else:
                    for b in range(c):
                        part = part + z_s[g, b]
                    z = jnp.broadcast_to(jnp.sum(part, axis=1, keepdims=True), (128, 128))
                    zb_s[g] = jnp.where(head_mask(), z, 0.0).astype(BF)
            return chain(D // 256, operands, _dot_nt, finish, before)
        return [t for c in range(S // 256) for t in block(c)]

    def a_gram(g):
        def block(n):
            def operands(kk):
                return (_cat([_ld(pkt_s, (g, 2 * kk + t), 0, 128) for t in range(2)], 1),
                        _cat([_ld(x_v, 2 * n + t + zero(NT + g), kk * 256, 256) for t in range(2)], 1))

            def finish(acc):
                g_s[g, 2 * n] = acc[:, :128].astype(BF)
                g_s[g, 2 * n + 1] = acc[:, 128:].astype(BF)
            return chain(S // 256, operands, _dot, finish)
        return [t for n in range(D // 256) for t in block(n)]

    def a_kv(g):
        def run():
            if g == 0:
                wait(cp_wv)
            kv = _dot(_cat([_ld(g_s, (g, j), 0, 128) for j in range(NT)], 1), _ld(wv_v, g, 0, D))
            kv_s[g] = jnp.where(head_mask(), kv, 0.0).astype(BF)
        return 256, run

    def a_mix(g, half):
        def run():
            if g == 0 and half == 0:
                wait(cp_wo)
            js = range(4 * half, 4 * half + 4)
            m = _dot(_ld(kv_s, g, 0, 128), _cat([_ld(wo_v, j, g * 128, 128) for j in js], 1))
            for t, j in enumerate(js):
                m_s[j, pl.ds(g * 128, 128), :] = m[:, t * 128:(t + 1) * 128].astype(BF)
        return 128, run

    def a_query(c, n):
        def operands(kk):
            return (_cat([_ld(x_v, 2 * kk + t + zero(2 * NT + n), c * 128, 128) for t in range(2)], 1),
                    _cat([_ld(wq_v, 2 * n + t + zero(c), kk * 256, 256) for t in range(2)], 1))

        def before(kk):
            if c == 0 and n == 0 and kk == 0:
                wait(cp_wq)

        def finish(acc):
            pq = _phi(acc)
            pq_s[c, 2 * n] = pq[:, :128].astype(BF)
            pq_s[c, 2 * n + 1] = pq[:, 128:].astype(BF)
        return chain(D // 256, operands, _dot, finish, before)

    def a_normalise(c, n):
        def run():
            for g in (2 * n, 2 * n + 1):
                pq = _ld(pq_s, (c, g), 0, 128)
                den = _dot(pq, _ld(zb_s, g + zero(c), 0, 128)) + 1e-6
                inv = pl.reciprocal(den, approx=True)
                inv = inv * (2.0 - den * inv)
                r_s[c, g] = (pq.astype(F32) * inv).astype(BF)
        return 64, run

    def a_out(c, n):
        def operands(kk):
            return (_cat([_ld(r_s, (c, 2 * kk + t), 0, 128) for t in range(2)], 1),
                    _cat([_ld(m_s, 2 * n + t + zero(c), kk * 256, 256) for t in range(2)], 1))

        def finish(acc):
            oa_s[pl.ds(c * 128, 128), pl.ds(n * 256, 256)] = acc.astype(BF)
            if n == D // 256 - 1 and (c + 1) * 128 % OC == 0:
                start(cp_oa[c * 128 // OC])
        return chain(D // 256, operands, _dot, finish)

    def starter(*groups):
        def run():
            for g in groups:
                start(g)
        return 0, run

    a_stream = []
    for g in range(NT):
        extra = [(12, a_transpose_wk(g + 1))] if g + 1 < NT else []
        if g > 0:
            extra += [(4, a_kv(g - 1)), (8, a_mix(g - 1, 0)), (8, a_mix(g - 1, 1))]
        if g + 2 < NT:
            extra += [(0, starter(cp_wk[g + 2]))]
        if g == 0:
            extra += [(16, starter(cp_dft)), (28, starter(cp_wv, cp_wo))]
        if g == 2:
            extra += [(0, starter(cp_wq))]
        a_stream += _spread(a_keys(g), extra) + a_gram(g)
    n_c = S // 128
    for c in range(n_c + 1):
        stream, extra = [], []
        if c < n_c:
            stream += [t for n in range(D // 256) for t in a_query(c, n)]
            extra += [(4 * n + 8, a_normalise(c, n)) for n in range(D // 256 - 1)]
        if c == 0:
            extra += [(4, a_kv(NT - 1)), (8, a_mix(NT - 1, 0)), (8, a_mix(NT - 1, 1))]
        if c > 0:
            extra += [(4, a_normalise(c - 1, D // 256 - 1))]
            outs = [t for n in range(D // 256) for t in a_out(c - 1, n)]
            stream = stream + outs if c < n_c else _spread(outs, [(0, extra.pop()[1])])
        a_stream += _spread(stream, extra)

    v_regions, m_regions = [], []
    for r in range(NB + 2):
        v = [starter(cp_h[r + 1], cp_kv[r + 1])] if r + 1 < NB and 'nodma' not in DBG else []
        v += [starter(cp_q[r - 1])] if 1 <= r <= NB and 'nodma' not in DBG else []
        v += b_inverse(r - 2) if r >= 2 else []
        v += b_forward(r) if r < NB else []
        v_regions.append(v)
        m_regions.append(b_middle(r - 1) if 1 <= r <= NB and 'nomid' not in DBG else [])
    v_cost = [sum(c for c, _ in v) for v in v_regions]
    m_cost = [sum(c for grp in m for c, _ in grp) for m in m_regions]
    total = sum(c for c, _ in a_stream) + sum(m_cost)
    weight = [c + w for c, w in zip(v_cost, REGION_BIAS)]

    for g in (cp_wk[0], cp_x[0], cp_h[0], cp_x[256], cp_kv[0], cp_x[512], cp_wk[1], cp_x[1024]):
        start(g)
    kf_s[pl.ds(0, HALO), :] = jnp.zeros((HALO, CB), F32)
    for ref in (pkt_s, r_s, g_s, kv_s, pq_s, a_s, z_s):
        lead = (zero(0),) + (0,) * (len(ref.shape) - 3)
        ref[(*lead, pl.ds(0, 16), slice(None))] = jnp.zeros((16, CB), ref.dtype)
    a_transpose_wk(0)[1]()

    ai, clock = 0, 0
    for r in range(NB + 2):
        end = total * sum(weight[:r + 1]) / sum(weight)
        a_end, t = ai, clock + m_cost[r]
        while a_end < len(a_stream) and (t < end or a_stream[a_end][1] in mid_chain or r == NB + 1):
            t += a_stream[a_end][0]
            a_end += 1
        length = t - clock
        v, m = v_regions[r], m_regions[r]
        lead, trail = V_LEAD.get(r, 0), V_TRAIL.get(r, 0)
        v_time, acc_cost = [], 0
        for c, _ in v:
            v_time.append(lead + (length - lead - trail) * acc_cost / v_cost[r])
            acc_cost += c

        def region():
            now, pa, pm, pv = 0, ai, 0, 0
            while pa < a_end or pm < len(m):
                if pm < len(m) and ((length - M_TRAIL) * pm / len(m) <= now or pa == a_end):
                    todo = m[pm]
                    pm += 1
                else:
                    todo = [a_stream[pa]]
                    pa += 1
                for cost, run in todo:
                    run()
                    now += cost
                while pv < len(v) and v_time[pv] <= now:
                    v[pv][1]()
                    pv += 1
            for _, run in v[pv:]:
                run()

        if r in REGIONS:
            if 'loop' in DBG:
                jax.lax.fori_loop(0, zero(r) + 1, lambda _, c: (region(), c)[1], 0)
            else:
                pl.when(zero(r) == 0)(region)
        ai, clock = a_end, t

    if len(REGIONS) < NB + 2:
        for ref in (pkt_s, r_s, g_s, kv_s, pq_s, tf_s, a_s, yf_s, b_s, ti_s, z_s, m_s, zb_s, ob_s, wkt_s):
            lead = (zero(1),) + (0,) * (len(ref.shape) - 3)
            oa_s[pl.ds(0, 16), pl.ds(0, 128)] += ref[(*lead, pl.ds(0, 16), slice(None))].astype(BF)
        start(cp_oa[0])
    for g in cp_oa + cp_ob:
        wait(g)


@jax.jit
def pallas_concat_heads__linear_attn_block__ssm_conv_h3__prompt_kernel(
    A_x: jax.Array,
    A_wqkv: jax.Array,
    A_wo: jax.Array,
    B_q: jax.Array,
    B_k: jax.Array,
    B_v: jax.Array,
    B_shift_k: jax.Array,
    B_ssm_k: jax.Array,
    B_ssm_D: jax.Array,
):
    hbm = pl.BlockSpec(memory_space=pl.ANY)
    vmem = pl.BlockSpec(memory_space=pltpu.VMEM)
    scratch = [
        pltpu.VMEM((NT, S, 128), BF),
        pltpu.VMEM((NT, D, 128), BF),
        pltpu.VMEM((NT, D, 128), BF),
        pltpu.VMEM((NT, D, 128), BF),
        pltpu.VMEM((NT, D, 128), BF),
        pltpu.VMEM((NB, S, CB), BF),
        pltpu.VMEM((NB, S, CB), BF),
        pltpu.VMEM((NB, S, CB), BF),
        pltpu.VMEM((NB, CB, S), BF),
        pltpu.VMEM((N2, 128, 128), BF),
        pltpu.VMEM((N2, 128, 128), BF),
        pltpu.VMEM((NT, NT, 128, 128), BF),
        pltpu.VMEM((NT, S // 128, 128, 128), BF),
        pltpu.VMEM((NT, NT, 128, 128), BF),
        pltpu.VMEM((NT, 128, 128), BF),
        pltpu.VMEM((NT, D, 128), BF),
        pltpu.VMEM((NT, 128, 128), BF),
        pltpu.VMEM((S // 128, NT, 128, 128), BF),
        pltpu.VMEM((S // 128, NT, 128, 128), BF),
        pltpu.VMEM((S, D), BF),
        pltpu.VMEM((NB, S, CB), BF),
        pltpu.VMEM((HALO + S + 8, CB), F32),
        pltpu.VMEM((S + 8, CB), F32),
        pltpu.VMEM((S + 8, CB), F32),
        pltpu.VMEM((3, N1 // 8, 512, CB), F32),
        pltpu.VMEM((2, 2, N2, 128, CB), BF),
        pltpu.VMEM((N2 + 1, 128, CB), BF),
        pltpu.VMEM((3, N2, 128, CB), F32),
        pltpu.VMEM((N1 // 8 + 1, 512, CB), F32),
        pltpu.VMEM((NT, S // 256, 128, 128), F32),
        pltpu.SemaphoreType.DMA((64,)),
    ]
    out = pl.pallas_call(
        _kernel,
        out_shape=jax.ShapeDtypeStruct((S, 2 * D), BF),
        in_specs=[pl.BlockSpec(memory_space=pltpu.SMEM), hbm, hbm, hbm, hbm, hbm, hbm, vmem, hbm, vmem, hbm, hbm],
        out_specs=hbm,
        scratch_shapes=scratch,
        compiler_params=pltpu.CompilerParams(vmem_limit_bytes=100 * 1024 * 1024),
    )(np.zeros((NZ,), np.int32), A_x.reshape(S, D), A_wqkv, A_wo, B_q.reshape(S, D), B_k.reshape(S, D), B_v.reshape(S, D),
      B_shift_k.T, B_ssm_k, B_ssm_D.reshape(1, D), _FWD, _INV)
    return out.reshape(1, S, 2 * D)
```

```python
import numpy as np
import jax
import jax.numpy as jnp
import jax.experimental.pallas as pl
import jax.experimental.pallas.tpu as pltpu

S = 2048
D = 1024
DH = 32
N1, N2 = 64, 32
CB = 128
NB = D // CB
NT = D // 128
HALO = 8
NZ = 32
F0_AT = 112
V_LEAD, V_TRAIL, M_TRAIL = {0: (F0_AT + 2) * 128}, {NB + 1: 2500}, 300
REGION_BIAS = [20000] + [0] * NB + [2500]
REGIONS = range(NB + 2)
DBG = ''
FENCE, FROW = 1, 0
BF = jnp.bfloat16
F32 = jnp.float32


def _dft_tables():
    idx = np.arange(N1)
    col = 16 * (idx // 8) + (idx % 8)
    e = np.exp(-2j * np.pi * np.outer(idx, idx) / N1)
    t = np.exp(-2j * np.pi * np.outer(np.arange(N2) + 0.25, idx) / S)
    tab = np.zeros((2 * 128 + 2 * N2, 128), np.float64)
    p, q, tr, ti = tab[:128], tab[128:256], tab[256:256 + N2], tab[256 + N2:]
    p[:N1, col], p[:N1, col + 8], p[N1:, col], p[N1:, col + 8] = e.real, -e.imag, e.imag, e.real
    q[:N1, col], q[:N1, col + 8], q[N1:, col], q[N1:, col + 8] = -e.imag, -e.real, e.real, -e.imag
    tr[:, col], tr[:, col + 8], ti[:, col], ti[:, col + 8] = t.real, t.real, t.imag, t.imag
    return tab.astype(np.float32)


_TABLES = _dft_tables()


def _add(a, b):
    (sa, xa), (sb, xb) = a, b
    if sa == sb:
        return (sa, xa + xb)
    return (1, xa - xb) if sa > 0 else (1, xb - xa)


def _neg(a):
    return (-a[0], a[1])


def _sub(a, b):
    return _add(a, _neg(b))


def _scale(a, c):
    return (1, a[1] * np.float32(a[0] * c))


def _val(a):
    return a[1] if a[0] > 0 else -a[1]


def _cadd(a, b):
    return (_add(a[0], b[0]), _add(a[1], b[1]))


def _csub(a, b):
    return (_sub(a[0], b[0]), _sub(a[1], b[1]))


def _cmul_i(a, s):
    return (_neg(a[1]), a[0]) if s > 0 else (a[1], _neg(a[0]))


def _cmul_const(a, w):
    c, s = float(np.real(w)), float(np.imag(w))
    return (_add(_scale(a[0], c), _scale(a[1], -s)), _add(_scale(a[0], s), _scale(a[1], c)))


def _fft4(x, s):
    a0, a1 = _cadd(x[0], x[2]), _cadd(x[1], x[3])
    b0, b1 = _csub(x[0], x[2]), _cmul_i(_csub(x[1], x[3]), s)
    return [_cadd(a0, a1), _cadd(b0, b1), _csub(a0, a1), _csub(b0, b1)]


def _fft8(x, s):
    r = np.sqrt(0.5)
    a = [_cadd(x[n], x[n + 4]) for n in range(4)]
    b = [_csub(x[n], x[n + 4]) for n in range(4)]
    t = _cadd(b[1], _cmul_i(b[1], s))
    b[1] = (_scale(t[0], r), _scale(t[1], r))
    b[2] = _cmul_i(b[2], s)
    t = _csub(_cmul_i(b[3], s), b[3])
    b[3] = (_scale(t[0], r), _scale(t[1], r))
    ev, od = _fft4(a, s), _fft4(b, s)
    return [ev[0], od[0], ev[1], od[1], ev[2], od[2], ev[3], od[3]]


_C1, _S1, _R2 = np.cos(np.pi / 8), np.sin(np.pi / 8), np.sqrt(0.5)


def _tw(n, j, s):
    return np.exp(s * 2j * np.pi * n * (4 * j + 1) / 128)


def _fwd_stage1(n, u0, u1, u2, u3):
    u0, u1, u2, u3 = (1, u0), (1, u1), (1, u2), (1, u3)
    t = _scale(u2, _R2)
    p, m_ = _add(u0, t), _sub(u0, t)
    c1u1, s1u1, c1u3, s1u3 = _scale(u1, _C1), _scale(u1, _S1), _scale(u3, _C1), _scale(u3, _S1)
    a, b = _add(c1u1, s1u3), _add(s1u1, c1u3)
    d, e = _sub(c1u1, s1u3), _sub(s1u1, c1u3)
    sj = [(_add(p, a), _neg(_add(t, b))), (_sub(m_, e), _sub(t, d)),
          (_sub(p, a), _sub(b, t)), (_add(m_, e), _add(t, d))]
    out = [sj[j] if n == 0 else _cmul_const(sj[j], _tw(n, j, -1)) for j in range(4)]
    return [(_val(re), _val(im)) for re, im in out]


def _fwd_stage2(t):
    out = _fft8([((1, re), (1, im)) for re, im in t], -1)
    return [(_val(re), _val(im)) for re, im in out]


def _inv_stage1(j, b):
    out = _fft8([((1, re), (1, im)) for re, im in b], 1)
    out = [out[n] if n == 0 else _cmul_const(out[n], _tw(n, j, 1)) for n in range(8)]
    return [(_val(re), _val(im)) for re, im in out]


def _inv_stage2(s):
    (x0, y0), (x1, y1), (x2, y2), (x3, y3) = [((1, re), (1, im)) for re, im in s]
    p, a, b = _add(x0, x2), _sub(x0, x2), _sub(y2, y0)
    m_, e, d = _add(x1, x3), _sub(x3, x1), _sub(y3, y1)
    t = _add(_sub(_add(y1, y3), _add(y0, y2)), _sub(p, m_))
    return [_val(_add(p, m_)),
            _val(_add(_scale(_add(a, d), _C1), _scale(_add(b, e), _S1))),
            _val(_scale(t, _R2)),
            _val(_add(_scale(_sub(a, d), _S1), _scale(_sub(b, e), _C1)))]


def _phi(t):
    return jnp.where(t > 0, t + 1.0, jnp.exp(t)) + 1e-6


def _dot(a, b):
    return jnp.dot(a, b, preferred_element_type=F32)


def _dot_nt(a, b):
    return jax.lax.dot_general(a, b, (((1,), (1,)), ((), ())), preferred_element_type=F32)


def _ld(ref, lead, r0, n):
    lead = lead if isinstance(lead, tuple) else (lead,)
    return pltpu.bitcast(ref.bitcast(jnp.uint32)[(*lead, pl.ds(r0 // 2, n // 2), slice(None))], BF)


def _cat(parts, axis):
    return parts[0] if len(parts) == 1 else jnp.concatenate(parts, axis=axis)


def _spread(stream, extra):
    out = []
    extra = sorted(extra, key=lambda e: e[0])
    e = 0
    for pos, item in enumerate(stream):
        while e < len(extra) and extra[e][0] <= pos:
            out.append(extra[e][1])
            e += 1
        out.append(item)
    return out + [t for _, t in extra[e:]]


def _kernel(zero_ref, x_hbm, wqkv_hbm, wo_hbm, q_hbm, k_hbm, v_hbm, sk_ref, h_hbm, d_ref, tab_hbm,
            out_hbm,
            x_v, wq_v, wk_v, wv_v, wo_v, q_v, k_v, v_v, h_v, tab_v, fwd_v, inv_v,
            wkt_s, pkt_s, g_s, kv_s, m_s, zb_s, pq_s, r_s, oa_s, ob_s,
            kf_s, u_s, ht_s, tf_s, a_s, yf_s, b_s, ti_s, z_s, sems):
    n_sem = [0]
    n_wait = [0]

    def zero(i):
        return zero_ref[i % NZ]

    def group(pairs):
        sem = sems.at[n_sem[0]]
        n_sem[0] += 1
        return [pltpu.make_async_copy(src, dst, sem) for src, dst in pairs]

    def start(g):
        for c in (g if 'nodma' not in DBG else []):
            c.start()

    def wait(g):
        if 'scope' in DBG:
            n_wait[0] += 1
            with jax.named_scope(f"region_w{n_wait[0]}"):
                for c in g:
                    c.wait()
            return
        for c in (g if 'nodma' not in DBG else []):
            c.wait()

    def col(ref, j):
        return ref.at[:, pl.ds(j * 128, 128)]

    def split(src, dst, n):
        step = src.shape[0] // n
        return [(src.at[pl.ds(t * step, step), :], dst.at[pl.ds(t * step, step), :]) for t in range(n)]

    cp_x = [group([(x_hbm.at[pl.ds(r0, 256), pl.ds(j * 128, 128)], x_v.at[j, pl.ds(r0, 256), :])
                   for j in range(NT)]) for r0 in range(0, S, 256)]
    cp_wq = group([(col(wqkv_hbm, j), wq_v.at[j]) for j in range(NT)])
    cp_wk = [group(split(col(wqkv_hbm, NT + g), wk_v.at[g], 4)) for g in range(NT)]
    cp_wvo = group([(col(wqkv_hbm, 2 * NT + g), wv_v.at[g]) for g in range(NT)]
                   + [(col(wo_hbm, j), wo_v.at[j]) for j in range(NT)])
    parts = [8, 8] + [2] * (NB - 2)
    cp_q = [group(split(col(q_hbm, i), q_v.at[i], 2)) for i in range(NB)]
    cp_kv = [group(split(col(k_hbm, i), k_v.at[i], parts[i]) + split(col(v_hbm, i), v_v.at[i], parts[i]))
             for i in range(NB)]
    cp_h = [group(split(h_hbm.at[pl.ds(i * CB, CB), :], h_v.at[i], parts[i])) for i in range(NB)]
    cp_tab = group(split(tab_hbm, tab_v, 4))
    cp_ob = [group(split(ob_s.at[i], col(out_hbm, NT + i), 8 if i == NB - 1 else 2)) for i in range(NB)]
    oa_spans = []

    def cp_oa(t):
        r0, n = oa_spans[t]
        pairs = split(oa_s.at[pl.ds(r0, n), :], out_hbm.at[pl.ds(r0, n), pl.ds(0, D)], 8)
        return [pltpu.make_async_copy(src, dst, sems.at[n_sem[0] + t]) for src, dst in pairs]

    rows_done = [0, 0]

    def sync(waits=(), starts=()):
        def run():
            for g in starts:
                start(g)
            done, sent = rows_done
            if done > sent:
                oa_spans.append((sent, done - sent))
                start(cp_oa(len(oa_spans) - 1))
                rows_done[1] = done
            for g in waits:
                wait(g)
        return 0, run

    RP = 128

    def b_forward(i):
        def widen(p):
            def run():
                kf_s[pl.ds(HALO + p * RP, RP), :] = _ld(k_v, i, p * RP, RP).astype(F32)
            return 16, run

        def gate(p):
            def run():
                taps = sk_ref[:, pl.ds(i * CB, CB)].astype(F32)
                acc = kf_s[pl.ds(HALO + p * RP, RP), :] * taps[0:1, :]
                for j in range(1, 4):
                    acc = acc + kf_s[pl.ds(HALO + p * RP - j, RP), :] * taps[j:j + 1, :]
                u_s[pl.ds(p * RP, RP), :] = acc * _ld(v_v, i, p * RP, RP).astype(F32)
            return 150, run

        def transpose(p):
            def run():
                ht = h_v[i, :, pl.ds(p * RP, RP)].astype(F32).T
                if p == 0:
                    skip = d_ref[:, pl.ds(i * CB, CB)].astype(F32)
                    lag = jax.lax.broadcasted_iota(jnp.int32, (RP, CB), 0)
                    ht = ht + jnp.where(lag == 0, skip, 0.0)
                ht_s[pl.ds(p * RP, RP), :] = ht
            return 40, run

        def stage1(src, h, j, n):
            def run():
                out = _fwd_stage1(n, *[src[pl.ds(N1 * (n + 8 * m) + 8 * j, 8), :] for m in range(4)])
                for r in range(4):
                    tf_s[h, j, pl.ds(16 * (8 * r + n), 8), :] = out[r][0]
                    tf_s[h, j, pl.ds(16 * (8 * r + n) + 8, 8), :] = out[r][1]
            return (43 if n else 21), run

        def stage2(h, j, r):
            def run():
                out = _fwd_stage2([(tf_s[h, j, pl.ds(16 * (8 * r + n), 8), :],
                                    tf_s[h, j, pl.ds(16 * (8 * r + n) + 8, 8), :]) for n in range(8)])
                for l in range(8):
                    a_s[i % 2, h, r + 4 * l, pl.ds(16 * j, 16), :] = _cat(out[l], 0).astype(BF)
            return 64, run

        tasks = [transpose(p) for p in range(S // RP)] if 'notr' not in DBG else []
        prep = ([sync([cp_kv[0]])] if i == 0 else []) + [widen(0)]
        for p in range(S // RP):
            prep += ([widen(p + 1)] if p + 1 < S // RP else []) + [gate(p)]
        cols = [(ht_s, 1, j) for j in range(N1 // 8)] + [(u_s, 0, j) for j in range(N1 // 8)]
        for c, (src, h, j) in enumerate(cols):
            tasks += [stage1(src, h, j, n) for n in range(8)]
            if i > 0 and c < 8:
                tasks += prep[4 * c:4 * c + 4]
            if i == 0 and c == 7:
                tasks += prep
            if c > 0:
                tasks += [stage2(cols[c - 1][1], cols[c - 1][2], r) for r in range(4)]
        return tasks + [stage2(cols[-1][1], cols[-1][2], r) for r in range(4)]

    def b_inverse(i):
        def stage1(j, r):
            def run():
                out = _inv_stage1(r, [(b_s[i % 2, r + 4 * l, pl.ds(16 * j, 8), :],
                                       b_s[i % 2, r + 4 * l, pl.ds(16 * j + 8, 8), :]) for l in range(8)])
                for n in range(8):
                    ti_s[j, pl.ds(16 * (4 * n + r), 8), :] = out[n][0]
                    ti_s[j, pl.ds(16 * (4 * n + r) + 8, 8), :] = out[n][1]
            return 98, run

        def stage2(jp, n):
            def run():
                ys = [_inv_stage2([(ti_s[j, pl.ds(16 * (4 * n + r), 8), :],
                                    ti_s[j, pl.ds(16 * (4 * n + r) + 8, 8), :]) for r in range(4)])
                      for j in (2 * jp, 2 * jp + 1)]
                for m in range(4):
                    r0 = N1 * (n + 8 * m) + 16 * jp
                    y = _cat([ys[0][m], ys[1][m]], 0)
                    ob_s[i, pl.ds(r0, 16), :] = (_ld(q_v, i, r0, 16).astype(F32) * y).astype(BF)
            return 66, run

        tasks = []
        for jp in range(N1 // 16 + 1):
            if jp < N1 // 16:
                tasks += [stage1(j, r) for j in (2 * jp, 2 * jp + 1) for r in range(4)]
            if jp > 0:
                tasks += [stage2(jp - 1, n) for n in range(8)]
        return tasks

    def dft_matrix(k2):
        def run():
            f = (tab_v[pl.ds(0, 128), :] * tab_v[pl.ds(256 + k2, 1), :]
                 + tab_v[pl.ds(128, 128), :] * tab_v[pl.ds(256 + N2 + k2, 1), :])
            fwd_v[k2] = f.astype(BF)
            inv_v[k2] = (f.T * (1.0 / S)).astype(BF)
        return 0, run

    def b_middle(i):
        def forward(k2):
            def run():
                rhs = _cat([_ld(a_s, (i % 2, h, k2), 0, 128) for h in range(2)], 1)
                xf = _dot(_ld(fwd_v, k2 + zero(i), 0, 128), rhs)
                ur, ui, hr, hi = xf[:N1, :CB], xf[N1:, :CB], xf[:N1, CB:], xf[N1:, CB:]
                yf_s[k2] = _cat([ur * hr - ui * hi, ur * hi + ui * hr], 0).astype(BF)
            return 64, run

        def inverse(k2):
            def run():
                b_s[i % 2, k2] = _dot(_ld(inv_v, k2 + zero(i), 0, 128), _ld(yf_s, k2, 0, 128))
            return 32, run

        tasks = []
        for k4 in range(N2 // 4 + 1):
            if k4 < N2 // 4:
                tasks += [[forward(4 * k4), forward(4 * k4 + 1)], [forward(4 * k4 + 2), forward(4 * k4 + 3)]]
            if k4 > 0:
                tasks += [[inverse(4 * k4 - 4 + r) for r in range(4)]]
        return tasks

    def head_mask():
        r = jax.lax.broadcasted_iota(jnp.int32, (128, 128), 0) // DH
        c = jax.lax.broadcasted_iota(jnp.int32, (128, 128), 1) // DH
        return r == c

    mid_chain = set()

    n_piece = [0]

    def fence(value):
        for ref in (kf_s, u_s, ht_s):
            ref[pl.ds(pl.multiple_of(zero(0) + (ref.shape[0] - 8), 8), 8), :] = value
        for ref in (tf_s, b_s, ti_s):
            lead = (zero(0) + (ref.shape[0] - 1),) + (0,) * (len(ref.shape) - 3)
            ref[(*lead, pl.ds(0, 8), slice(None))] = value
        yf_s.bitcast(jnp.uint32)[zero(0) + N2, pl.ds(0, 8), :] = pltpu.bitcast(value, jnp.uint32)

    def chain(n_k, operands, dot, finish):
        acc = [None]

        def piece(kk):
            def run():
                d = dot(*operands(kk))
                acc[0] = d if kk == 0 else acc[0] + d
                n_piece[0] += 1
                if n_piece[0] % FENCE == 0:
                    fence(d[FROW:FROW + 8, :128])
                if kk == n_k - 1:
                    finish(acc[0])
            if kk > 0:
                mid_chain.add(run)
            return 128, run
        return [piece(kk) for kk in range(n_k)]

    def a_transpose_wk(g):
        def tile(j):
            def run():
                wkt_s[g, j] = _ld(wk_v, g, j * 128, 128).astype(F32).T.astype(BF)
            return 0, run
        return [tile(j) for j in range(NT)]

    def a_keys(g, c):
        def operands(kk):
            js = (2 * kk, 2 * kk + 1)
            return (_cat([_ld(wkt_s, (g + zero(c), j), 0, 128) for j in js], 1),
                    _cat([_ld(x_v, j + zero(g), c * 256, 256) for j in js], 1))

        def finish(acc):
            pk = _phi(acc)
            pkt_s[g, 2 * c] = pk[:, :128].astype(BF)
            pkt_s[g, 2 * c + 1] = pk[:, 128:].astype(BF)
            part = pk[:, :128] + pk[:, 128:]
            if c < S // 256 - 1:
                z_s[g, c] = part
            else:
                for b in range(c):
                    part = part + z_s[g, b]
                z = jnp.broadcast_to(jnp.sum(part, axis=1, keepdims=True), (128, 128))
                zb_s[g] = jnp.where(head_mask(), z, 0.0).astype(BF)
        return chain(D // 256, operands, _dot_nt, finish)

    def a_gram(g):
        def block(n):
            def operands(kk):
                return (_cat([_ld(pkt_s, (g, 2 * kk + t), 0, 128) for t in range(2)], 1),
                        _cat([_ld(x_v, 2 * n + t + zero(NT + g), kk * 256, 256) for t in range(2)], 1))

            def finish(acc):
                g_s[g, 2 * n] = acc[:, :128].astype(BF)
                g_s[g, 2 * n + 1] = acc[:, 128:].astype(BF)
            return chain(S // 256, operands, _dot, finish)
        return [t for n in range(D // 256) for t in block(n)]

    def a_kv(g):
        def run():
            kv = _dot(_cat([_ld(g_s, (g, j), 0, 128) for j in range(NT)], 1), _ld(wv_v, g, 0, D))
            kv_s[g] = jnp.where(head_mask(), kv, 0.0).astype(BF)
        return 256, run

    def a_mix(g, half):
        def run():
            js = range(4 * half, 4 * half + 4)
            m = _dot(_ld(kv_s, g, 0, 128), _cat([_ld(wo_v, j, g * 128, 128) for j in js], 1))
            for t, j in enumerate(js):
                m_s[j, pl.ds(g * 128, 128), :] = m[:, t * 128:(t + 1) * 128].astype(BF)
        return 128, run

    def a_query(c, n):
        def operands(kk):
            return (_cat([_ld(x_v, 2 * kk + t + zero(2 * NT + n), c * 128, 128) for t in range(2)], 1),
                    _cat([_ld(wq_v, 2 * n + t + zero(c), kk * 256, 256) for t in range(2)], 1))

        def finish(acc):
            pq = _phi(acc)
            pq_s[c, 2 * n] = pq[:, :128].astype(BF)
            pq_s[c, 2 * n + 1] = pq[:, 128:].astype(BF)
        return chain(D // 256, operands, _dot, finish)

    def a_normalise(c, n):
        def run():
            for g in (2 * n, 2 * n + 1):
                pq = _ld(pq_s, (c, g), 0, 128)
                den = _dot(pq, _ld(zb_s, g + zero(c), 0, 128)) + 1e-6
                inv = pl.reciprocal(den, approx=True)
                inv = inv * (2.0 - den * inv)
                r_s[c, g] = (pq.astype(F32) * inv).astype(BF)
        return 64, run

    def a_out(c, n):
        def operands(kk):
            return (_cat([_ld(r_s, (c, 2 * kk + t), 0, 128) for t in range(2)], 1),
                    _cat([_ld(m_s, 2 * n + t + zero(c), kk * 256, 256) for t in range(2)], 1))

        def finish(acc):
            oa_s[pl.ds(c * 128, 128), pl.ds(n * 256, 256)] = acc.astype(BF)
            if n == D // 256 - 1:
                rows_done[0] = (c + 1) * 128
        return chain(D // 256, operands, _dot, finish)

    def starter(*groups):
        def run():
            for g in groups:
                start(g)
        return 0, run

    a_stream, extra = [], []
    n_g = n_c = 0
    for grow in "gcgcggcggcggcccc":
        if grow == "g":
            a_stream += [t for c in range(n_c) for t in a_keys(n_g, c)]
            n_g += 1
        else:
            a_stream += [t for g in range(n_g) for t in a_keys(g, n_c)]
            n_c += 1
    extra += [(0, sync([cp_x[0]], [cp_wk[2], cp_wk[3]])),
              (2, sync([cp_wk[1]])),
              (8, sync([cp_x[1], cp_wk[2]], [cp_x[2], cp_wk[4], cp_wk[5]])),
              (16, sync([cp_wk[3]])),
              (32, sync([cp_x[2], cp_wk[4], cp_wk[5]], [cp_x[3], cp_wk[6], cp_wk[7], cp_tab])),
              (72, sync([cp_x[3], cp_wk[6], cp_wk[7], cp_tab], [cp_x[4], cp_h[0]])),
              (F0_AT, sync([cp_x[4], cp_h[0]], [cp_x[5], cp_kv[0]])),
              (160, sync([cp_x[5]], [cp_x[6]])),
              (192, sync([cp_x[6]], [cp_x[7], cp_h[1]])),
              (224, sync([cp_x[7]], [cp_kv[1]]))]
    extra += [(74 + k2, dft_matrix(k2)) for k2 in range(N2)]
    for g, (at, step) in {1: (2, 0.2), 2: (8, 0.75), 3: (16, 0.75), 4: (32, 1.5), 5: (46, 1.5), 6: (72, 2),
                          7: (90, 2)}.items():
        extra += [(at + int(step * j), t) for j, t in enumerate(a_transpose_wk(g))]
    for g in range(NT):
        at = len(a_stream)
        if g >= 5:
            for t, gg in enumerate(range(3 * (g - 5), min(3 * (g - 4), NT - 1))):
                extra += [(at + 8 * t + 8, a_kv(gg)), (at + 8 * t + 16, a_mix(gg, 0)), (at + 8 * t + 16, a_mix(gg, 1))]
        a_stream += a_gram(g)
    a_stream = _spread(a_stream, extra)
    n_c = S // 128
    for c in range(n_c + 1):
        stream, extra = [], []
        if c < n_c:
            stream += [t for n in range(D // 256) for t in a_query(c, n)]
            extra += [(4 * n + 8, a_normalise(c, n)) for n in range(D // 256 - 1)]
        if c == 0:
            extra += [(4, a_kv(NT - 1)), (8, a_mix(NT - 1, 0)), (8, a_mix(NT - 1, 1))]
        if c > 0:
            extra += [(4, a_normalise(c - 1, D // 256 - 1))]
            outs = [t for n in range(D // 256) for t in a_out(c - 1, n)]
            stream = stream + outs if c < n_c else _spread(outs, [(0, extra.pop()[1])])
        a_stream += _spread(stream, extra)

    v_regions, m_regions = [], []
    for r in range(NB + 2):
        v = b_inverse(r - 2) if r >= 2 else []
        v += b_forward(r) if r < NB else []
        if r == NB + 1:
            v.append(sync(starts=[cp_ob[NB - 1]]))
        v_regions.append(v)
        m_regions.append(b_middle(r - 1) if 1 <= r <= NB and 'nomid' not in DBG else [])
    v_cost = [sum(c for c, _ in v) for v in v_regions]
    m_cost = [sum(c for grp in m for c, _ in grp) for m in m_regions]
    total = sum(c for c, _ in a_stream) + sum(m_cost)
    weight = [c + w for c, w in zip(v_cost, REGION_BIAS)]

    sync(starts=[cp_wk[0], cp_x[0]])[1]()
    kf_s[pl.ds(0, HALO), :] = jnp.zeros((HALO, CB), F32)
    for ref in (pkt_s, r_s, g_s, kv_s, pq_s, a_s, z_s, fwd_v, inv_v):
        lead = (zero(0),) + (0,) * (len(ref.shape) - 3)
        ref[(*lead, pl.ds(0, 16), slice(None))] = jnp.zeros((16, CB), ref.dtype)
    sync([cp_wk[0]], [cp_wk[1], cp_x[1]])[1]()
    for _, run in a_transpose_wk(0):
        run()

    ai, clock = 0, 0
    for r in range(NB + 2):
        end = total * sum(weight[:r + 1]) / sum(weight)
        a_end, t = ai, clock + m_cost[r]
        while a_end < len(a_stream) and (t < end or a_stream[a_end][1] in mid_chain or r == NB + 1):
            t += a_stream[a_end][0]
            a_end += 1
        length = t - clock
        v, m = v_regions[r], m_regions[r]
        lead, trail = V_LEAD.get(r, 0), V_TRAIL.get(r, 0)
        v_time, acc_cost = [], 0
        for c, _ in v:
            v_time.append(lead + (length - lead - trail) * acc_cost / v_cost[r])
            acc_cost += c

        def region():
            now, pa, pm, pv = 0, ai, 0, 0
            while pa < a_end or pm < len(m):
                if pm < len(m) and ((length - M_TRAIL) * pm / len(m) <= now or pa == a_end):
                    todo = m[pm]
                    pm += 1
                else:
                    todo = [a_stream[pa]]
                    pa += 1
                for cost, run in todo:
                    run()
                    now += cost
                while pv < len(v) and v_time[pv] <= now:
                    v[pv][1]()
                    pv += 1
            for _, run in v[pv:]:
                run()

        waits = ([cp_h[r], cp_kv[r]] if 1 <= r < NB else []) + ([cp_q[r - 2]] if r >= 2 else [])
        starts = (([cp_h[r + 1], cp_kv[r + 1]] if 1 <= r < NB - 1 else []) + ([cp_q[r - 1]] if 1 <= r <= NB else [])
                  + ([cp_ob[r - 3]] if r >= 3 else []))
        pieces = sum(c > 0 for c, _ in a_stream[:ai])
        if r == 1:
            assert pieces > 224
            starts = starts + [cp_wvo]
        if r == 2:
            assert pieces <= 256 + 5 * 32
            waits, starts = waits + [cp_wvo], [cp_wq] + starts
        if r == 3:
            assert pieces <= 512 + 14
            waits = waits + [cp_wq]
        sync(waits, starts)[1]()
        if r in REGIONS:
            with jax.named_scope(f"region{r}"):
                pl.when(zero(r) == 0)(region)
        ai, clock = a_end, t

    if len(REGIONS) < NB + 2:
        for ref in (pkt_s, r_s, g_s, kv_s, pq_s, tf_s, a_s, yf_s, b_s, ti_s, z_s, m_s, zb_s, ob_s, wkt_s):
            lead = (zero(1),) + (0,) * (len(ref.shape) - 3)
            oa_s[pl.ds(0, 16), pl.ds(0, 128)] += ref[(*lead, pl.ds(0, 16), slice(None))].astype(BF)
        rows_done[0] = rows_done[1] + 128
    sync()[1]()
    with jax.named_scope("drain"):
        for g in [cp_oa(t) for t in range(len(oa_spans))] + cp_ob:
            wait(g)


@jax.jit
def pallas_concat_heads__linear_attn_block__ssm_conv_h3__prompt_kernel(
    A_x: jax.Array,
    A_wqkv: jax.Array,
    A_wo: jax.Array,
    B_q: jax.Array,
    B_k: jax.Array,
    B_v: jax.Array,
    B_shift_k: jax.Array,
    B_ssm_k: jax.Array,
    B_ssm_D: jax.Array,
):
    hbm = pl.BlockSpec(memory_space=pl.ANY)
    vmem = pl.BlockSpec(memory_space=pltpu.VMEM)
    scratch = [
        pltpu.VMEM((NT, S, 128), BF),
        pltpu.VMEM((NT, D, 128), BF),
        pltpu.VMEM((NT, D, 128), BF),
        pltpu.VMEM((NT, D, 128), BF),
        pltpu.VMEM((NT, D, 128), BF),
        pltpu.VMEM((NB, S, CB), BF),
        pltpu.VMEM((NB, S, CB), BF),
        pltpu.VMEM((NB, S, CB), BF),
        pltpu.VMEM((NB, CB, S), BF),
        pltpu.VMEM(_TABLES.shape, F32),
        pltpu.VMEM((N2, 128, 128), BF),
        pltpu.VMEM((N2, 128, 128), BF),
        pltpu.VMEM((NT, NT, 128, 128), BF),
        pltpu.VMEM((NT, S // 128, 128, 128), BF),
        pltpu.VMEM((NT, NT, 128, 128), BF),
        pltpu.VMEM((NT, 128, 128), BF),
        pltpu.VMEM((NT, D, 128), BF),
        pltpu.VMEM((NT, 128, 128), BF),
        pltpu.VMEM((S // 128, NT, 128, 128), BF),
        pltpu.VMEM((S // 128, NT, 128, 128), BF),
        pltpu.VMEM((S, D), BF),
        pltpu.VMEM((NB, S, CB), BF),
        pltpu.VMEM((HALO + S + 8, CB), F32),
        pltpu.VMEM((S + 8, CB), F32),
        pltpu.VMEM((S + 8, CB), F32),
        pltpu.VMEM((3, N1 // 8, 512, CB), F32),
        pltpu.VMEM((2, 2, N2, 128, CB), BF),
        pltpu.VMEM((N2 + 1, 128, CB), BF),
        pltpu.VMEM((3, N2, 128, CB), F32),
        pltpu.VMEM((N1 // 8 + 1, 512, CB), F32),
        pltpu.VMEM((NT, S // 256, 128, 128), F32),
        pltpu.SemaphoreType.DMA((64,)),
    ]
    out = pl.pallas_call(
        _kernel,
        out_shape=jax.ShapeDtypeStruct((S, 2 * D), BF),
        in_specs=[pl.BlockSpec(memory_space=pltpu.SMEM), hbm, hbm, hbm, hbm, hbm, hbm, vmem, hbm, vmem, hbm],
        out_specs=hbm,
        scratch_shapes=scratch,
        compiler_params=pltpu.CompilerParams(vmem_limit_bytes=100 * 1024 * 1024),
    )(np.zeros((NZ,), np.int32), A_x.reshape(S, D), A_wqkv, A_wo, B_q.reshape(S, D), B_k.reshape(S, D), B_v.reshape(S, D),
      B_shift_k.T, B_ssm_k, B_ssm_D.reshape(1, D), _TABLES)
    return out.reshape(1, S, 2 * D)
```

```python
import numpy as np
import jax
import jax.numpy as jnp
import jax.experimental.pallas as pl
import jax.experimental.pallas.tpu as pltpu

S = 2048
D = 1024
DH = 32
N1, N2 = 64, 32
CB = 128
NB = D // CB
NT = D // 128
HALO = 8
_AREAS = (("k", HALO + S), ("u", S), ("h", S), ("tf", 4 * S), ("b", 2 * N2 * 128), ("ti", 2 * S),
          ("acc", 4 * 256), ("fence", 8))
AT = {name: sum(n for _, n in _AREAS[:i]) for i, (name, _) in enumerate(_AREAS)}
W_ROWS = sum(n for _, n in _AREAS)
NZ = 32
F0_AT = 60
V_LEAD, V_TRAIL, M_TRAIL = {0: (F0_AT + 2) * 128}, {NB + 1: 2500}, 300
REGION_BIAS = [10000] + [0] * NB + [2500]
REGIONS = range(NB + 2)
DBG = ''
PRIO, PKIND, XF, M_WEIGHT = 7, 'exp', 'fin', 0.0
BF = jnp.bfloat16
F32 = jnp.float32


def _dft_tables():
    idx = np.arange(N1)
    col = 16 * (idx // 8) + (idx % 8)
    e = np.exp(-2j * np.pi * np.outer(idx, idx) / N1)
    t = np.exp(-2j * np.pi * np.outer(np.arange(N2) + 0.25, idx) / S)
    tab = np.zeros((2 * 128 + 2 * N2, 128), np.float64)
    p, q, tr, ti = tab[:128], tab[128:256], tab[256:256 + N2], tab[256 + N2:]
    p[:N1, col], p[:N1, col + 8], p[N1:, col], p[N1:, col + 8] = e.real, -e.imag, e.imag, e.real
    q[:N1, col], q[:N1, col + 8], q[N1:, col], q[N1:, col + 8] = -e.imag, -e.real, e.real, -e.imag
    tr[:, col], tr[:, col + 8], ti[:, col], ti[:, col + 8] = t.real, t.real, t.imag, t.imag
    return tab.astype(np.float32)


_TABLES = _dft_tables()


def _add(a, b):
    (sa, xa), (sb, xb) = a, b
    if sa == sb:
        return (sa, xa + xb)
    return (1, xa - xb) if sa > 0 else (1, xb - xa)


def _neg(a):
    return (-a[0], a[1])


def _sub(a, b):
    return _add(a, _neg(b))


def _scale(a, c):
    return (1, a[1] * np.float32(a[0] * c))


def _val(a):
    return a[1] if a[0] > 0 else -a[1]


def _cadd(a, b):
    return (_add(a[0], b[0]), _add(a[1], b[1]))


def _csub(a, b):
    return (_sub(a[0], b[0]), _sub(a[1], b[1]))


def _cmul_i(a, s):
    return (_neg(a[1]), a[0]) if s > 0 else (a[1], _neg(a[0]))


def _cmul_const(a, w):
    c, s = float(np.real(w)), float(np.imag(w))
    return (_add(_scale(a[0], c), _scale(a[1], -s)), _add(_scale(a[0], s), _scale(a[1], c)))


def _fft4(x, s):
    a0, a1 = _cadd(x[0], x[2]), _cadd(x[1], x[3])
    b0, b1 = _csub(x[0], x[2]), _cmul_i(_csub(x[1], x[3]), s)
    return [_cadd(a0, a1), _cadd(b0, b1), _csub(a0, a1), _csub(b0, b1)]


def _fft8(x, s):
    r = np.sqrt(0.5)
    a = [_cadd(x[n], x[n + 4]) for n in range(4)]
    b = [_csub(x[n], x[n + 4]) for n in range(4)]
    t = _cadd(b[1], _cmul_i(b[1], s))
    b[1] = (_scale(t[0], r), _scale(t[1], r))
    b[2] = _cmul_i(b[2], s)
    t = _csub(_cmul_i(b[3], s), b[3])
    b[3] = (_scale(t[0], r), _scale(t[1], r))
    ev, od = _fft4(a, s), _fft4(b, s)
    return [ev[0], od[0], ev[1], od[1], ev[2], od[2], ev[3], od[3]]


_C1, _S1, _R2 = np.cos(np.pi / 8), np.sin(np.pi / 8), np.sqrt(0.5)


def _tw(n, j, s):
    return np.exp(s * 2j * np.pi * n * (4 * j + 1) / 128)


def _fwd_stage1(n, u0, u1, u2, u3):
    u0, u1, u2, u3 = (1, u0), (1, u1), (1, u2), (1, u3)
    t = _scale(u2, _R2)
    p, m_ = _add(u0, t), _sub(u0, t)
    c1u1, s1u1, c1u3, s1u3 = _scale(u1, _C1), _scale(u1, _S1), _scale(u3, _C1), _scale(u3, _S1)
    a, b = _add(c1u1, s1u3), _add(s1u1, c1u3)
    d, e = _sub(c1u1, s1u3), _sub(s1u1, c1u3)
    sj = [(_add(p, a), _neg(_add(t, b))), (_sub(m_, e), _sub(t, d)),
          (_sub(p, a), _sub(b, t)), (_add(m_, e), _add(t, d))]
    out = [sj[j] if n == 0 else _cmul_const(sj[j], _tw(n, j, -1)) for j in range(4)]
    return [(_val(re), _val(im)) for re, im in out]


def _fwd_stage2(t):
    out = _fft8([((1, re), (1, im)) for re, im in t], -1)
    return [(_val(re), _val(im)) for re, im in out]


def _inv_stage1(j, b):
    out = _fft8([((1, re), (1, im)) for re, im in b], 1)
    out = [out[n] if n == 0 else _cmul_const(out[n], _tw(n, j, 1)) for n in range(8)]
    return [(_val(re), _val(im)) for re, im in out]


def _inv_stage2(s):
    (x0, y0), (x1, y1), (x2, y2), (x3, y3) = [((1, re), (1, im)) for re, im in s]
    p, a, b = _add(x0, x2), _sub(x0, x2), _sub(y2, y0)
    m_, e, d = _add(x1, x3), _sub(x3, x1), _sub(y3, y1)
    t = _add(_sub(_add(y1, y3), _add(y0, y2)), _sub(p, m_))
    return [_val(_add(p, m_)),
            _val(_add(_scale(_add(a, d), _C1), _scale(_add(b, e), _S1))),
            _val(_scale(t, _R2)),
            _val(_add(_scale(_sub(a, d), _S1), _scale(_sub(b, e), _C1)))]


def _phi(t):
    return jnp.where(t > 0, t + 1.0, jnp.exp(t)) + 1e-6


def _dot(a, b):
    return jnp.dot(a, b, preferred_element_type=F32)


def _dot_nt(a, b):
    return jax.lax.dot_general(a, b, (((1,), (1,)), ((), ())), preferred_element_type=F32)


def _ld(ref, lead, r0, n):
    lead = lead if isinstance(lead, tuple) else (lead,)
    return pltpu.bitcast(ref.bitcast(jnp.uint32)[(*lead, pl.ds(r0 // 2, n // 2), slice(None))], BF)


def _cat(parts, axis):
    return parts[0] if len(parts) == 1 else jnp.concatenate(parts, axis=axis)


def _spread(stream, extra):
    out = []
    extra = sorted(extra, key=lambda e: e[0])
    e = 0
    for pos, item in enumerate(stream):
        while e < len(extra) and extra[e][0] <= pos:
            out.append(extra[e][1])
            e += 1
        out.append(item)
    return out + [t for _, t in extra[e:]]


def _merge(a, b):
    keyed = [((t + 0.5) / len(x), s, item) for s, x in enumerate((a, b)) for t, item in enumerate(x)]
    return [item for _, _, item in sorted(keyed, key=lambda e: e[:2])]


def _kernel(zero_hbm, x_hbm, wqkv_hbm, wo_hbm, q_hbm, k_hbm, v_hbm, sk_hbm, h_hbm, d_hbm, tab_hbm,
            out_hbm,
            x_v, wq_v, wk_v, wv_v, wo_v, q_v, k_v, v_v, h_v, tab_v, fwd_v, inv_v,
            wkt_s, pkt_s, g_s, kv_s, m_s, zb_s, pq_s, r_s, oa_s, ob_s,
            a_s, yf_s, z_s, w_s, zero_ref, sk_ref, d_ref, sems):
    n_sem = [0]
    n_wait = [0]

    def zero(i):
        return zero_ref[i % NZ]

    def group(pairs):
        sem = sems.at[n_sem[0]]
        n_sem[0] += 1
        return [pltpu.make_async_copy(src, dst, sem) for src, dst in pairs]

    def start(g):
        for c in (g if 'nodma' not in DBG else []):
            c.start()

    def wait(g):
        if 'scope' in DBG:
            n_wait[0] += 1
            with jax.named_scope(f"region_w{n_wait[0]}"):
                for c in g:
                    c.wait()
            return
        for c in (g if 'nodma' not in DBG else []):
            c.wait()

    def col(ref, j):
        return ref.at[:, pl.ds(j * 128, 128)]

    def split(src, dst, n):
        step = src.shape[0] // n
        return [(src.at[pl.ds(t * step, step), :], dst.at[pl.ds(t * step, step), :]) for t in range(n)]

    cp_x = [group([(x_hbm.at[pl.ds(r0, 256), pl.ds(j * 128, 128)], x_v.at[j, pl.ds(r0, 256), :])
                   for j in range(NT)]) for r0 in range(0, S, 256)]
    cp_wq = group([(col(wqkv_hbm, j), wq_v.at[j]) for j in range(NT)])
    cp_wk = [group(split(col(wqkv_hbm, NT + g), wk_v.at[g], 4)) for g in range(NT)]
    cp_wvo = group([(col(wqkv_hbm, 2 * NT + g), wv_v.at[g]) for g in range(NT)]
                   + [(col(wo_hbm, j), wo_v.at[j]) for j in range(NT)])
    parts = [8, 8] + [2] * (NB - 2)
    cp_q = [group(split(col(q_hbm, i), q_v.at[i], 2)) for i in range(NB)]
    cp_kv = [group(split(col(k_hbm, i), k_v.at[i], parts[i]) + split(col(v_hbm, i), v_v.at[i], parts[i]))
             for i in range(NB)]
    cp_h = [group(split(h_hbm.at[pl.ds(i * CB, CB), :], h_v.at[i], parts[i])) for i in range(NB)]
    cp_tab = group([(tab_hbm, tab_v), (sk_hbm, sk_ref), (d_hbm, d_ref)])
    cp_zero = group([(zero_hbm, zero_ref)])
    cp_ob = [group(split(ob_s.at[i], col(out_hbm, NT + i), 8 if i == NB - 1 else 2)) for i in range(NB)]
    oa_spans = []

    def cp_oa(t):
        r0, n = oa_spans[t]
        pairs = split(oa_s.at[pl.ds(r0, n), :], out_hbm.at[pl.ds(r0, n), pl.ds(0, D)], 8)
        return [pltpu.make_async_copy(src, dst, sems.at[n_sem[0] + t]) for src, dst in pairs]

    rows_done = [0, 0]

    def sync(waits=(), starts=()):
        def run():
            for g in starts:
                start(g)
            done, sent = rows_done
            if done > sent:
                oa_spans.append((sent, done - sent))
                start(cp_oa(len(oa_spans) - 1))
                rows_done[1] = done
            for g in waits:
                wait(g)
        return 0, run

    RP = 64

    def area(name, r0, n=8):
        return pl.ds(AT[name] + r0, n), slice(None)

    def b_prepare(i):
        def widen(p):
            def run():
                w_s[area("k", HALO + p * RP, RP)] = _ld(k_v, i, p * RP, RP).astype(F32)
            return 30, run

        def gate(p):
            def run():
                taps = sk_ref[:, pl.ds(i * CB, CB)].astype(F32)
                acc = w_s[area("k", HALO + p * RP, RP)] * taps[0:1, :]
                for j in range(1, 4):
                    acc = acc + w_s[area("k", HALO + p * RP - j, RP)] * taps[j:j + 1, :]
                w_s[area("u", p * RP, RP)] = acc * _ld(v_v, i, p * RP, RP).astype(F32)
            return 80, run

        def transpose(p):
            def run():
                ht = h_v[i, :, pl.ds(p * 128, 128)].astype(F32).T
                if p == 0:
                    skip = d_ref[:, pl.ds(i * CB, CB)].astype(F32)
                    lag = jax.lax.broadcasted_iota(jnp.int32, (128, CB), 0)
                    ht = ht + jnp.where(lag == 0, skip, 0.0)
                w_s[area("h", p * 128, 128)] = ht
            return 70, run

        prep = ([sync([cp_kv[0]])] if i == 0 else []) + [widen(0)]
        for p in range(S // RP):
            prep += ([widen(p + 1)] if p + 1 < S // RP else []) + [gate(p)]
        return [transpose(p) for p in range(S // 128)], prep

    def b_forward(i, prep):
        def stage1(h, j, n):
            def run():
                out = _fwd_stage1(n, *[w_s[area("uh"[h], N1 * (n + 8 * m) + 8 * j)] for m in range(4)])
                for r in range(4):
                    for part in range(2):
                        w_s[area("tf", 512 * (8 * h + j) + 16 * (8 * r + n) + 8 * part)] = out[r][part]
            return (46 if n else 32), run

        def stage2(h, j, r):
            def run():
                out = _fwd_stage2([[w_s[area("tf", 512 * (8 * h + j) + 16 * (8 * r + n) + 8 * part)]
                                    for part in range(2)] for n in range(8)])
                for l in range(8):
                    a_s[i % 2, h, r + 4 * l, pl.ds(16 * j, 16), :] = _cat(out[l], 0).astype(BF)
            return 64, run

        tasks = []
        cols = [(h, j) for h in (1, 0) for j in range(N1 // 8)]
        for c, (h, j) in enumerate(cols):
            now = [stage1(h, j, n) for n in range(8)]
            now += [stage2(*cols[c - 1], r) for r in range(4)] if c > 0 else []
            lo = 4 if i == 0 else 0
            if lo <= c < 8:
                share = prep[len(prep) * (c - lo) // (8 - lo):len(prep) * (c + 1 - lo) // (8 - lo)]
                now = _merge(now, share)
            tasks += now
        return tasks + [stage2(*cols[-1], r) for r in range(4)]

    def b_inverse(i):
        def stage1(j, r):
            def run():
                out = _inv_stage1(r, [[w_s[area("b", 128 * (N2 * (i % 2) + r + 4 * l) + 16 * j + 8 * part)]
                                       for part in range(2)] for l in range(8)])
                for n in range(8):
                    for part in range(2):
                        w_s[area("ti", 512 * j + 16 * (4 * n + r) + 8 * part)] = out[n][part]
            return 100, run

        def stage2(jp, n):
            def run():
                ys = [_inv_stage2([[w_s[area("ti", 512 * j + 16 * (4 * n + r) + 8 * part)] for part in range(2)]
                                   for r in range(4)]) for j in (2 * jp, 2 * jp + 1)]
                for m in range(4):
                    r0 = N1 * (n + 8 * m) + 16 * jp
                    y = _cat([ys[0][m], ys[1][m]], 0)
                    ob_s[i, pl.ds(r0, 16), :] = (_ld(q_v, i, r0, 16).astype(F32) * y).astype(BF)
            return 66, run

        tasks = []
        for jp in range(N1 // 16 + 1):
            first = [stage1(j, r) for j in (2 * jp, 2 * jp + 1) for r in range(4)] if jp < N1 // 16 else []
            tasks += _merge(first, [stage2(jp - 1, n) for n in range(8)] if jp > 0 else [])
        return tasks

    def dft_matrix(k2):
        def run():
            f = (tab_v[pl.ds(0, 128), :] * tab_v[pl.ds(256 + k2, 1), :]
                 + tab_v[pl.ds(128, 128), :] * tab_v[pl.ds(256 + N2 + k2, 1), :])
            fwd_v[k2] = f.astype(BF)
            inv_v[k2] = (f.T * (1.0 / S)).astype(BF)
        return 0, run

    def b_middle(i):
        def forward(k2):
            def run():
                rhs = _cat([_ld(a_s, (i % 2, h, k2), 0, 128) for h in range(2)], 1)
                xf = _dot(_ld(fwd_v, k2 + zero(i), 0, 128), rhs)
                ur, ui, hr, hi = xf[:N1, :CB], xf[N1:, :CB], xf[:N1, CB:], xf[N1:, CB:]
                if 'f' in XF and k2 % 2 == 0:
                    urgent(xf[:8, :128])
                yf_s[k2] = _cat([ur * hr - ui * hi, ur * hi + ui * hr], 0).astype(BF)
            return 64, run

        def inverse(k2):
            def run():
                b = _dot(_ld(inv_v, k2 + zero(i), 0, 128), _ld(yf_s, k2, 0, 128))
                if 'i' in XF and k2 % 4 == 0:
                    urgent(b[:8, :])
                w_s[area("b", 128 * (N2 * (i % 2) + k2), 128)] = b
            return 32, run

        tasks = []
        for k4 in range(N2 // 4 + 1):
            if k4 < N2 // 4:
                tasks += [[forward(4 * k4), forward(4 * k4 + 1)], [forward(4 * k4 + 2), forward(4 * k4 + 3)]]
            if k4 > 0:
                tasks += [[inverse(4 * k4 - 4 + r) for r in range(4)]]
        return tasks

    def head_mask():
        r = jax.lax.broadcasted_iota(jnp.int32, (128, 128), 0) // DH
        c = jax.lax.broadcasted_iota(jnp.int32, (128, 128), 1) // DH
        return r == c

    mid_chain = set()

    lead_chain = [None]

    def urgent(value):
        if PRIO:
            c = value if lead_chain[0] is None else lead_chain[0] + value
            for _ in range(PRIO):
                c = pltpu.roll(c, 1, 1) if PKIND == 'roll' else jnp.exp(c)
            lead_chain[0] = c

    def fence(value):
        w_s[pl.ds(pl.multiple_of(zero(0) + AT["fence"], 8), 8), :] = value
        yf_s.bitcast(jnp.uint32)[zero(0) + N2, pl.ds(0, 8), :] = pltpu.bitcast(value, jnp.uint32)

    def chain(n_k, operands, dot, finish):
        acc = [None]

        def piece(kk):
            def run():
                d = dot(*operands(kk))
                acc[0] = d if kk == 0 else acc[0] + d
                fence(d[:8, :128])
                urgent(d[:8, :128])
                if kk == n_k - 1:
                    finish(acc[0])
            if kk > 0:
                mid_chain.add(run)
            return 128, run
        return [piece(kk) for kk in range(n_k)]

    followers = {}

    def chain_then(n_k, operands, dot, part):
        slot = len(followers) % 4

        def park(acc):
            w_s[area("acc", 256 * slot, 128)] = acc[:, :128]
            w_s[area("acc", 256 * slot + 128, 128)] = acc[:, 128:]

        def quarter(t):
            def run():
                part(pl.ds(32 * t, 32), 32 * t, *[w_s[area("acc", 256 * slot + 128 * half + 32 * t, 32)] for half in range(2)])
            return 0, run
        pieces = chain(n_k, operands, dot, park)
        followers[pieces[-1][1]] = [quarter(t) for t in range(4)]
        return pieces

    def a_transpose_wk(g):
        def tile(j):
            def run():
                wkt_s[g, j] = _ld(wk_v, g, j * 128, 128).astype(F32).T.astype(BF)
            return 0, run
        return [tile(j) for j in range(NT)]

    def a_keys(g, c):
        def operands(kk):
            js = (2 * kk, 2 * kk + 1)
            return (_cat([_ld(wkt_s, (g + zero(c), j), 0, 128) for j in js], 1),
                    _cat([_ld(x_v, j + zero(g), c * 256, 256) for j in js], 1))

        def part(rows, r0, lo, hi):
            lo, hi = _phi(lo), _phi(hi)
            pkt_s[g, 2 * c, rows, :] = lo.astype(BF)
            pkt_s[g, 2 * c + 1, rows, :] = hi.astype(BF)
            total = lo + hi
            if c < S // 256 - 1:
                z_s[g, c, rows, :] = total
            else:
                for b in range(c):
                    total = total + z_s[g, b, rows, :]
                z = jnp.broadcast_to(jnp.sum(total, axis=1, keepdims=True), (32, 128))
                head = jax.lax.broadcasted_iota(jnp.int32, (32, 128), 1) // DH
                zb_s[g, rows, :] = jnp.where(head == r0 // DH, z, 0.0).astype(BF)
        return chain_then(D // 256, operands, _dot_nt, part)

    def a_gram(g):
        def block(n):
            def operands(kk):
                return (_cat([_ld(pkt_s, (g, 2 * kk + t), 0, 128) for t in range(2)], 1),
                        _cat([_ld(x_v, 2 * n + t + zero(NT + g), kk * 256, 256) for t in range(2)], 1))

            def finish(acc):
                g_s[g, 2 * n] = acc[:, :128].astype(BF)
                g_s[g, 2 * n + 1] = acc[:, 128:].astype(BF)
            return chain(S // 256, operands, _dot, finish)
        return [t for n in range(D // 256) for t in block(n)]

    def a_kv(g):
        def operands(kk):
            return (_cat([_ld(g_s, (g, j), 0, 128) for j in range(4 * kk, 4 * kk + 4)], 1),
                    _ld(wv_v, g, kk * 512, 512))

        def finish(kv):
            kv_s[g] = jnp.where(head_mask(), kv, 0.0).astype(BF)
        return chain(2, operands, _dot, finish)

    def a_mix(g, half):
        def run():
            js = range(4 * half, 4 * half + 4)
            m = _dot(_ld(kv_s, g, 0, 128), _cat([_ld(wo_v, j, g * 128, 128) for j in js], 1))
            for t, j in enumerate(js):
                m_s[j, pl.ds(g * 128, 128), :] = m[:, t * 128:(t + 1) * 128].astype(BF)
        return 128, run

    def a_query(c, n):
        def operands(kk):
            return (_cat([_ld(x_v, 2 * kk + t + zero(2 * NT + n), c * 128, 128) for t in range(2)], 1),
                    _cat([_ld(wq_v, 2 * n + t + zero(c), kk * 256, 256) for t in range(2)], 1))

        def part(rows, r0, lo, hi):
            pq_s[c, 2 * n, rows, :] = _phi(lo).astype(BF)
            pq_s[c, 2 * n + 1, rows, :] = _phi(hi).astype(BF)
        return chain_then(D // 256, operands, _dot, part)

    def a_normalise(c, half):
        def run():
            for g in range(4 * half, 4 * half + 4):
                pq = _ld(pq_s, (c, g), 0, 128)
                den = _dot(pq, _ld(zb_s, g + zero(c), 0, 128)) + 1e-6
                if 'n' in XF and g % 4 == 0:
                    urgent(den[:8, :])
                inv = pl.reciprocal(den, approx=True)
                inv = inv * (2.0 - den * inv)
                r_s[c, g] = (pq.astype(F32) * inv).astype(BF)
        return 128, run

    def a_out(c, n):
        def operands(kk):
            return (_cat([_ld(r_s, (c, 2 * kk + t), 0, 128) for t in range(2)], 1),
                    _cat([_ld(m_s, 2 * n + t + zero(c), kk * 256, 256) for t in range(2)], 1))

        def finish(acc):
            oa_s[pl.ds(c * 128, 128), pl.ds(n * 256, 256)] = acc.astype(BF)
            if n == D // 256 - 1:
                rows_done[0] = (c + 1) * 128
        return chain(D // 256, operands, _dot, finish)

    def starter(*groups):
        def run():
            for g in groups:
                start(g)
        return 0, run

    a_stream, extra = [], []
    n_g = n_c = 0
    for grow in "gcgcggcggcggcccc":
        if grow == "g":
            a_stream += [t for c in range(n_c) for t in a_keys(n_g, c)]
            n_g += 1
        else:
            a_stream += [t for g in range(n_g) for t in a_keys(g, n_c)]
            n_c += 1
    extra += [(0, sync([cp_x[0]], [cp_wk[2], cp_wk[3]])),
              (2, sync([cp_wk[1]])),
              (8, sync([cp_x[1], cp_wk[2]], [cp_x[2], cp_wk[4], cp_wk[5]])),
              (16, sync([cp_wk[3]])),
              (32, sync([cp_x[2], cp_wk[4], cp_wk[5]], [cp_x[3], cp_wk[6], cp_wk[7], cp_tab, cp_h[0]])),
              (F0_AT, sync([cp_x[3], cp_wk[6], cp_wk[7], cp_tab, cp_h[0]], [cp_x[4], cp_x[5], cp_kv[0]])),
              (128, sync([cp_x[4], cp_x[5]], [cp_x[6], cp_x[7], cp_h[1], cp_kv[1]]))]
    extra += [(F0_AT + 2 + 2 * k2, dft_matrix(k2)) for k2 in range(N2)]
    for g, (at, step) in {1: (2, 0.2), 2: (8, 0.75), 3: (16, 0.75), 4: (32, 1.5), 5: (46, 1.5), 6: (62, 3),
                          7: (86, 3)}.items():
        extra += [(at + int(step * j), t) for j, t in enumerate(a_transpose_wk(g))]
    for g in range(NT):
        at = len(a_stream)
        if g >= 5:
            for t, gg in enumerate(range(3 * (g - 5), min(3 * (g - 4), NT - 1))):
                extra += [(at + 8 * t + 8, p) for p in a_kv(gg)] + [(at + 8 * t + 16, a_mix(gg, 0)), (at + 8 * t + 16, a_mix(gg, 1))]
        a_stream += a_gram(g)
    a_stream = _spread(a_stream, extra)
    tail = []
    n_c = S // 128
    for c in range(n_c + 1):
        stream = [t for n in range(D // 256) for t in a_query(c, n)] if c < n_c else []
        stream += [t for n in range(D // 256) for t in a_out(c - 1, n)] if c > 0 else []
        at = len(a_stream)
        if c == 0:
            tail += [(at + 4, p) for p in a_kv(NT - 1)] + [(at + 8, a_mix(NT - 1, 0)), (at + 8, a_mix(NT - 1, 1))]
        if c < n_c:
            tail += [(at + 12, a_normalise(c, 0)), (at + 24, a_normalise(c, 1))]
        a_stream += stream
    a_stream = _spread(a_stream, tail)
    spread, pending = [], []
    for item in a_stream:
        spread.append(item)
        if item[0] > 0 and pending:
            spread.append(pending.pop(0))
        pending += followers.get(item[1], [])
    a_stream = spread + pending

    v_regions, m_regions = [], []
    for r in range(NB + 2):
        v = b_inverse(r - 2) if r >= 2 else []
        if r < NB:
            transposes, prep = b_prepare(r)
            v = _merge(v, transposes) + b_forward(r, prep)
        if r == NB + 1:
            v.append(sync(starts=[cp_ob[NB - 1]]))
        v_regions.append(v)
        m_regions.append(b_middle(r - 1) if 1 <= r <= NB and 'nomid' not in DBG else [])
    v_cost = [sum(c for c, _ in v) for v in v_regions]
    m_cost = [sum(c for grp in m for c, _ in grp) for m in m_regions]
    total = sum(c for c, _ in a_stream) + sum(m_cost)
    weight = [c + w for c, w in zip(v_cost, REGION_BIAS)]

    sync([cp_zero], [cp_zero, cp_wk[0], cp_x[0]])[1]()
    w_s[area("k", 0)] = jnp.zeros((HALO, CB), F32)
    for ref in (pkt_s, r_s, g_s, kv_s, pq_s, a_s, z_s, fwd_v, inv_v):
        lead = (zero(0),) + (0,) * (len(ref.shape) - 3)
        ref[(*lead, pl.ds(0, 16), slice(None))] = jnp.zeros((16, CB), ref.dtype)
    sync([cp_wk[0]], [cp_wk[1], cp_x[1]])[1]()
    for _, run in a_transpose_wk(0):
        run()

    ai, clock = 0, 0
    for r in range(NB + 2):
        end = total * sum(weight[:r + 1]) / sum(weight)
        a_end, t = ai, clock + m_cost[r]
        while a_end < len(a_stream) and (t < end or a_stream[a_end][0] == 0
                                         or a_stream[a_end][1] in mid_chain or r == NB + 1):
            t += a_stream[a_end][0]
            a_end += 1
        length = t - clock - (1 - M_WEIGHT) * m_cost[r]
        v, m = v_regions[r], m_regions[r]
        lead, trail = V_LEAD.get(r, 0), V_TRAIL.get(r, 0)
        v_time, acc_cost = [], 0
        for c, _ in v:
            v_time.append(lead + (length - lead - trail) * acc_cost / v_cost[r])
            acc_cost += c

        def region():
            now, pa, pm, pv = 0, ai, 0, 0
            while pa < a_end or pm < len(m):
                if pm < len(m) and ((length - M_TRAIL) * pm / len(m) <= now or pa == a_end):
                    todo = m[pm]
                    pm += 1
                else:
                    todo = [a_stream[pa]]
                    pa += 1
                for cost, run in todo:
                    run()
                    now += cost * (M_WEIGHT if len(todo) > 1 else 1)
                while pv < len(v) and v_time[pv] <= now:
                    v[pv][1]()
                    pv += 1
            for _, run in v[pv:]:
                run()
            if lead_chain[0] is not None:
                fence(lead_chain[0])
                lead_chain[0] = None

        waits = ([cp_h[r], cp_kv[r]] if 1 <= r < NB else []) + ([cp_q[r - 2]] if r >= 2 else [])
        starts = (([cp_h[r + 1], cp_kv[r + 1]] if 1 <= r < NB - 1 else []) + ([cp_q[r - 1]] if 1 <= r <= NB else [])
                  + ([cp_ob[r - 3]] if r >= 3 else []))
        pieces = sum(c > 0 for c, _ in a_stream[:ai])
        if r == 1:
            assert F0_AT + 2 * N2 + 2 < pieces <= 192
            waits, starts = waits + [cp_x[6], cp_x[7]], starts + [cp_wvo]
        if r == 2:
            assert pieces <= 256 + 5 * 32
            starts = starts + [cp_wq]
        if r == 3:
            assert pieces <= 256 + 5 * 32 + 8
            waits = waits + [cp_wvo, cp_wq]
        sync(waits, starts)[1]()
        if r in REGIONS:
            with jax.named_scope(f"region{r}"):
                pl.when(zero(r) == 0)(region)
        ai, clock = a_end, t

    if len(REGIONS) < NB + 2:
        for ref in (pkt_s, r_s, g_s, kv_s, pq_s, a_s, yf_s, z_s, m_s, zb_s, ob_s, wkt_s):
            lead = (zero(1),) + (0,) * (len(ref.shape) - 3)
            oa_s[pl.ds(0, 16), pl.ds(0, 128)] += ref[(*lead, pl.ds(0, 16), slice(None))].astype(BF)
        rows_done[0] = rows_done[1] + 128
    sync()[1]()
    with jax.named_scope("drain"):
        for g in [cp_oa(t) for t in range(len(oa_spans))] + cp_ob:
            wait(g)


@jax.jit
def pallas_concat_heads__linear_attn_block__ssm_conv_h3__prompt_kernel(
    A_x: jax.Array,
    A_wqkv: jax.Array,
    A_wo: jax.Array,
    B_q: jax.Array,
    B_k: jax.Array,
    B_v: jax.Array,
    B_shift_k: jax.Array,
    B_ssm_k: jax.Array,
    B_ssm_D: jax.Array,
):
    hbm = pl.BlockSpec(memory_space=pl.ANY)
    scratch = [
        pltpu.VMEM((NT, S, 128), BF),
        pltpu.VMEM((NT, D, 128), BF),
        pltpu.VMEM((NT, D, 128), BF),
        pltpu.VMEM((NT, D, 128), BF),
        pltpu.VMEM((NT, D, 128), BF),
        pltpu.VMEM((NB, S, CB), BF),
        pltpu.VMEM((NB, S, CB), BF),
        pltpu.VMEM((NB, S, CB), BF),
        pltpu.VMEM((NB, CB, S), BF),
        pltpu.VMEM(_TABLES.shape, F32),
        pltpu.VMEM((N2, 128, 128), BF),
        pltpu.VMEM((N2, 128, 128), BF),
        pltpu.VMEM((NT, NT, 128, 128), BF),
        pltpu.VMEM((NT, S // 128, 128, 128), BF),
        pltpu.VMEM((NT, NT, 128, 128), BF),
        pltpu.VMEM((NT, 128, 128), BF),
        pltpu.VMEM((NT, D, 128), BF),
        pltpu.VMEM((NT, 128, 128), BF),
        pltpu.VMEM((S // 128, NT, 128, 128), BF),
        pltpu.VMEM((S // 128, NT, 128, 128), BF),
        pltpu.VMEM((S, D), BF),
        pltpu.VMEM((NB, S, CB), BF),
        pltpu.VMEM((2, 2, N2, 128, CB), BF),
        pltpu.VMEM((N2 + 1, 128, CB), BF),
        pltpu.VMEM((NT, S // 256, 128, 128), F32),
        pltpu.VMEM((W_ROWS, 128), F32),
        pltpu.SMEM((NZ,), jnp.int32),
        pltpu.VMEM((4, D), BF),
        pltpu.VMEM((1, D), BF),
        pltpu.SemaphoreType.DMA((64,)),
    ]
    out = pl.pallas_call(
        _kernel,
        out_shape=jax.ShapeDtypeStruct((S, 2 * D), BF),
        in_specs=[hbm] * 11,
        out_specs=hbm,
        scratch_shapes=scratch,
        compiler_params=pltpu.CompilerParams(vmem_limit_bytes=100 * 1024 * 1024),
    )(np.zeros((NZ,), np.int32), A_x.reshape(S, D), A_wqkv, A_wo, B_q.reshape(S, D), B_k.reshape(S, D), B_v.reshape(S, D),
      B_shift_k.T, B_ssm_k, B_ssm_D.reshape(1, D), _TABLES)
    return out.reshape(1, S, 2 * D)
```

```python
import functools

import numpy as np
import jax
import jax.numpy as jnp
import jax.experimental.pallas as pl
import jax.experimental.pallas.tpu as pltpu

S = 2048
D = 1024
DH = 32
N1, N2 = 64, 32
CB = 128
NB = D // CB
NT = D // 128
HALO = 8
_AREAS = (("k", HALO + S), ("u", S), ("h", S), ("tf", 4 * S), ("b", 2 * N2 * 128), ("ti", 2 * S),
          ("acc", 4 * 256), ("fence", 8))
AT = {name: sum(n for _, n in _AREAS[:i]) for i, (name, _) in enumerate(_AREAS)}
W_ROWS = sum(n for _, n in _AREAS)
NZ = 32
F0_AT = 60
V_TRAIL, M_TRAIL = 2500, 300
ROOM = (128, 0, 0)
FIRST = 160 * 128
REGION_BIAS = [0] + [0] * NB + [2500]
DBG = ''
INREG = False
WIDE, BLOCKS = True, range(NB + 2)
PRIO, PKIND, XF, M_WEIGHT = 7, 'exp', 'fin', 0.0
BF = jnp.bfloat16
F32 = jnp.float32


def _dft_tables():
    idx = np.arange(N1)
    col = 16 * (idx // 8) + (idx % 8)
    e = np.exp(-2j * np.pi * np.outer(idx, idx) / N1)
    t = np.exp(-2j * np.pi * np.outer(np.arange(N2) + 0.25, idx) / S)
    tab = np.zeros((2 * 128 + 2 * N2, 128), np.float64)
    p, q, tr, ti = tab[:128], tab[128:256], tab[256:256 + N2], tab[256 + N2:]
    p[:N1, col], p[:N1, col + 8], p[N1:, col], p[N1:, col + 8] = e.real, -e.imag, e.imag, e.real
    q[:N1, col], q[:N1, col + 8], q[N1:, col], q[N1:, col + 8] = -e.imag, -e.real, e.real, -e.imag
    tr[:, col], tr[:, col + 8], ti[:, col], ti[:, col + 8] = t.real, t.real, t.imag, t.imag
    return tab.astype(np.float32)


_TABLES = _dft_tables()


def _add(a, b):
    (sa, xa), (sb, xb) = a, b
    if sa == sb:
        return (sa, xa + xb)
    return (1, xa - xb) if sa > 0 else (1, xb - xa)


def _neg(a):
    return (-a[0], a[1])


def _sub(a, b):
    return _add(a, _neg(b))


def _scale(a, c):
    return (1, a[1] * np.float32(a[0] * c))


def _val(a):
    return a[1] if a[0] > 0 else -a[1]


def _cadd(a, b):
    return (_add(a[0], b[0]), _add(a[1], b[1]))


def _csub(a, b):
    return (_sub(a[0], b[0]), _sub(a[1], b[1]))


def _cmul_i(a, s):
    return (_neg(a[1]), a[0]) if s > 0 else (a[1], _neg(a[0]))


def _cmul_const(a, w):
    c, s = float(np.real(w)), float(np.imag(w))
    return (_add(_scale(a[0], c), _scale(a[1], -s)), _add(_scale(a[0], s), _scale(a[1], c)))


def _fft4(x, s):
    a0, a1 = _cadd(x[0], x[2]), _cadd(x[1], x[3])
    b0, b1 = _csub(x[0], x[2]), _cmul_i(_csub(x[1], x[3]), s)
    return [_cadd(a0, a1), _cadd(b0, b1), _csub(a0, a1), _csub(b0, b1)]


def _fft8(x, s):
    r = np.sqrt(0.5)
    a = [_cadd(x[n], x[n + 4]) for n in range(4)]
    b = [_csub(x[n], x[n + 4]) for n in range(4)]
    t = _cadd(b[1], _cmul_i(b[1], s))
    b[1] = (_scale(t[0], r), _scale(t[1], r))
    b[2] = _cmul_i(b[2], s)
    t = _csub(_cmul_i(b[3], s), b[3])
    b[3] = (_scale(t[0], r), _scale(t[1], r))
    ev, od = _fft4(a, s), _fft4(b, s)
    return [ev[0], od[0], ev[1], od[1], ev[2], od[2], ev[3], od[3]]


_C1, _S1, _R2 = np.cos(np.pi / 8), np.sin(np.pi / 8), np.sqrt(0.5)


def _tw(n, j, s):
    return np.exp(s * 2j * np.pi * n * (4 * j + 1) / 128)


def _fwd_stage1(n, u0, u1, u2, u3):
    u0, u1, u2, u3 = (1, u0), (1, u1), (1, u2), (1, u3)
    t = _scale(u2, _R2)
    p, m_ = _add(u0, t), _sub(u0, t)
    c1u1, s1u1, c1u3, s1u3 = _scale(u1, _C1), _scale(u1, _S1), _scale(u3, _C1), _scale(u3, _S1)
    a, b = _add(c1u1, s1u3), _add(s1u1, c1u3)
    d, e = _sub(c1u1, s1u3), _sub(s1u1, c1u3)
    sj = [(_add(p, a), _neg(_add(t, b))), (_sub(m_, e), _sub(t, d)),
          (_sub(p, a), _sub(b, t)), (_add(m_, e), _add(t, d))]
    out = [sj[j] if n == 0 else _cmul_const(sj[j], _tw(n, j, -1)) for j in range(4)]
    return [(_val(re), _val(im)) for re, im in out]


def _fwd_stage2(t):
    out = _fft8([((1, re), (1, im)) for re, im in t], -1)
    return [(_val(re), _val(im)) for re, im in out]


def _inv_stage1(j, b):
    out = _fft8([((1, re), (1, im)) for re, im in b], 1)
    out = [out[n] if n == 0 else _cmul_const(out[n], _tw(n, j, 1)) for n in range(8)]
    return [(_val(re), _val(im)) for re, im in out]


def _inv_stage2(s):
    (x0, y0), (x1, y1), (x2, y2), (x3, y3) = [((1, re), (1, im)) for re, im in s]
    p, a, b = _add(x0, x2), _sub(x0, x2), _sub(y2, y0)
    m_, e, d = _add(x1, x3), _sub(x3, x1), _sub(y3, y1)
    t = _add(_sub(_add(y1, y3), _add(y0, y2)), _sub(p, m_))
    return [_val(_add(p, m_)),
            _val(_add(_scale(_add(a, d), _C1), _scale(_add(b, e), _S1))),
            _val(_scale(t, _R2)),
            _val(_add(_scale(_sub(a, d), _S1), _scale(_sub(b, e), _C1)))]


def _phi(t):
    return jnp.where(t > 0, t + 1.0, jnp.exp(t)) + 1e-6


def _dot(a, b):
    return jnp.dot(a, b, preferred_element_type=F32)


def _dot_nt(a, b):
    return jax.lax.dot_general(a, b, (((1,), (1,)), ((), ())), preferred_element_type=F32)


def _ld(ref, lead, r0, n):
    lead = lead if isinstance(lead, tuple) else (lead,)
    return pltpu.bitcast(ref.bitcast(jnp.uint32)[(*lead, pl.ds(r0 // 2, n // 2), slice(None))], BF)


def _cat(parts, axis):
    return parts[0] if len(parts) == 1 else jnp.concatenate(parts, axis=axis)


def _spread(stream, extra):
    out = []
    extra = sorted(extra, key=lambda e: e[0])
    e = 0
    for pos, item in enumerate(stream):
        while e < len(extra) and extra[e][0] <= pos:
            out.append(extra[e][1])
            e += 1
        out.append(item)
    return out + [t for _, t in extra[e:]]


def _merge(a, b):
    keyed = [((t + 0.5) / len(x), s, item) for s, x in enumerate((a, b)) for t, item in enumerate(x)]
    return [item for _, _, item in sorted(keyed, key=lambda e: e[:2])]


def _kernel(zero_hbm, x_hbm, wqkv_hbm, wo_hbm, q_hbm, k_hbm, v_hbm, sk_hbm, h_hbm, d_hbm, tab_hbm,
            out_hbm,
            x_v, wq_v, wk_v, wv_v, wo_v, q_v, k_v, v_v, h_v, tab_v, fwd_v, inv_v,
            wkt_s, pkt_s, g_s, kv_s, m_s, zb_s, pq_s, r_s, oa_s, ob_s,
            a_s, yf_s, z_s, w_s, zero_ref, sk_ref, d_ref, sems):
    n_sem = [0]
    n_wait = [0]

    def zero(i):
        return zero_ref[i % NZ]

    def group(pairs):
        sem = sems.at[n_sem[0]]
        n_sem[0] += 1
        return [pltpu.make_async_copy(src, dst, sem) for src, dst in pairs]

    def start(g):
        for c in (g if 'nodma' not in DBG else []):
            c.start()

    def wait(g):
        if 'scope' in DBG:
            n_wait[0] += 1
            with jax.named_scope(f"region_w{n_wait[0]}"):
                for c in g:
                    c.wait()
            return
        for c in (g if 'nodma' not in DBG else []):
            c.wait()

    def col(ref, j):
        return ref.at[:, pl.ds(j * 128, 128)]

    def split(src, dst, n):
        step = src.shape[0] // n
        return [(src.at[pl.ds(t * step, step), :], dst.at[pl.ds(t * step, step), :]) for t in range(n)]

    cp_x = [group([(x_hbm.at[pl.ds(r0, 256), pl.ds(j * 128, 128)], x_v.at[j, pl.ds(r0, 256), :])
                   for j in range(NT)]) for r0 in range(0, S, 256)]
    cp_wq = group([(col(wqkv_hbm, j), wq_v.at[j]) for j in range(NT)])
    cp_wk = [group(split(col(wqkv_hbm, NT + g), wk_v.at[g], 4)) for g in range(NT)]
    cp_wvo = group([(col(wqkv_hbm, 2 * NT + g), wv_v.at[g]) for g in range(NT)]
                   + [(col(wo_hbm, j), wo_v.at[j]) for j in range(NT)])
    parts = [8, 8] + [2] * (NB - 2)
    cp_q = [group(split(col(q_hbm, i), q_v.at[i], 2)) for i in range(NB)]
    cp_kv = [group(split(col(k_hbm, i), k_v.at[i], parts[i]) + split(col(v_hbm, i), v_v.at[i], parts[i]))
             for i in range(NB)]
    cp_h = [group(split(h_hbm.at[pl.ds(i * CB, CB), :], h_v.at[i], parts[i])) for i in range(NB)]
    cp_tab = group([(tab_hbm, tab_v), (sk_hbm, sk_ref), (d_hbm, d_ref)])
    cp_zero = group([(zero_hbm, zero_ref)])
    cp_ob = [group(split(ob_s.at[i], col(out_hbm, NT + i), 8 if i == NB - 1 else 2)) for i in range(NB)]
    oa_spans = []

    def cp_oa(t):
        r0, n = oa_spans[t]
        pairs = split(oa_s.at[pl.ds(r0, n), :], out_hbm.at[pl.ds(r0, n), pl.ds(0, D)], 8)
        return [pltpu.make_async_copy(src, dst, sems.at[n_sem[0] + t]) for src, dst in pairs]

    rows_done = [0, 0]

    def sync(waits=(), starts=()):
        def run():
            for g in starts:
                start(g)
            done, sent = rows_done
            if done > sent:
                oa_spans.append((sent, done - sent))
                start(cp_oa(len(oa_spans) - 1))
                rows_done[1] = done
            for g in waits:
                wait(g)
        return 0, run

    RP = 64

    def area(name, r0, n=8):
        return pl.ds(AT[name] + r0, n), slice(None)

    def b_prepare(i):
        def widen(p):
            def run():
                w_s[area("k", HALO + p * RP, RP)] = _ld(k_v, i, p * RP, RP).astype(F32)
            return 30, run

        def gate(p):
            def run():
                taps = sk_ref[:, pl.ds(i * CB, CB)].astype(F32)
                if INREG:
                    k = (_ld(k_v, i, p * RP - 16, RP + 16).astype(F32) if p > 0 else
                         _cat([jnp.zeros((16, CB), F32), _ld(k_v, i, 0, RP).astype(F32)], 0))
                    acc = k[16:] * taps[0:1, :]
                    for j in range(1, 4):
                        acc = acc + k[16 - j:16 - j + RP] * taps[j:j + 1, :]
                else:
                    acc = w_s[area("k", HALO + p * RP, RP)] * taps[0:1, :]
                    for j in range(1, 4):
                        acc = acc + w_s[area("k", HALO + p * RP - j, RP)] * taps[j:j + 1, :]
                w_s[area("u", p * RP, RP)] = acc * _ld(v_v, i, p * RP, RP).astype(F32)
            return (130 if INREG else 80), run

        def transpose(p):
            def run():
                ht = h_v[i, :, pl.ds(p * 128, 128)].astype(F32).T
                if p == 0:
                    skip = d_ref[:, pl.ds(i * CB, CB)].astype(F32)
                    lag = jax.lax.broadcasted_iota(jnp.int32, (128, CB), 0)
                    ht = ht + jnp.where(lag == 0, skip, 0.0)
                w_s[area("h", p * 128, 128)] = ht
            return 70, run

        prep = ([sync([cp_kv[0], cp_x[4]], cp_x[5:] + [cp_h[1], cp_kv[1]])] if i == 0 else []) + ([] if INREG else [widen(0)])
        for p in range(S // RP):
            prep += ([widen(p + 1)] if p + 1 < S // RP and not INREG else []) + [gate(p)]
        return [transpose(p) for p in range(S // 128)], prep

    def b_forward(i, prep):
        def stage1(h, j, n):
            def run():
                out = _fwd_stage1(n, *[w_s[area("uh"[h], N1 * (n + 8 * m) + 8 * j)] for m in range(4)])
                for r in range(4):
                    for part in range(2):
                        w_s[area("tf", 512 * (8 * h + j) + 16 * (8 * r + n) + 8 * part)] = out[r][part]
            return (46 if n else 32), run

        def stage2(h, j, r):
            def run():
                out = _fwd_stage2([[w_s[area("tf", 512 * (8 * h + j) + 16 * (8 * r + n) + 8 * part)]
                                    for part in range(2)] for n in range(8)])
                for l in range(8):
                    a_s[i % 2, h, r + 4 * l, pl.ds(16 * j, 16), :] = _cat(out[l], 0).astype(BF)
            return 64, run

        tasks = []
        cols = [(h, j) for h in (1, 0) for j in range(N1 // 8)]
        for c, (h, j) in enumerate(cols):
            now = [stage1(h, j, n) for n in range(8)]
            now += [stage2(*cols[c - 1], r) for r in range(4)] if c > 0 else []
            lo = 4 if i == 0 else 0
            if lo <= c < 8:
                share = prep[len(prep) * (c - lo) // (8 - lo):len(prep) * (c + 1 - lo) // (8 - lo)]
                now = _merge(now, share)
            tasks += now
        return tasks + [stage2(*cols[-1], r) for r in range(4)]

    def b_inverse(i):
        def stage1(j, r):
            def run():
                out = _inv_stage1(r, [[w_s[area("b", 128 * (N2 * (i % 2) + r + 4 * l) + 16 * j + 8 * part)]
                                       for part in range(2)] for l in range(8)])
                for n in range(8):
                    for part in range(2):
                        w_s[area("ti", 512 * j + 16 * (4 * n + r) + 8 * part)] = out[n][part]
            return 100, run

        def stage2(jp, n):
            def run():
                ys = [_inv_stage2([[w_s[area("ti", 512 * j + 16 * (4 * n + r) + 8 * part)] for part in range(2)]
                                   for r in range(4)]) for j in (2 * jp, 2 * jp + 1)]
                for m in range(4):
                    r0 = N1 * (n + 8 * m) + 16 * jp
                    y = _cat([ys[0][m], ys[1][m]], 0)
                    ob_s[i, pl.ds(r0, 16), :] = (_ld(q_v, i, r0, 16).astype(F32) * y).astype(BF)
            return 66, run

        tasks = []
        for jp in range(N1 // 16 + 1):
            first = [stage1(j, r) for j in (2 * jp, 2 * jp + 1) for r in range(4)] if jp < N1 // 16 else []
            tasks += _merge(first, [stage2(jp - 1, n) for n in range(8)] if jp > 0 else [])
        return tasks

    def dft_matrix(k2):
        def run():
            f = (tab_v[pl.ds(0, 128), :] * tab_v[pl.ds(256 + k2, 1), :]
                 + tab_v[pl.ds(128, 128), :] * tab_v[pl.ds(256 + N2 + k2, 1), :])
            fwd_v[k2] = f.astype(BF)
            inv_v[k2] = (f.T * (1.0 / S)).astype(BF)
        return 0, run

    def b_middle(i):
        def forward(k2):
            def run():
                rhs = _cat([_ld(a_s, (i % 2, h, k2), 0, 128) for h in range(2)], 1)
                xf = _dot(_ld(fwd_v, k2 + zero(i), 0, 128), rhs)
                ur, ui, hr, hi = xf[:N1, :CB], xf[N1:, :CB], xf[:N1, CB:], xf[N1:, CB:]
                if 'f' in XF and k2 % 2 == 0:
                    urgent(xf[:8, :128])
                yf_s[k2] = _cat([ur * hr - ui * hi, ur * hi + ui * hr], 0).astype(BF)
            return 64, run

        def inverse(k2):
            def run():
                b = _dot(_ld(inv_v, k2 + zero(i), 0, 128), _ld(yf_s, k2, 0, 128))
                if 'i' in XF and k2 % 4 == 0:
                    urgent(b[:8, :])
                w_s[area("b", 128 * (N2 * (i % 2) + k2), 128)] = b
            return 32, run

        tasks = []
        for k4 in range(N2 // 4 + 1):
            if k4 < N2 // 4:
                tasks += [[forward(4 * k4), forward(4 * k4 + 1)], [forward(4 * k4 + 2), forward(4 * k4 + 3)]]
            if k4 > 0:
                tasks += [[inverse(4 * k4 - 4 + r) for r in range(4)]]
        return tasks

    def head_mask():
        r = jax.lax.broadcasted_iota(jnp.int32, (128, 128), 0) // DH
        c = jax.lax.broadcasted_iota(jnp.int32, (128, 128), 1) // DH
        return r == c

    room = {}
    mid_chain = set()

    lead_chain = [None]

    def urgent(value):
        if PRIO:
            c = value if lead_chain[0] is None else lead_chain[0] + value
            for _ in range(PRIO):
                c = pltpu.roll(c, 1, 1) if PKIND == 'roll' else jnp.exp(c)
            lead_chain[0] = c

    def fence(value):
        w_s[pl.ds(pl.multiple_of(zero(0) + AT["fence"], 8), 8), :] = value
        yf_s.bitcast(jnp.uint32)[zero(0) + N2, pl.ds(0, 8), :] = pltpu.bitcast(value, jnp.uint32)

    def chain(n_tiles, n_cols, operands, dot, finish):
        wide = n_cols if WIDE else 1
        deep = 4 // wide
        acc = [None]

        def piece(j0, k0):
            def run():
                d = dot(*operands(range(k0, k0 + deep), range(j0, j0 + wide)))
                acc[0] = d if k0 == 0 else acc[0] + d
                fence(d[:8, :128])
                urgent(d[:8, :128])
                if k0 + deep == n_tiles:
                    for t in range(wide):
                        finish(j0 + t, acc[0][:, 128 * t:128 * t + 128])
            if j0 + k0 > 0:
                mid_chain.add(run)
            if k0 + deep == n_tiles:
                room[run] = ROOM[0]
            return 128, run
        return [piece(j0, k0) for j0 in range(0, n_cols, wide) for k0 in range(0, n_tiles, deep)]

    followers = {}

    def chain_then(operands, dot, part):
        slot = len(followers) % 4

        def park(j, acc):
            w_s[area("acc", 256 * slot + 128 * j, 128)] = acc

        def quarter(t):
            def run():
                part(pl.ds(32 * t, 32), 32 * t, *[w_s[area("acc", 256 * slot + 128 * half + 32 * t, 32)] for half in range(2)])
            room[run] = ROOM[1]
            return 0, run
        pieces = chain(NT, 2, operands, dot, park)
        followers[pieces[-1][1]] = [quarter(t) for t in range(4)]
        return pieces

    def a_transpose_wk(g):
        def tile(j):
            def run():
                wkt_s[g, j] = _ld(wk_v, g, j * 128, 128).astype(F32).T.astype(BF)
            return 0, run
        return [tile(j) for j in range(NT)]

    def a_keys(g, c):
        def operands(ks, js):
            return (_cat([_ld(wkt_s, (g + zero(c), k), 0, 128) for k in ks], 1),
                    _cat([_ld(x_v, k + zero(g), c * 256 + 128 * js[0], 128 * len(js)) for k in ks], 1))

        def part(rows, r0, lo, hi):
            lo, hi = _phi(lo), _phi(hi)
            pkt_s[g, 2 * c, rows, :] = lo.astype(BF)
            pkt_s[g, 2 * c + 1, rows, :] = hi.astype(BF)
            total = lo + hi
            if c < S // 256 - 1:
                z_s[g, c, rows, :] = total
            else:
                for b in range(c):
                    total = total + z_s[g, b, rows, :]
                z = jnp.broadcast_to(jnp.sum(total, axis=1, keepdims=True), (32, 128))
                head = jax.lax.broadcasted_iota(jnp.int32, (32, 128), 1) // DH
                zb_s[g, rows, :] = jnp.where(head == r0 // DH, z, 0.0).astype(BF)
        return chain_then(operands, _dot_nt, part)

    def a_gram(g):
        def block(n):
            def operands(ks, js):
                return (_cat([_ld(pkt_s, (g, k), 0, 128) for k in ks], 1),
                        _cat([_ld(x_v, 2 * n + j + zero(NT + g), 128 * ks[0], 128 * len(ks)) for j in js], 1))

            def finish(j, acc):
                g_s[g, 2 * n + j] = acc.astype(BF)
            return chain(S // 128, 2, operands, _dot, finish)
        return [t for n in range(D // 256) for t in block(n)]

    def a_kv(g):
        acc = [None]

        def piece(kk):
            def run():
                d = _dot(_cat([_ld(g_s, (g, j), 0, 128) for j in range(4 * kk, 4 * kk + 4)], 1),
                         _ld(wv_v, g, kk * 512, 512))
                fence(d[:8, :])
                urgent(d[:8, :])
                if kk == 0:
                    acc[0] = d
                else:
                    kv_s[g] = jnp.where(head_mask(), acc[0] + d, 0.0).astype(BF)
            if kk > 0:
                mid_chain.add(run)
            return 128, run
        return [piece(0), piece(1)]

    def a_mix(g, half):
        def run():
            js = range(4 * half, 4 * half + 4)
            m = _dot(_ld(kv_s, g, 0, 128), _cat([_ld(wo_v, j, g * 128, 128) for j in js], 1))
            for t, j in enumerate(js):
                m_s[j, pl.ds(g * 128, 128), :] = m[:, t * 128:(t + 1) * 128].astype(BF)
        return 128, run

    def a_query(c, n):
        def operands(ks, js):
            return (_cat([_ld(x_v, k + zero(2 * NT + 2 * n + js[0]), c * 128, 128) for k in ks], 1),
                    _cat([_ld(wq_v, 2 * n + j + zero(c), 128 * ks[0], 128 * len(ks)) for j in js], 1))

        def part(rows, r0, lo, hi):
            pq_s[c, 2 * n, rows, :] = _phi(lo).astype(BF)
            pq_s[c, 2 * n + 1, rows, :] = _phi(hi).astype(BF)
        return chain_then(operands, _dot, part)

    def a_normalise(c, half):
        def run():
            for g in range(4 * half, 4 * half + 4):
                pq = _ld(pq_s, (c, g), 0, 128)
                den = _dot(pq, _ld(zb_s, g + zero(c), 0, 128)) + 1e-6
                if 'n' in XF and g % 4 == 0:
                    urgent(den[:8, :])
                inv = pl.reciprocal(den, approx=True)
                inv = inv * (2.0 - den * inv)
                r_s[c, g] = (pq.astype(F32) * inv).astype(BF)
        room[run] = ROOM[2]
        return 128, run

    def a_out(c, n):
        def operands(ks, js):
            return (_cat([_ld(r_s, (c, k), 0, 128) for k in ks], 1),
                    _cat([_ld(m_s, 2 * n + j + zero(c), 128 * ks[0], 128 * len(ks)) for j in js], 1))

        def finish(j, acc):
            oa_s[pl.ds(c * 128, 128), pl.ds(n * 256 + j * 128, 128)] = acc.astype(BF)
            if n == D // 256 - 1 and j == 1:
                rows_done[0] = (c + 1) * 128
        return chain(NT, 2, operands, _dot, finish)

    def starter(*groups):
        def run():
            for g in groups:
                start(g)
        return 0, run

    a_stream, extra = [], []
    n_g = n_c = 0
    for grow in "gcgcggcggcggcccc":
        if grow == "g":
            a_stream += [t for c in range(n_c) for t in a_keys(n_g, c)]
            n_g += 1
        else:
            a_stream += [t for g in range(n_g) for t in a_keys(g, n_c)]
            n_c += 1
    extra += [(0, sync([cp_x[0], cp_wk[1]], [cp_wk[2], cp_wk[3]])),
              (8, sync([cp_x[1], cp_wk[2], cp_wk[3]], [cp_x[2], cp_wk[4], cp_wk[5]])),
              (32, sync([cp_x[2], cp_wk[4], cp_wk[5]], [cp_x[3], cp_wk[6], cp_wk[7], cp_tab, cp_h[0]])),
              (F0_AT, sync([cp_x[3], cp_wk[6], cp_wk[7], cp_tab, cp_h[0]], [cp_kv[0], cp_x[4]]))]
    extra += [(F0_AT + 2 + 2 * k2, dft_matrix(k2)) for k2 in range(N2)]
    for g, (at, step) in {1: (0, 0.45), 2: (8, 0.75), 3: (16, 0.75), 4: (32, 1.5), 5: (46, 1.5), 6: (62, 3),
                          7: (86, 3)}.items():
        extra += [(at + int(step * j), t) for j, t in enumerate(a_transpose_wk(g))]
    for g in range(NT):
        at = len(a_stream)
        if g >= 5:
            for t, gg in enumerate(range(3 * (g - 5), min(3 * (g - 4), NT - 1))):
                extra += [(at + 8 * t + 8, p) for p in a_kv(gg)] + [(at + 8 * t + 16, a_mix(gg, 0)), (at + 8 * t + 16, a_mix(gg, 1))]
        a_stream += a_gram(g)
    a_stream = _spread(a_stream, extra)
    tail = []
    n_c = S // 128
    for c in range(n_c + 1):
        stream = [t for n in range(D // 256) for t in a_query(c, n)] if c < n_c else []
        stream += [t for n in range(D // 256) for t in a_out(c - 1, n)] if c > 0 else []
        at = len(a_stream)
        if c == 0:
            tail += [(at + 4, p) for p in a_kv(NT - 1)] + [(at + 8, a_mix(NT - 1, 0)), (at + 8, a_mix(NT - 1, 1))]
        if c < n_c:
            tail += [(at + 12, a_normalise(c, 0)), (at + 24, a_normalise(c, 1))]
        a_stream += stream
    a_stream = _spread(a_stream, tail)
    spread, pending = [], []
    for item in a_stream:
        spread.append(item)
        if item[0] > 0 and pending:
            spread.append(pending.pop(0))
        pending += followers.get(item[1], [])
    a_stream = spread + pending

    v_regions, m_regions = [], []
    for r in range(NB + 2):
        v = b_inverse(r - 2) if r >= 2 else []
        if r < NB:
            transposes, prep = b_prepare(r)
            v = _merge(v, transposes) + b_forward(r, prep)
        if r == NB + 1:
            v.append(sync(starts=[cp_ob[NB - 1]]))
        v_regions.append(v)
        m_regions.append(b_middle(r - 1) if 1 <= r <= NB and 'nomid' not in DBG else [])
    v_cost = [sum(c for c, _ in v) for v in v_regions]
    m_cost = [sum(c for grp in m for c, _ in grp) for m in m_regions]
    total = sum(c for c, _ in a_stream) + sum(m_cost)
    weight = [c + w for c, w in zip(v_cost, REGION_BIAS)]

    sync([cp_zero], [cp_zero, cp_wk[0], cp_x[0]])[1]()
    w_s[area("k", 0)] = jnp.zeros((HALO, CB), F32)
    for ref in (pkt_s, r_s, g_s, kv_s, pq_s, a_s, z_s, fwd_v, inv_v):
        lead = (zero(0),) + (0,) * (len(ref.shape) - 3)
        ref[(*lead, pl.ds(0, 16), slice(None))] = jnp.zeros((16, CB), ref.dtype)
    sync([cp_wk[0]], [cp_wk[1], cp_x[1]])[1]()
    for _, run in a_transpose_wk(0):
        run()

    ai, clock, ob_sent = 0, 0, [0]
    for r in range(NB + 2):
        end = FIRST + (total - FIRST) * sum(weight[1:r + 1]) / sum(weight[1:])
        a_end, t = ai, clock + m_cost[r]
        while a_end < len(a_stream) and (t < end or a_stream[a_end][0] == 0
                                         or a_stream[a_end][1] in mid_chain or r == NB + 1):
            t += a_stream[a_end][0]
            a_end += 1
        length = sum(room.get(run, cost) for cost, run in a_stream[ai:a_end])
        v, m = v_regions[r], m_regions[r]
        lead, trail = 0, (V_TRAIL if r == NB + 1 else 0)
        if r == 0:
            first = [p for p, (cost, _) in enumerate(a_stream) if cost > 0][F0_AT + 2]
            lead = sum(room.get(run, cost) for cost, run in a_stream[:first])
        v_time, acc_cost = [], 0
        for c, _ in v:
            v_time.append(lead + (length - lead - trail) * acc_cost / v_cost[r])
            acc_cost += c

        def region(ai, a_end, length, v, m, v_time):
            now, pa, pm, pv = 0, ai, 0, 0
            while pa < a_end or pm < len(m):
                if pm < len(m) and ((length - M_TRAIL) * pm / len(m) <= now or pa == a_end):
                    todo = m[pm]
                    pm += 1
                else:
                    todo = [a_stream[pa]]
                    pa += 1
                for cost, run in todo:
                    run()
                    now += 0 if len(todo) > 1 else room.get(run, cost)
                while pv < len(v) and v_time[pv] <= now:
                    v[pv][1]()
                    pv += 1
            for _, run in v[pv:]:
                run()
            if lead_chain[0] is not None:
                fence(lead_chain[0])
                lead_chain[0] = None

        if r in BLOCKS:
            nxt = min([b for b in BLOCKS if b > r] + [NB + 2])
            far = min([b for b in BLOCKS if b > nxt] + [NB + 2])

            def needs(lo, hi):
                return ([g for i in range(max(lo, 1), min(hi, NB)) for g in (cp_h[i], cp_kv[i])]
                        + [cp_q[i - 2] for i in range(max(lo, 2), hi)])
            waits, starts = needs(r, nxt), (needs(nxt, far) if r > 0 else [])
            while ob_sent[0] + 3 <= r:
                starts.append(cp_ob[ob_sent[0]])
                ob_sent[0] += 1
            pieces = sum(c > 0 for c, _ in a_stream[:ai])
            if r == 1:
                assert F0_AT + 2 * N2 + 2 < pieces <= 160 and nxt == 2
                waits, starts = waits + cp_x[5:], starts + [cp_wvo]
            if r == 2:
                starts = starts + [cp_wq]
            if r == 3:
                assert pieces <= 256 + 5 * 32 + 8
                waits = waits + [cp_wvo, cp_wq]
            sync(waits, starts)[1]()
            todo_regions = []
        todo_regions.append(functools.partial(region, ai, a_end, length, v, m, v_time))
        if r + 1 in BLOCKS or r == NB + 1:
            with jax.named_scope(f"region{r}"):
                pl.when(zero(r) == 0)(lambda: [run() for run in todo_regions] and None)
        ai, clock = a_end, t

    sync()[1]()
    with jax.named_scope("drain"):
        for g in [cp_oa(t) for t in range(len(oa_spans))] + cp_ob:
            wait(g)


@jax.jit
def pallas_concat_heads__linear_attn_block__ssm_conv_h3__prompt_kernel(
    A_x: jax.Array,
    A_wqkv: jax.Array,
    A_wo: jax.Array,
    B_q: jax.Array,
    B_k: jax.Array,
    B_v: jax.Array,
    B_shift_k: jax.Array,
    B_ssm_k: jax.Array,
    B_ssm_D: jax.Array,
):
    hbm = pl.BlockSpec(memory_space=pl.ANY)
    scratch = [
        pltpu.VMEM((NT, S, 128), BF),
        pltpu.VMEM((NT, D, 128), BF),
        pltpu.VMEM((NT, D, 128), BF),
        pltpu.VMEM((NT, D, 128), BF),
        pltpu.VMEM((NT, D, 128), BF),
        pltpu.VMEM((NB, S, CB), BF),
        pltpu.VMEM((NB, S, CB), BF),
        pltpu.VMEM((NB, S, CB), BF),
        pltpu.VMEM((NB, CB, S), BF),
        pltpu.VMEM(_TABLES.shape, F32),
        pltpu.VMEM((N2, 128, 128), BF),
        pltpu.VMEM((N2, 128, 128), BF),
        pltpu.VMEM((NT, NT, 128, 128), BF),
        pltpu.VMEM((NT, S // 128, 128, 128), BF),
        pltpu.VMEM((NT, NT, 128, 128), BF),
        pltpu.VMEM((NT, 128, 128), BF),
        pltpu.VMEM((NT, D, 128), BF),
        pltpu.VMEM((NT, 128, 128), BF),
        pltpu.VMEM((S // 128, NT, 128, 128), BF),
        pltpu.VMEM((S // 128, NT, 128, 128), BF),
        pltpu.VMEM((S, D), BF),
        pltpu.VMEM((NB, S, CB), BF),
        pltpu.VMEM((2, 2, N2, 128, CB), BF),
        pltpu.VMEM((N2 + 1, 128, CB), BF),
        pltpu.VMEM((NT, S // 256, 128, 128), F32),
        pltpu.VMEM((W_ROWS, 128), F32),
        pltpu.SMEM((NZ,), jnp.int32),
        pltpu.VMEM((4, D), BF),
        pltpu.VMEM((1, D), BF),
        pltpu.SemaphoreType.DMA((64,)),
    ]
    out = pl.pallas_call(
        _kernel,
        out_shape=jax.ShapeDtypeStruct((S, 2 * D), BF),
        in_specs=[hbm] * 11,
        out_specs=hbm,
        scratch_shapes=scratch,
        compiler_params=pltpu.CompilerParams(vmem_limit_bytes=100 * 1024 * 1024),
    )(np.zeros((NZ,), np.int32), A_x.reshape(S, D), A_wqkv, A_wo, B_q.reshape(S, D), B_k.reshape(S, D), B_v.reshape(S, D),
      B_shift_k.T, B_ssm_k, B_ssm_D.reshape(1, D), _TABLES)
    return out.reshape(1, S, 2 * D)
```

```python
import functools

import numpy as np
import jax
import jax.numpy as jnp
import jax.experimental.pallas as pl
import jax.experimental.pallas.tpu as pltpu

S = 2048
D = 1024
DH = 32
N1, N2 = 64, 32
CB = 128
NB = D // CB
NT = D // 128
HALO = 8
_AREAS = (("k", HALO + S), ("u", S), ("h", S), ("tf", 4 * S), ("b", 2 * N2 * 128), ("ti", 2 * S),
          ("acc", 4 * 256), ("fence", 8))
AT = {name: sum(n for _, n in _AREAS[:i]) for i, (name, _) in enumerate(_AREAS)}
W_ROWS = sum(n for _, n in _AREAS)
NZ = 32
F0_AT = 48
V_TRAIL, M_TRAIL = 2500, 300
ROOM = (128, 0, 0)
FIRST = 160 * 128
REGION_BIAS = [0] + [0] * NB + [2500]
DBG = ''
INREG = False
WIDE, BLOCKS = True, range(NB + 2)
PRIO, PKIND, XF, M_WEIGHT = 7, 'exp', 'fin', 0.0
BF = jnp.bfloat16
F32 = jnp.float32


def _dft_tables():
    idx = np.arange(N1)
    col = 16 * (idx // 8) + (idx % 8)
    e = np.exp(-2j * np.pi * np.outer(idx, idx) / N1)
    t = np.exp(-2j * np.pi * np.outer(np.arange(N2) + 0.25, idx) / S)
    tab = np.zeros((2 * 128 + 2 * N2, 128), np.float64)
    p, q, tr, ti = tab[:128], tab[128:256], tab[256:256 + N2], tab[256 + N2:]
    p[:N1, col], p[:N1, col + 8], p[N1:, col], p[N1:, col + 8] = e.real, -e.imag, e.imag, e.real
    q[:N1, col], q[:N1, col + 8], q[N1:, col], q[N1:, col + 8] = -e.imag, -e.real, e.real, -e.imag
    tr[:, col], tr[:, col + 8], ti[:, col], ti[:, col + 8] = t.real, t.real, t.imag, t.imag
    return tab.astype(np.float32)


_TABLES = _dft_tables()


def _add(a, b):
    (sa, xa), (sb, xb) = a, b
    if sa == sb:
        return (sa, xa + xb)
    return (1, xa - xb) if sa > 0 else (1, xb - xa)


def _neg(a):
    return (-a[0], a[1])


def _sub(a, b):
    return _add(a, _neg(b))


def _scale(a, c):
    return (1, a[1] * np.float32(a[0] * c))


def _val(a):
    return a[1] if a[0] > 0 else -a[1]


def _cadd(a, b):
    return (_add(a[0], b[0]), _add(a[1], b[1]))


def _csub(a, b):
    return (_sub(a[0], b[0]), _sub(a[1], b[1]))


def _cmul_i(a, s):
    return (_neg(a[1]), a[0]) if s > 0 else (a[1], _neg(a[0]))


def _cmul_const(a, w):
    c, s = float(np.real(w)), float(np.imag(w))
    return (_add(_scale(a[0], c), _scale(a[1], -s)), _add(_scale(a[0], s), _scale(a[1], c)))


def _fft4(x, s):
    a0, a1 = _cadd(x[0], x[2]), _cadd(x[1], x[3])
    b0, b1 = _csub(x[0], x[2]), _cmul_i(_csub(x[1], x[3]), s)
    return [_cadd(a0, a1), _cadd(b0, b1), _csub(a0, a1), _csub(b0, b1)]


def _fft8(x, s):
    r = np.sqrt(0.5)
    a = [_cadd(x[n], x[n + 4]) for n in range(4)]
    b = [_csub(x[n], x[n + 4]) for n in range(4)]
    t = _cadd(b[1], _cmul_i(b[1], s))
    b[1] = (_scale(t[0], r), _scale(t[1], r))
    b[2] = _cmul_i(b[2], s)
    t = _csub(_cmul_i(b[3], s), b[3])
    b[3] = (_scale(t[0], r), _scale(t[1], r))
    ev, od = _fft4(a, s), _fft4(b, s)
    return [ev[0], od[0], ev[1], od[1], ev[2], od[2], ev[3], od[3]]


_C1, _S1, _R2 = np.cos(np.pi / 8), np.sin(np.pi / 8), np.sqrt(0.5)


def _tw(n, j, s):
    return np.exp(s * 2j * np.pi * n * (4 * j + 1) / 128)


def _fwd_stage1(n, u0, u1, u2, u3):
    u0, u1, u2, u3 = (1, u0), (1, u1), (1, u2), (1, u3)
    t = _scale(u2, _R2)
    p, m_ = _add(u0, t), _sub(u0, t)
    c1u1, s1u1, c1u3, s1u3 = _scale(u1, _C1), _scale(u1, _S1), _scale(u3, _C1), _scale(u3, _S1)
    a, b = _add(c1u1, s1u3), _add(s1u1, c1u3)
    d, e = _sub(c1u1, s1u3), _sub(s1u1, c1u3)
    sj = [(_add(p, a), _neg(_add(t, b))), (_sub(m_, e), _sub(t, d)),
          (_sub(p, a), _sub(b, t)), (_add(m_, e), _add(t, d))]
    out = [sj[j] if n == 0 else _cmul_const(sj[j], _tw(n, j, -1)) for j in range(4)]
    return [(_val(re), _val(im)) for re, im in out]


def _fwd_stage2(t):
    out = _fft8([((1, re), (1, im)) for re, im in t], -1)
    return [(_val(re), _val(im)) for re, im in out]


def _inv_stage1(j, b):
    out = _fft8([((1, re), (1, im)) for re, im in b], 1)
    out = [out[n] if n == 0 else _cmul_const(out[n], _tw(n, j, 1)) for n in range(8)]
    return [(_val(re), _val(im)) for re, im in out]


def _inv_stage2(s):
    (x0, y0), (x1, y1), (x2, y2), (x3, y3) = [((1, re), (1, im)) for re, im in s]
    p, a, b = _add(x0, x2), _sub(x0, x2), _sub(y2, y0)
    m_, e, d = _add(x1, x3), _sub(x3, x1), _sub(y3, y1)
    t = _add(_sub(_add(y1, y3), _add(y0, y2)), _sub(p, m_))
    return [_val(_add(p, m_)),
            _val(_add(_scale(_add(a, d), _C1), _scale(_add(b, e), _S1))),
            _val(_scale(t, _R2)),
            _val(_add(_scale(_sub(a, d), _S1), _scale(_sub(b, e), _C1)))]


def _phi(t):
    return jnp.where(t > 0, t + 1.0, jnp.exp(t)) + 1e-6


def _dot(a, b):
    return jnp.dot(a, b, preferred_element_type=F32)


def _dot_nt(a, b):
    return jax.lax.dot_general(a, b, (((1,), (1,)), ((), ())), preferred_element_type=F32)


def _ld(ref, lead, r0, n):
    lead = lead if isinstance(lead, tuple) else (lead,)
    return pltpu.bitcast(ref.bitcast(jnp.uint32)[(*lead, pl.ds(r0 // 2, n // 2), slice(None))], BF)


def _cat(parts, axis):
    return parts[0] if len(parts) == 1 else jnp.concatenate(parts, axis=axis)


def _spread(stream, extra):
    out = []
    extra = sorted(extra, key=lambda e: e[0])
    e = 0
    for pos, item in enumerate(stream):
        while e < len(extra) and extra[e][0] <= pos:
            out.append(extra[e][1])
            e += 1
        out.append(item)
    return out + [t for _, t in extra[e:]]


def _merge(a, b):
    keyed = [((t + 0.5) / len(x), s, item) for s, x in enumerate((a, b)) for t, item in enumerate(x)]
    return [item for _, _, item in sorted(keyed, key=lambda e: e[:2])]


def _kernel(zero_hbm, x_hbm, wqkv_hbm, wo_hbm, q_hbm, k_hbm, v_hbm, sk_hbm, h_hbm, d_hbm, tab_hbm,
            out_hbm,
            x_v, wq_v, wk_v, wv_v, wo_v, q_v, k_v, v_v, h_v, tab_v, fwd_v, inv_v,
            wkt_s, pkt_s, g_s, kv_s, m_s, zb_s, pq_s, r_s, oa_s, ob_s,
            a_s, yf_s, z_s, w_s, zero_ref, sk_ref, d_ref, sems):
    n_sem = [0]
    n_wait = [0]

    def zero(i):
        return zero_ref[i % NZ]

    def group(pairs):
        sem = sems.at[n_sem[0]]
        n_sem[0] += 1
        return [pltpu.make_async_copy(src, dst, sem) for src, dst in pairs]

    def start(g):
        for c in (g if 'nodma' not in DBG else []):
            c.start()

    def wait(g):
        if 'scope' in DBG:
            n_wait[0] += 1
            with jax.named_scope(f"region_w{n_wait[0]}"):
                for c in g:
                    c.wait()
            return
        for c in (g if 'nodma' not in DBG else []):
            c.wait()

    def col(ref, j):
        return ref.at[:, pl.ds(j * 128, 128)]

    def split(src, dst, n):
        step = src.shape[0] // n
        return [(src.at[pl.ds(t * step, step), :], dst.at[pl.ds(t * step, step), :]) for t in range(n)]

    cp_x = [group([(x_hbm.at[pl.ds(r0, 256), pl.ds(j * 128, 128)], x_v.at[j, pl.ds(r0, 256), :])
                   for j in range(NT)]) for r0 in range(0, S, 256)]
    cp_wq = group([(col(wqkv_hbm, j), wq_v.at[j]) for j in range(NT)])
    cp_wk = [group(split(col(wqkv_hbm, NT + g), wk_v.at[g], 4)) for g in range(NT)]
    cp_wvo = group([(col(wqkv_hbm, 2 * NT + g), wv_v.at[g]) for g in range(NT)]
                   + [(col(wo_hbm, j), wo_v.at[j]) for j in range(NT)])
    parts = [8, 8] + [2] * (NB - 2)
    cp_q = [group(split(col(q_hbm, i), q_v.at[i], 2)) for i in range(NB)]
    cp_kv = [group(split(col(k_hbm, i), k_v.at[i], parts[i]) + split(col(v_hbm, i), v_v.at[i], parts[i]))
             for i in range(NB)]
    cp_h = [group(split(h_hbm.at[pl.ds(i * CB, CB), :], h_v.at[i], parts[i])) for i in range(NB)]
    cp_tab = group([(tab_hbm, tab_v), (sk_hbm, sk_ref), (d_hbm, d_ref)])
    cp_zero = group([(zero_hbm, zero_ref)])
    cp_ob = [group(split(ob_s.at[i], col(out_hbm, NT + i), 8 if i == NB - 1 else 2)) for i in range(NB)]
    oa_spans = []

    def cp_oa(t):
        r0, n = oa_spans[t]
        pairs = split(oa_s.at[pl.ds(r0, n), :], out_hbm.at[pl.ds(r0, n), pl.ds(0, D)], 8)
        return [pltpu.make_async_copy(src, dst, sems.at[n_sem[0] + t]) for src, dst in pairs]

    rows_done = [0, 0]

    def sync(waits=(), starts=()):
        def run():
            for g in starts:
                start(g)
            done, sent = rows_done
            if done > sent:
                oa_spans.append((sent, done - sent))
                start(cp_oa(len(oa_spans) - 1))
                rows_done[1] = done
            for g in waits:
                wait(g)
        return 0, run

    RP = 64

    def area(name, r0, n=8):
        return pl.ds(AT[name] + r0, n), slice(None)

    def b_prepare(i):
        def widen(p):
            def run():
                w_s[area("k", HALO + p * RP, RP)] = _ld(k_v, i, p * RP, RP).astype(F32)
            return 30, run

        def gate(p):
            def run():
                taps = sk_ref[:, pl.ds(i * CB, CB)].astype(F32)
                if INREG:
                    k = (_ld(k_v, i, p * RP - 16, RP + 16).astype(F32) if p > 0 else
                         _cat([jnp.zeros((16, CB), F32), _ld(k_v, i, 0, RP).astype(F32)], 0))
                    acc = k[16:] * taps[0:1, :]
                    for j in range(1, 4):
                        acc = acc + k[16 - j:16 - j + RP] * taps[j:j + 1, :]
                else:
                    acc = w_s[area("k", HALO + p * RP, RP)] * taps[0:1, :]
                    for j in range(1, 4):
                        acc = acc + w_s[area("k", HALO + p * RP - j, RP)] * taps[j:j + 1, :]
                w_s[area("u", p * RP, RP)] = acc * _ld(v_v, i, p * RP, RP).astype(F32)
            return (130 if INREG else 80), run

        def transpose(p):
            def run():
                ht = h_v[i, :, pl.ds(p * 128, 128)].astype(F32).T
                if p == 0:
                    skip = d_ref[:, pl.ds(i * CB, CB)].astype(F32)
                    lag = jax.lax.broadcasted_iota(jnp.int32, (128, CB), 0)
                    ht = ht + jnp.where(lag == 0, skip, 0.0)
                w_s[area("h", p * 128, 128)] = ht
            return 70, run

        prep = ([sync([cp_kv[0]], cp_x[5:] + [cp_h[1], cp_kv[1]])] if i == 0 else []) + ([] if INREG else [widen(0)])
        for p in range(S // RP):
            prep += ([widen(p + 1)] if p + 1 < S // RP and not INREG else []) + [gate(p)]
        return [transpose(p) for p in range(S // 128)], prep

    def b_forward(i, prep):
        def stage1(h, j, n):
            def run():
                out = _fwd_stage1(n, *[w_s[area("uh"[h], N1 * (n + 8 * m) + 8 * j)] for m in range(4)])
                for r in range(4):
                    for part in range(2):
                        w_s[area("tf", 512 * (8 * h + j) + 16 * (8 * r + n) + 8 * part)] = out[r][part]
            return (46 if n else 32), run

        def stage2(h, j, r):
            def run():
                out = _fwd_stage2([[w_s[area("tf", 512 * (8 * h + j) + 16 * (8 * r + n) + 8 * part)]
                                    for part in range(2)] for n in range(8)])
                for l in range(8):
                    a_s[i % 2, h, r + 4 * l, pl.ds(16 * j, 16), :] = _cat(out[l], 0).astype(BF)
            return 64, run

        tasks = []
        cols = [(h, j) for h in (1, 0) for j in range(N1 // 8)]
        for c, (h, j) in enumerate(cols):
            now = [stage1(h, j, n) for n in range(8)]
            now += [stage2(*cols[c - 1], r) for r in range(4)] if c > 0 else []
            lo = 4 if i == 0 else 0
            if lo <= c < 8:
                share = prep[len(prep) * (c - lo) // (8 - lo):len(prep) * (c + 1 - lo) // (8 - lo)]
                now = _merge(now, share)
            tasks += now
        return tasks + [stage2(*cols[-1], r) for r in range(4)]

    def b_inverse(i):
        def stage1(j, r):
            def run():
                out = _inv_stage1(r, [[w_s[area("b", 128 * (N2 * (i % 2) + r + 4 * l) + 16 * j + 8 * part)]
                                       for part in range(2)] for l in range(8)])
                for n in range(8):
                    for part in range(2):
                        w_s[area("ti", 512 * j + 16 * (4 * n + r) + 8 * part)] = out[n][part]
            return 100, run

        def stage2(jp, n):
            def run():
                ys = [_inv_stage2([[w_s[area("ti", 512 * j + 16 * (4 * n + r) + 8 * part)] for part in range(2)]
                                   for r in range(4)]) for j in (2 * jp, 2 * jp + 1)]
                for m in range(4):
                    r0 = N1 * (n + 8 * m) + 16 * jp
                    y = _cat([ys[0][m], ys[1][m]], 0)
                    ob_s[i, pl.ds(r0, 16), :] = (_ld(q_v, i, r0, 16).astype(F32) * y).astype(BF)
            return 66, run

        tasks = []
        for jp in range(N1 // 16 + 1):
            first = [stage1(j, r) for j in (2 * jp, 2 * jp + 1) for r in range(4)] if jp < N1 // 16 else []
            tasks += _merge(first, [stage2(jp - 1, n) for n in range(8)] if jp > 0 else [])
        return tasks

    def dft_matrix(k2):
        def run():
            f = (tab_v[pl.ds(0, 128), :] * tab_v[pl.ds(256 + k2, 1), :]
                 + tab_v[pl.ds(128, 128), :] * tab_v[pl.ds(256 + N2 + k2, 1), :])
            fwd_v[k2] = f.astype(BF)
            inv_v[k2] = (f.T * (1.0 / S)).astype(BF)
        return 0, run

    def b_middle(i):
        def forward(k2):
            def run():
                rhs = _cat([_ld(a_s, (i % 2, h, k2), 0, 128) for h in range(2)], 1)
                xf = _dot(_ld(fwd_v, k2 + zero(i), 0, 128), rhs)
                ur, ui, hr, hi = xf[:N1, :CB], xf[N1:, :CB], xf[:N1, CB:], xf[N1:, CB:]
                if 'f' in XF and k2 % 2 == 0:
                    urgent(xf[:8, :128])
                yf_s[k2] = _cat([ur * hr - ui * hi, ur * hi + ui * hr], 0).astype(BF)
            return 64, run

        def inverse(k2):
            def run():
                b = _dot(_ld(inv_v, k2 + zero(i), 0, 128), _ld(yf_s, k2, 0, 128))
                if 'i' in XF and k2 % 4 == 0:
                    urgent(b[:8, :])
                w_s[area("b", 128 * (N2 * (i % 2) + k2), 128)] = b
            return 32, run

        tasks = []
        for k4 in range(N2 // 4 + 1):
            if k4 < N2 // 4:
                tasks += [[forward(4 * k4), forward(4 * k4 + 1)], [forward(4 * k4 + 2), forward(4 * k4 + 3)]]
            if k4 > 0:
                tasks += [[inverse(4 * k4 - 4 + r) for r in range(4)]]
        return tasks

    def head_mask():
        r = jax.lax.broadcasted_iota(jnp.int32, (128, 128), 0) // DH
        c = jax.lax.broadcasted_iota(jnp.int32, (128, 128), 1) // DH
        return r == c

    room = {}
    mid_chain = set()

    lead_chain = [None]

    def urgent(value):
        if PRIO:
            c = value if lead_chain[0] is None else lead_chain[0] + value
            for _ in range(PRIO):
                c = pltpu.roll(c, 1, 1) if PKIND == 'roll' else jnp.exp(c)
            lead_chain[0] = c

    def fence(value):
        w_s[pl.ds(pl.multiple_of(zero(0) + AT["fence"], 8), 8), :] = value
        yf_s.bitcast(jnp.uint32)[zero(0) + N2, pl.ds(0, 8), :] = pltpu.bitcast(value, jnp.uint32)

    def chain(n_tiles, n_cols, operands, dot, finish):
        wide = n_cols if WIDE else 1
        deep = 4 // wide
        acc = [None]

        def piece(j0, k0):
            def run():
                d = dot(*operands(range(k0, k0 + deep), range(j0, j0 + wide)))
                acc[0] = d if k0 == 0 else acc[0] + d
                fence(d[:8, :128])
                urgent(d[:8, :128])
                if k0 + deep == n_tiles:
                    for t in range(wide):
                        finish(j0 + t, acc[0][:, 128 * t:128 * t + 128])
            if j0 + k0 > 0:
                mid_chain.add(run)
            if k0 + deep == n_tiles:
                room[run] = ROOM[0]
            return 128, run
        return [piece(j0, k0) for j0 in range(0, n_cols, wide) for k0 in range(0, n_tiles, deep)]

    followers = {}

    def chain_then(operands, dot, part):
        slot = len(followers) % 4

        def park(j, acc):
            w_s[area("acc", 256 * slot + 128 * j, 128)] = acc

        def quarter(t):
            def run():
                part(pl.ds(32 * t, 32), 32 * t, *[w_s[area("acc", 256 * slot + 128 * half + 32 * t, 32)] for half in range(2)])
            room[run] = ROOM[1]
            return 0, run
        pieces = chain(NT, 2, operands, dot, park)
        followers[pieces[-1][1]] = [quarter(t) for t in range(4)]
        return pieces

    def a_transpose_wk(g):
        def tile(j):
            def run():
                wkt_s[g, j] = _ld(wk_v, g, j * 128, 128).astype(F32).T.astype(BF)
            return 0, run
        return [tile(j) for j in range(NT)]

    def a_keys(g, c):
        def operands(ks, js):
            return (_cat([_ld(wkt_s, (g + zero(c), k), 0, 128) for k in ks], 1),
                    _cat([_ld(x_v, k + zero(g), c * 256 + 128 * js[0], 128 * len(js)) for k in ks], 1))

        def part(rows, r0, lo, hi):
            lo, hi = _phi(lo), _phi(hi)
            pkt_s[g, 2 * c, rows, :] = lo.astype(BF)
            pkt_s[g, 2 * c + 1, rows, :] = hi.astype(BF)
            total = lo + hi
            if c < S // 256 - 1:
                z_s[g, c, rows, :] = total
            else:
                for b in range(c):
                    total = total + z_s[g, b, rows, :]
                z = jnp.broadcast_to(jnp.sum(total, axis=1, keepdims=True), (32, 128))
                head = jax.lax.broadcasted_iota(jnp.int32, (32, 128), 1) // DH
                zb_s[g, rows, :] = jnp.where(head == r0 // DH, z, 0.0).astype(BF)
        return chain_then(operands, _dot_nt, part)

    def a_gram(g):
        def block(n):
            def operands(ks, js):
                return (_cat([_ld(pkt_s, (g, k), 0, 128) for k in ks], 1),
                        _cat([_ld(x_v, 2 * n + j + zero(NT + g), 128 * ks[0], 128 * len(ks)) for j in js], 1))

            def finish(j, acc):
                g_s[g, 2 * n + j] = acc.astype(BF)
            return chain(S // 128, 2, operands, _dot, finish)
        return [t for n in range(D // 256) for t in block(n)]

    def a_kv(g):
        acc = [None]

        def piece(kk):
            def run():
                d = _dot(_cat([_ld(g_s, (g, j), 0, 128) for j in range(4 * kk, 4 * kk + 4)], 1),
                         _ld(wv_v, g, kk * 512, 512))
                fence(d[:8, :])
                urgent(d[:8, :])
                if kk == 0:
                    acc[0] = d
                else:
                    kv_s[g] = jnp.where(head_mask(), acc[0] + d, 0.0).astype(BF)
            if kk > 0:
                mid_chain.add(run)
            return 128, run
        return [piece(0), piece(1)]

    def a_mix(g, half):
        def run():
            js = range(4 * half, 4 * half + 4)
            m = _dot(_ld(kv_s, g, 0, 128), _cat([_ld(wo_v, j, g * 128, 128) for j in js], 1))
            for t, j in enumerate(js):
                m_s[j, pl.ds(g * 128, 128), :] = m[:, t * 128:(t + 1) * 128].astype(BF)
        return 128, run

    def a_query(c, n):
        def operands(ks, js):
            return (_cat([_ld(x_v, k + zero(2 * NT + 2 * n + js[0]), c * 128, 128) for k in ks], 1),
                    _cat([_ld(wq_v, 2 * n + j + zero(c), 128 * ks[0], 128 * len(ks)) for j in js], 1))

        def part(rows, r0, lo, hi):
            pq_s[c, 2 * n, rows, :] = _phi(lo).astype(BF)
            pq_s[c, 2 * n + 1, rows, :] = _phi(hi).astype(BF)
        return chain_then(operands, _dot, part)

    def a_normalise(c, half):
        def run():
            for g in range(4 * half, 4 * half + 4):
                pq = _ld(pq_s, (c, g), 0, 128)
                den = _dot(pq, _ld(zb_s, g + zero(c), 0, 128)) + 1e-6
                if 'n' in XF and g % 4 == 0:
                    urgent(den[:8, :])
                inv = pl.reciprocal(den, approx=True)
                inv = inv * (2.0 - den * inv)
                r_s[c, g] = (pq.astype(F32) * inv).astype(BF)
        room[run] = ROOM[2]
        return 128, run

    def a_out(c, n):
        def operands(ks, js):
            return (_cat([_ld(r_s, (c, k), 0, 128) for k in ks], 1),
                    _cat([_ld(m_s, 2 * n + j + zero(c), 128 * ks[0], 128 * len(ks)) for j in js], 1))

        def finish(j, acc):
            oa_s[pl.ds(c * 128, 128), pl.ds(n * 256 + j * 128, 128)] = acc.astype(BF)
            if n == D // 256 - 1 and j == 1:
                rows_done[0] = (c + 1) * 128
        return chain(NT, 2, operands, _dot, finish)

    def starter(*groups):
        def run():
            for g in groups:
                start(g)
        return 0, run

    a_stream, extra = [], []
    n_g = n_c = 0
    for grow in "gcgggcggcggccccc":
        if grow == "g":
            a_stream += [t for c in range(n_c) for t in a_keys(n_g, c)]
            n_g += 1
        else:
            a_stream += [t for g in range(n_g) for t in a_keys(g, n_c)]
            n_c += 1
    extra += [(0, sync([cp_x[0], cp_wk[1]], [cp_wk[2], cp_wk[3]])),
              (4, sync([cp_wk[2], cp_wk[3]], [cp_x[1], cp_wk[4], cp_wk[5]])),
              (16, sync([cp_x[1]], [cp_x[2], cp_h[0], cp_tab])),
              (24, sync([cp_wk[4], cp_wk[5]], [cp_wk[6], cp_wk[7]])),
              (F0_AT, sync([cp_x[2], cp_wk[6], cp_wk[7], cp_tab, cp_h[0]], [cp_x[3], cp_kv[0], cp_x[4]])),
              (96, sync([cp_x[3], cp_x[4]]))]
    extra += [(F0_AT + 2 + 2 * k2, dft_matrix(k2)) for k2 in range(N2)]
    for g, (at, step) in {1: (0, 0.45), 2: (4, 0.45), 3: (8, 0.45), 4: (24, 0.9), 5: (32, 0.9), 6: (50, 2),
                          7: (68, 1.8)}.items():
        extra += [(at + int(step * j), t) for j, t in enumerate(a_transpose_wk(g))]
    for g in range(NT):
        at = len(a_stream)
        if g >= 5:
            for t, gg in enumerate(range(3 * (g - 5), min(3 * (g - 4), NT - 1))):
                extra += [(at + 8 * t + 8, p) for p in a_kv(gg)] + [(at + 8 * t + 16, a_mix(gg, 0)), (at + 8 * t + 16, a_mix(gg, 1))]
        a_stream += a_gram(g)
    a_stream = _spread(a_stream, extra)
    tail = []
    n_c = S // 128
    for c in range(n_c + 1):
        stream = [t for n in range(D // 256) for t in a_query(c, n)] if c < n_c else []
        stream += [t for n in range(D // 256) for t in a_out(c - 1, n)] if c > 0 else []
        at = len(a_stream)
        if c == 0:
            tail += [(at + 4, p) for p in a_kv(NT - 1)] + [(at + 8, a_mix(NT - 1, 0)), (at + 8, a_mix(NT - 1, 1))]
        if c < n_c:
            tail += [(at + 12, a_normalise(c, 0)), (at + 24, a_normalise(c, 1))]
        a_stream += stream
    a_stream = _spread(a_stream, tail)
    spread, pending = [], []
    for item in a_stream:
        spread.append(item)
        if item[0] > 0 and pending:
            spread.append(pending.pop(0))
        pending += followers.get(item[1], [])
    a_stream = spread + pending

    v_regions, m_regions = [], []
    for r in range(NB + 2):
        v = b_inverse(r - 2) if r >= 2 else []
        if r < NB:
            transposes, prep = b_prepare(r)
            v = _merge(v, transposes) + b_forward(r, prep)
        if r == NB + 1:
            v.append(sync(starts=[cp_ob[NB - 1]]))
        v_regions.append(v)
        m_regions.append(b_middle(r - 1) if 1 <= r <= NB and 'nomid' not in DBG else [])
    v_cost = [sum(c for c, _ in v) for v in v_regions]
    m_cost = [sum(c for grp in m for c, _ in grp) for m in m_regions]
    total = sum(c for c, _ in a_stream) + sum(m_cost)
    weight = [c + w for c, w in zip(v_cost, REGION_BIAS)]

    sync([cp_zero], [cp_zero, cp_wk[0], cp_x[0]])[1]()
    w_s[area("k", 0)] = jnp.zeros((HALO, CB), F32)
    for ref in (pkt_s, r_s, g_s, kv_s, pq_s, a_s, z_s, fwd_v, inv_v):
        lead = (zero(0),) + (0,) * (len(ref.shape) - 3)
        ref[(*lead, pl.ds(0, 16), slice(None))] = jnp.zeros((16, CB), ref.dtype)
    sync([cp_wk[0]], [cp_wk[1]])[1]()
    for _, run in a_transpose_wk(0):
        run()

    ai, clock, ob_sent = 0, 0, [0]
    for r in range(NB + 2):
        end = FIRST + (total - FIRST) * sum(weight[1:r + 1]) / sum(weight[1:])
        a_end, t = ai, clock + m_cost[r]
        while a_end < len(a_stream) and (t < end or a_stream[a_end][0] == 0
                                         or a_stream[a_end][1] in mid_chain or r == NB + 1):
            t += a_stream[a_end][0]
            a_end += 1
        length = sum(room.get(run, cost) for cost, run in a_stream[ai:a_end])
        v, m = v_regions[r], m_regions[r]
        lead, trail = 0, (V_TRAIL if r == NB + 1 else 0)
        if r == 0:
            first = [p for p, (cost, _) in enumerate(a_stream) if cost > 0][F0_AT + 2]
            lead = sum(room.get(run, cost) for cost, run in a_stream[:first])
        v_time, acc_cost = [], 0
        for c, _ in v:
            v_time.append(lead + (length - lead - trail) * acc_cost / v_cost[r])
            acc_cost += c

        def region(ai, a_end, length, v, m, v_time):
            now, pa, pm, pv = 0, ai, 0, 0
            while pa < a_end or pm < len(m):
                if pm < len(m) and ((length - M_TRAIL) * pm / len(m) <= now or pa == a_end):
                    todo = m[pm]
                    pm += 1
                else:
                    todo = [a_stream[pa]]
                    pa += 1
                for cost, run in todo:
                    run()
                    now += 0 if len(todo) > 1 else room.get(run, cost)
                while pv < len(v) and v_time[pv] <= now:
                    v[pv][1]()
                    pv += 1
            for _, run in v[pv:]:
                run()
            if lead_chain[0] is not None:
                fence(lead_chain[0])
                lead_chain[0] = None

        if r in BLOCKS:
            nxt = min([b for b in BLOCKS if b > r] + [NB + 2])
            far = min([b for b in BLOCKS if b > nxt] + [NB + 2])

            def needs(lo, hi):
                return ([g for i in range(max(lo, 1), min(hi, NB)) for g in (cp_h[i], cp_kv[i])]
                        + [cp_q[i - 2] for i in range(max(lo, 2), hi)])
            waits, starts = needs(r, nxt), (needs(nxt, far) if r > 0 else [])
            while ob_sent[0] + 3 <= r:
                starts.append(cp_ob[ob_sent[0]])
                ob_sent[0] += 1
            pieces = sum(c > 0 for c, _ in a_stream[:ai])
            if r == 1:
                assert F0_AT + 2 * N2 + 2 < pieces <= 160 and nxt == 2
                waits, starts = waits + cp_x[5:], starts + [cp_wvo]
            if r == 2:
                starts = starts + [cp_wq]
            if r == 3:
                assert pieces <= 256 + 5 * 32 + 8
                waits = waits + [cp_wvo, cp_wq]
            sync(waits, starts)[1]()
            todo_regions = []
        todo_regions.append(functools.partial(region, ai, a_end, length, v, m, v_time))
        if r + 1 in BLOCKS or r == NB + 1:
            with jax.named_scope(f"region{r}"):
                pl.when(zero(r) == 0)(lambda: [run() for run in todo_regions] and None)
        ai, clock = a_end, t

    sync()[1]()
    with jax.named_scope("drain"):
        for g in [cp_oa(t) for t in range(len(oa_spans))] + cp_ob:
            wait(g)


@jax.jit
def pallas_concat_heads__linear_attn_block__ssm_conv_h3__prompt_kernel(
    A_x: jax.Array,
    A_wqkv: jax.Array,
    A_wo: jax.Array,
    B_q: jax.Array,
    B_k: jax.Array,
    B_v: jax.Array,
    B_shift_k: jax.Array,
    B_ssm_k: jax.Array,
    B_ssm_D: jax.Array,
):
    hbm = pl.BlockSpec(memory_space=pl.ANY)
    scratch = [
        pltpu.VMEM((NT, S, 128), BF),
        pltpu.VMEM((NT, D, 128), BF),
        pltpu.VMEM((NT, D, 128), BF),
        pltpu.VMEM((NT, D, 128), BF),
        pltpu.VMEM((NT, D, 128), BF),
        pltpu.VMEM((NB, S, CB), BF),
        pltpu.VMEM((NB, S, CB), BF),
        pltpu.VMEM((NB, S, CB), BF),
        pltpu.VMEM((NB, CB, S), BF),
        pltpu.VMEM(_TABLES.shape, F32),
        pltpu.VMEM((N2, 128, 128), BF),
        pltpu.VMEM((N2, 128, 128), BF),
        pltpu.VMEM((NT, NT, 128, 128), BF),
        pltpu.VMEM((NT, S // 128, 128, 128), BF),
        pltpu.VMEM((NT, NT, 128, 128), BF),
        pltpu.VMEM((NT, 128, 128), BF),
        pltpu.VMEM((NT, D, 128), BF),
        pltpu.VMEM((NT, 128, 128), BF),
        pltpu.VMEM((S // 128, NT, 128, 128), BF),
        pltpu.VMEM((S // 128, NT, 128, 128), BF),
        pltpu.VMEM((S, D), BF),
        pltpu.VMEM((NB, S, CB), BF),
        pltpu.VMEM((2, 2, N2, 128, CB), BF),
        pltpu.VMEM((N2 + 1, 128, CB), BF),
        pltpu.VMEM((NT, S // 256, 128, 128), F32),
        pltpu.VMEM((W_ROWS, 128), F32),
        pltpu.SMEM((NZ,), jnp.int32),
        pltpu.VMEM((4, D), BF),
        pltpu.VMEM((1, D), BF),
        pltpu.SemaphoreType.DMA((64,)),
    ]
    out = pl.pallas_call(
        _kernel,
        out_shape=jax.ShapeDtypeStruct((S, 2 * D), BF),
        in_specs=[hbm] * 11,
        out_specs=hbm,
        scratch_shapes=scratch,
        compiler_params=pltpu.CompilerParams(vmem_limit_bytes=100 * 1024 * 1024),
    )(np.zeros((NZ,), np.int32), A_x.reshape(S, D), A_wqkv, A_wo, B_q.reshape(S, D), B_k.reshape(S, D), B_v.reshape(S, D),
      B_shift_k.T, B_ssm_k, B_ssm_D.reshape(1, D), _TABLES)
    return out.reshape(1, S, 2 * D)
```

```python
import functools

import numpy as np
import jax
import jax.numpy as jnp
import jax.experimental.pallas as pl
import jax.experimental.pallas.tpu as pltpu

S = 2048
D = 1024
DH = 32
N1, N2 = 64, 32
CB = 128
NB = D // CB
NT = D // 128
HALO = 8
_AREAS = (("k", HALO + S), ("u", S), ("h", S), ("tf", 4 * S), ("b", 2 * N2 * 128), ("ti", 2 * S),
          ("acc", 4 * 256), ("taps", 32), ("fence", 8))
AT = {name: sum(n for _, n in _AREAS[:i]) for i, (name, _) in enumerate(_AREAS)}
W_ROWS = sum(n for _, n in _AREAS)
NZ = 32
F0_AT = 48
V_TRAIL, M_TRAIL = 2500, 1200
ROOM = (128, 0, 0)
FIRST = 160 * 128
REGION_BIAS = [0] + [0] * NB + [2500]
DBG = ''
INREG, DYN = False, ''
FLAGS = None
WIDE, BLOCKS = "ko", range(NB + 2)
URGENT_ROWS, URGENT_STEPS, ALL_TILES = (0,), 9, False
BF = jnp.bfloat16
F32 = jnp.float32


def _dft_tables():
    idx = np.arange(N1)
    col = 16 * (idx // 8) + (idx % 8)
    e = np.exp(-2j * np.pi * np.outer(idx, idx) / N1)
    t = np.exp(-2j * np.pi * np.outer(np.arange(N2) + 0.25, idx) / S)
    tab = np.zeros((2 * 128 + 2 * N2, 128), np.float64)
    p, q, tr, ti = tab[:128], tab[128:256], tab[256:256 + N2], tab[256 + N2:]
    p[:N1, col], p[:N1, col + 8], p[N1:, col], p[N1:, col + 8] = e.real, -e.imag, e.imag, e.real
    q[:N1, col], q[:N1, col + 8], q[N1:, col], q[N1:, col + 8] = -e.imag, -e.real, e.real, -e.imag
    tr[:, col], tr[:, col + 8], ti[:, col], ti[:, col + 8] = t.real, t.real, t.imag, t.imag
    return tab.astype(np.float32)


_TABLES = _dft_tables()


def _add(a, b):
    (sa, xa), (sb, xb) = a, b
    if sa == sb:
        return (sa, xa + xb)
    return (1, xa - xb) if sa > 0 else (1, xb - xa)


def _neg(a):
    return (-a[0], a[1])


def _sub(a, b):
    return _add(a, _neg(b))


def _scale(a, c):
    return (1, a[1] * np.float32(a[0] * c))


def _val(a):
    return a[1] if a[0] > 0 else -a[1]


def _cadd(a, b):
    return (_add(a[0], b[0]), _add(a[1], b[1]))


def _csub(a, b):
    return (_sub(a[0], b[0]), _sub(a[1], b[1]))


def _cmul_i(a, s):
    return (_neg(a[1]), a[0]) if s > 0 else (a[1], _neg(a[0]))


def _cmul_const(a, w):
    c, s = float(np.real(w)), float(np.imag(w))
    return (_add(_scale(a[0], c), _scale(a[1], -s)), _add(_scale(a[0], s), _scale(a[1], c)))


def _fft4(x, s):
    a0, a1 = _cadd(x[0], x[2]), _cadd(x[1], x[3])
    b0, b1 = _csub(x[0], x[2]), _cmul_i(_csub(x[1], x[3]), s)
    return [_cadd(a0, a1), _cadd(b0, b1), _csub(a0, a1), _csub(b0, b1)]


def _fft8(x, s):
    r = np.sqrt(0.5)
    a = [_cadd(x[n], x[n + 4]) for n in range(4)]
    b = [_csub(x[n], x[n + 4]) for n in range(4)]
    t = _cadd(b[1], _cmul_i(b[1], s))
    b[1] = (_scale(t[0], r), _scale(t[1], r))
    b[2] = _cmul_i(b[2], s)
    t = _csub(_cmul_i(b[3], s), b[3])
    b[3] = (_scale(t[0], r), _scale(t[1], r))
    ev, od = _fft4(a, s), _fft4(b, s)
    return [ev[0], od[0], ev[1], od[1], ev[2], od[2], ev[3], od[3]]


_C1, _S1, _R2 = np.cos(np.pi / 8), np.sin(np.pi / 8), np.sqrt(0.5)


def _tw(n, j, s):
    return np.exp(s * 2j * np.pi * n * (4 * j + 1) / 128)


def _fwd_stage1(n, u0, u1, u2, u3):
    u0, u1, u2, u3 = (1, u0), (1, u1), (1, u2), (1, u3)
    t = _scale(u2, _R2)
    p, m_ = _add(u0, t), _sub(u0, t)
    c1u1, s1u1, c1u3, s1u3 = _scale(u1, _C1), _scale(u1, _S1), _scale(u3, _C1), _scale(u3, _S1)
    a, b = _add(c1u1, s1u3), _add(s1u1, c1u3)
    d, e = _sub(c1u1, s1u3), _sub(s1u1, c1u3)
    sj = [(_add(p, a), _neg(_add(t, b))), (_sub(m_, e), _sub(t, d)),
          (_sub(p, a), _sub(b, t)), (_add(m_, e), _add(t, d))]
    out = [sj[j] if n == 0 else _cmul_const(sj[j], _tw(n, j, -1)) for j in range(4)]
    return [(_val(re), _val(im)) for re, im in out]


def _fwd_stage2(t):
    out = _fft8([((1, re), (1, im)) for re, im in t], -1)
    return [(_val(re), _val(im)) for re, im in out]


def _inv_stage1(j, b):
    out = _fft8([((1, re), (1, im)) for re, im in b], 1)
    out = [out[n] if n == 0 else _cmul_const(out[n], _tw(n, j, 1)) for n in range(8)]
    return [(_val(re), _val(im)) for re, im in out]


def _inv_stage2(s):
    (x0, y0), (x1, y1), (x2, y2), (x3, y3) = [((1, re), (1, im)) for re, im in s]
    p, a, b = _add(x0, x2), _sub(x0, x2), _sub(y2, y0)
    m_, e, d = _add(x1, x3), _sub(x3, x1), _sub(y3, y1)
    t = _add(_sub(_add(y1, y3), _add(y0, y2)), _sub(p, m_))
    return [_val(_add(p, m_)),
            _val(_add(_scale(_add(a, d), _C1), _scale(_add(b, e), _S1))),
            _val(_scale(t, _R2)),
            _val(_add(_scale(_sub(a, d), _S1), _scale(_sub(b, e), _C1)))]


def _phi(t):
    return jnp.where(t > 0, t + 1.0, jnp.exp(t)) + 1e-6


def _dot(a, b):
    return jnp.dot(a, b, preferred_element_type=F32)


def _dot_nt(a, b):
    return jax.lax.dot_general(a, b, (((1,), (1,)), ((), ())), preferred_element_type=F32)


def _ld(ref, lead, r0, n):
    lead = lead if isinstance(lead, tuple) else (lead,)
    return pltpu.bitcast(ref.bitcast(jnp.uint32)[(*lead, pl.ds(r0 // 2, n // 2), slice(None))], BF)


def _cat(parts, axis):
    return parts[0] if len(parts) == 1 else jnp.concatenate(parts, axis=axis)


def _spread(stream, extra):
    out = []
    extra = sorted(extra, key=lambda e: e[0])
    e = 0
    for pos, item in enumerate(stream):
        while e < len(extra) and extra[e][0] <= pos:
            out.append(extra[e][1])
            e += 1
        out.append(item)
    return out + [t for _, t in extra[e:]]


def _merge(a, b):
    keyed = [((t + 0.5) / len(x), s, item) for s, x in enumerate((a, b)) for t, item in enumerate(x)]
    return [item for _, _, item in sorted(keyed, key=lambda e: e[:2])]


def _kernel(zero_hbm, x_hbm, wqkv_hbm, wo_hbm, q_hbm, k_hbm, v_hbm, sk_hbm, h_hbm, d_hbm, tab_hbm,
            out_hbm,
            x_v, wq_v, wk_v, wv_v, wo_v, q_v, k_v, v_v, h_v, tab_v, fwd_v, inv_v,
            wkt_s, pkt_s, g_s, kv_s, m_s, zb_s, pq_s, r_s, oa_s, ob_s,
            a_s, yf_s, z_s, w_s, zero_ref, sk_ref, d_ref, sems):
    n_sem = [0]
    n_wait = [0]

    def zero(i):
        return zero_ref[i % NZ]

    def group(pairs):
        sem = sems.at[n_sem[0]]
        n_sem[0] += 1
        return [pltpu.make_async_copy(src, dst, sem) for src, dst in pairs]

    def start(g):
        for c in (g if 'nodma' not in DBG else []):
            c.start()

    def wait(g):
        if 'scope' in DBG:
            n_wait[0] += 1
            with jax.named_scope(f"region_w{n_wait[0]}"):
                for c in g:
                    c.wait()
            return
        for c in (g if 'nodma' not in DBG else []):
            c.wait()

    def col(ref, j):
        return ref.at[:, pl.ds(j * 128, 128)]

    def split(src, dst, n):
        step = src.shape[0] // n
        return [(src.at[pl.ds(t * step, step), :], dst.at[pl.ds(t * step, step), :]) for t in range(n)]

    cp_x = [group([(x_hbm.at[pl.ds(r0, 256), pl.ds(j * 128, 128)], x_v.at[j, pl.ds(r0, 256), :])
                   for j in range(NT)]) for r0 in range(0, S, 256)]
    cp_wq = group([(col(wqkv_hbm, j), wq_v.at[j]) for j in range(NT)])
    cp_wk = [group(split(col(wqkv_hbm, NT + g), wk_v.at[g], 4)) for g in range(NT)]
    cp_wvo = group([(col(wqkv_hbm, 2 * NT + g), wv_v.at[g]) for g in range(NT)]
                   + [(col(wo_hbm, j), wo_v.at[j]) for j in range(NT)])
    parts = [8, 8] + [2] * (NB - 2)
    cp_q = [group(split(col(q_hbm, i), q_v.at[i], 2)) for i in range(NB)]
    cp_kv = [group(split(col(k_hbm, i), k_v.at[i], parts[i]) + split(col(v_hbm, i), v_v.at[i], parts[i]))
             for i in range(NB)]
    cp_h = [group(split(h_hbm.at[pl.ds(i * CB, CB), :], h_v.at[i], parts[i])) for i in range(NB)]
    cp_tab = group([(tab_hbm, tab_v), (sk_hbm, sk_ref), (d_hbm, d_ref)])
    cp_zero = group([(zero_hbm, zero_ref)])
    cp_ob = [group(split(ob_s.at[i], col(out_hbm, NT + i), 8 if i == NB - 1 else 2)) for i in range(NB)]
    oa_spans = []

    def cp_oa(t):
        r0, n = oa_spans[t]
        pairs = split(oa_s.at[pl.ds(r0, n), :], out_hbm.at[pl.ds(r0, n), pl.ds(0, D)], 8)
        return [pltpu.make_async_copy(src, dst, sems.at[n_sem[0] + t]) for src, dst in pairs]

    rows_done = [0, 0]

    def sync(waits=(), starts=()):
        def run():
            for g in starts:
                start(g)
            done, sent = rows_done
            if done > sent:
                oa_spans.append((sent, done - sent))
                start(cp_oa(len(oa_spans) - 1))
                rows_done[1] = done
            for g in waits:
                wait(g)
        return 0, run

    RP = 64

    def area(name, r0, n=8):
        return pl.ds(AT[name] + r0, n), slice(None)

    def b_prepare(i):
        def widen(p):
            def run():
                if p == 0 and 't' in DYN:
                    taps = sk_ref[:, pl.ds(i * CB, CB)].astype(F32)
                    for j in range(4):
                        w_s[area("taps", 8 * j)] = jnp.broadcast_to(taps[j:j + 1], (8, CB))
                w_s[area("k", HALO + p * RP, RP)] = _ld(k_v, i, p * RP, RP).astype(F32)
            return 30, run

        def gate(p):
            def run():
                if 't' in DYN:
                    taps = [w_s[area("taps", 8 * j)][:1] for j in range(4)]
                else:
                    taps = sk_ref[:, pl.ds(i * CB, CB)].astype(F32)
                    taps = [taps[j:j + 1] for j in range(4)]
                if INREG:
                    k = (_ld(k_v, i, p * RP - 16, RP + 16).astype(F32) if p > 0 else
                         _cat([jnp.zeros((16, CB), F32), _ld(k_v, i, 0, RP).astype(F32)], 0))
                    acc = k[16:] * taps[0]
                    for j in range(1, 4):
                        acc = acc + k[16 - j:16 - j + RP] * taps[j]
                else:
                    acc = w_s[area("k", HALO + p * RP, RP)] * taps[0]
                    for j in range(1, 4):
                        acc = acc + w_s[area("k", HALO + p * RP - j, RP)] * taps[j]
                w_s[area("u", p * RP, RP)] = acc * _ld(v_v, i, p * RP, RP).astype(F32)
            return (130 if INREG else 80), run

        def transpose(p):
            def run():
                ht = h_v[i, :, pl.ds(p * 128, 128)].astype(F32).T
                if p == 0:
                    skip = d_ref[:, pl.ds(i * CB, CB)].astype(F32)
                    lag = jax.lax.broadcasted_iota(jnp.int32, (128, CB), 0)
                    ht = ht + jnp.where(lag == 0, skip, 0.0)
                w_s[area("h", p * 128, 128)] = ht
            return 70, run

        prep = ([sync([cp_kv[0]], cp_x[5:] + [cp_h[1], cp_kv[1]])] if i == 0 else []) + ([] if INREG else [widen(0)])
        for p in range(S // RP):
            prep += ([widen(p + 1)] if p + 1 < S // RP and not INREG else []) + [gate(p)]
        return [transpose(p) for p in range(S // 128)], prep

    def b_forward(i, prep):
        def stage1(h, j, n):
            def run():
                out = _fwd_stage1(n, *[w_s[area("uh"[h], N1 * (n + 8 * m) + 8 * j)] for m in range(4)])
                for r in range(4):
                    for part in range(2):
                        w_s[area("tf", 512 * (8 * h + j) + 16 * (8 * r + n) + 8 * part)] = out[r][part]
            return (46 if n else 32), run

        def stage2(h, j, r):
            def run():
                out = _fwd_stage2([[w_s[area("tf", 512 * (8 * h + j) + 16 * (8 * r + n) + 8 * part)]
                                    for part in range(2)] for n in range(8)])
                for l in range(8):
                    a_s[i % 2, h, r + 4 * l, pl.ds(16 * j, 16), :] = _cat(out[l], 0).astype(BF)
            return 64, run

        tasks = []
        cols = [(h, j) for h in (1, 0) for j in range(N1 // 8)]
        for c, (h, j) in enumerate(cols):
            now = [stage1(h, j, n) for n in range(8)]
            now += [stage2(*cols[c - 1], r) for r in range(4)] if c > 0 else []
            lo = 4 if i == 0 else 0
            if lo <= c < 8:
                share = prep[len(prep) * (c - lo) // (8 - lo):len(prep) * (c + 1 - lo) // (8 - lo)]
                now = _merge(now, share)
            tasks += now
        return tasks + [stage2(*cols[-1], r) for r in range(4)]

    def b_inverse(i):
        def stage1(j, r):
            def run():
                out = _inv_stage1(r, [[w_s[area("b", 128 * (N2 * (i % 2) + r + 4 * l) + 16 * j + 8 * part)]
                                       for part in range(2)] for l in range(8)])
                for n in range(8):
                    for part in range(2):
                        w_s[area("ti", 512 * j + 16 * (4 * n + r) + 8 * part)] = out[n][part]
            return 100, run

        def stage2(jp, n):
            def run():
                ys = [_inv_stage2([[w_s[area("ti", 512 * j + 16 * (4 * n + r) + 8 * part)] for part in range(2)]
                                   for r in range(4)]) for j in (2 * jp, 2 * jp + 1)]
                for m in range(4):
                    r0 = N1 * (n + 8 * m) + 16 * jp
                    y = _cat([ys[0][m], ys[1][m]], 0)
                    ob_s[i, pl.ds(r0, 16), :] = (_ld(q_v, i, r0, 16).astype(F32) * y).astype(BF)
            return 66, run

        tasks = []
        for jp in range(N1 // 16 + 1):
            first = [stage1(j, r) for j in (2 * jp, 2 * jp + 1) for r in range(4)] if jp < N1 // 16 else []
            tasks += _merge(first, [stage2(jp - 1, n) for n in range(8)] if jp > 0 else [])
        return tasks

    def dft_matrix(k2):
        def run():
            f = (tab_v[pl.ds(0, 128), :] * tab_v[pl.ds(256 + k2, 1), :]
                 + tab_v[pl.ds(128, 128), :] * tab_v[pl.ds(256 + N2 + k2, 1), :])
            fwd_v[k2] = f.astype(BF)
            inv_v[k2] = (f.T * (1.0 / S)).astype(BF)
        return 0, run

    def b_middle(i):
        def forward(k2):
            def run():
                rhs = _cat([_ld(a_s, (i % 2, h, k2), 0, 128) for h in range(2)], 1)
                xf = _dot(_ld(fwd_v, k2 + zero(i), 0, 128), rhs)
                ur, ui, hr, hi = xf[:N1, :CB], xf[N1:, :CB], xf[:N1, CB:], xf[N1:, CB:]
                if k2 % 2 == 0:
                    urgent(xf)
                yf_s[k2] = _cat([ur * hr - ui * hi, ur * hi + ui * hr], 0).astype(BF)
            return 64, run

        def inverse(k2):
            def run():
                b = _dot(_ld(inv_v, k2 + zero(i), 0, 128), _ld(yf_s, k2, 0, 128))
                if k2 % 4 == 0:
                    urgent(b)
                w_s[area("b", 128 * (N2 * (i % 2) + k2), 128)] = b
            return 32, run

        tasks = []
        for k4 in range(N2 // 4 + 1):
            if k4 < N2 // 4:
                tasks += [[forward(4 * k4), forward(4 * k4 + 1)], [forward(4 * k4 + 2), forward(4 * k4 + 3)]]
            if k4 > 0:
                tasks += [[inverse(4 * k4 - 4 + r) for r in range(4)]]
        return tasks

    def head_mask():
        r = jax.lax.broadcasted_iota(jnp.int32, (128, 128), 0) // DH
        c = jax.lax.broadcasted_iota(jnp.int32, (128, 128), 1) // DH
        return r == c

    room = {}
    mid_chain = set()

    lead_chain = [None]

    def urgent(value):
        c = lead_chain[0]
        for r0 in URGENT_ROWS:
            for l0 in range(0, value.shape[1] if ALL_TILES else 128, 128):
                part = value[r0:r0 + 8, l0:l0 + 128]
                c = part if c is None else c + part
        for _ in range(URGENT_STEPS):
            c = jnp.exp(c)
        lead_chain[0] = c

    def fence(value):
        w_s[pl.ds(pl.multiple_of(zero(0) + AT["fence"], 8), 8), :] = value
        yf_s.bitcast(jnp.uint32)[zero(0) + N2, pl.ds(0, 8), :] = pltpu.bitcast(value, jnp.uint32)

    def chain(kind, n_tiles, n_cols, operands, dot, finish):
        wide = n_cols if kind in WIDE else 1
        deep = 4 // wide
        acc = [None]

        def piece(j0, k0):
            def run():
                d = dot(*operands(range(k0, k0 + deep), range(j0, j0 + wide)))
                acc[0] = d if k0 == 0 else acc[0] + d
                fence(d[:8, :128])
                urgent(d)
                if k0 + deep == n_tiles:
                    for t in range(wide):
                        finish(j0 + t, acc[0][:, 128 * t:128 * t + 128])
            if j0 + k0 > 0:
                mid_chain.add(run)
            if k0 + deep == n_tiles:
                room[run] = ROOM[0]
            return 128, run
        return [piece(j0, k0) for j0 in range(0, n_cols, wide) for k0 in range(0, n_tiles, deep)]

    followers = {}

    def chain_then(kind, operands, dot, part):
        slot = len(followers) % 4

        def park(j, acc):
            w_s[area("acc", 256 * slot + 128 * j, 128)] = acc

        def quarter(t):
            def run():
                part(pl.ds(32 * t, 32), 32 * t, *[w_s[area("acc", 256 * slot + 128 * half + 32 * t, 32)] for half in range(2)])
            room[run] = ROOM[1]
            return 0, run
        pieces = chain(kind, NT, 2, operands, dot, park)
        followers[pieces[-1][1]] = [quarter(t) for t in range(4)]
        return pieces

    def a_transpose_wk(g):
        def tile(j):
            def run():
                wkt_s[g, j] = _ld(wk_v, g, j * 128, 128).astype(F32).T.astype(BF)
            return 0, run
        return [tile(j) for j in range(NT)]

    def a_keys(g, c):
        def operands(ks, js):
            return (_cat([_ld(wkt_s, (g + zero(c), k), 0, 128) for k in ks], 1),
                    _cat([_ld(x_v, k + zero(g), c * 256 + 128 * js[0], 128 * len(js)) for k in ks], 1))

        def part(rows, r0, lo, hi):
            lo, hi = _phi(lo), _phi(hi)
            pkt_s[g, 2 * c, rows, :] = lo.astype(BF)
            pkt_s[g, 2 * c + 1, rows, :] = hi.astype(BF)
            total = lo + hi
            if c < S // 256 - 1:
                z_s[g, c, rows, :] = total
            else:
                for b in range(c):
                    total = total + z_s[g, b, rows, :]
                z = jnp.broadcast_to(jnp.sum(total, axis=1, keepdims=True), (32, 128))
                head = jax.lax.broadcasted_iota(jnp.int32, (32, 128), 1) // DH
                zb_s[g, rows, :] = jnp.where(head == r0 // DH, z, 0.0).astype(BF)
        return chain_then("k", operands, _dot_nt, part)

    def a_gram(g):
        def block(n):
            def operands(ks, js):
                return (_cat([_ld(pkt_s, (g + (zero(2 * n + js[0]) if 'p' in DYN else 0), k), 0, 128) for k in ks], 1),
                        _cat([_ld(x_v, 2 * n + j + zero(NT + g), 128 * ks[0], 128 * len(ks)) for j in js], 1))

            def finish(j, acc):
                g_s[g, 2 * n + j] = acc.astype(BF)
            return chain("g", S // 128, 2, operands, _dot, finish)
        return [t for n in range(D // 256) for t in block(n)]

    def a_kv(g):
        acc = [None]

        def piece(kk):
            def run():
                d = _dot(_cat([_ld(g_s, (g, j), 0, 128) for j in range(4 * kk, 4 * kk + 4)], 1),
                         _ld(wv_v, g, kk * 512, 512))
                fence(d[:8, :])
                urgent(d)
                if kk == 0:
                    acc[0] = d
                else:
                    kv_s[g] = jnp.where(head_mask(), acc[0] + d, 0.0).astype(BF)
            if kk > 0:
                mid_chain.add(run)
            return 128, run
        return [piece(0), piece(1)]

    def a_mix(g, half):
        def run():
            js = range(4 * half, 4 * half + 4)
            m = _dot(_ld(kv_s, g, 0, 128), _cat([_ld(wo_v, j, g * 128, 128) for j in js], 1))
            for t, j in enumerate(js):
                m_s[j, pl.ds(g * 128, 128), :] = m[:, t * 128:(t + 1) * 128].astype(BF)
        return 128, run

    def a_query(c, n):
        def operands(ks, js):
            return (_cat([_ld(x_v, k + zero(2 * NT + 2 * n + js[0]), c * 128, 128) for k in ks], 1),
                    _cat([_ld(wq_v, 2 * n + j + zero(c), 128 * ks[0], 128 * len(ks)) for j in js], 1))

        def part(rows, r0, lo, hi):
            pq_s[c, 2 * n, rows, :] = _phi(lo).astype(BF)
            pq_s[c, 2 * n + 1, rows, :] = _phi(hi).astype(BF)
        return chain_then("q", operands, _dot, part)

    def a_normalise(c, half):
        def run():
            for g in range(4 * half, 4 * half + 4):
                pq = _ld(pq_s, (c, g), 0, 128)
                den = _dot(pq, _ld(zb_s, g + zero(c), 0, 128)) + 1e-6
                if g % 4 == 0:
                    urgent(den)
                inv = pl.reciprocal(den, approx=True)
                inv = inv * (2.0 - den * inv)
                r_s[c, g] = (pq.astype(F32) * inv).astype(BF)
        room[run] = ROOM[2]
        return 128, run

    def a_out(c, n):
        def operands(ks, js):
            return (_cat([_ld(r_s, (c + (zero(2 * n + js[0]) if 'r' in DYN else 0), k), 0, 128) for k in ks], 1),
                    _cat([_ld(m_s, 2 * n + j + zero(c), 128 * ks[0], 128 * len(ks)) for j in js], 1))

        def finish(j, acc):
            oa_s[pl.ds(c * 128, 128), pl.ds(n * 256 + j * 128, 128)] = acc.astype(BF)
            if n == D // 256 - 1 and j == 1:
                rows_done[0] = (c + 1) * 128
        return chain("o", NT, 2, operands, _dot, finish)

    def starter(*groups):
        def run():
            for g in groups:
                start(g)
        return 0, run

    a_stream, extra = [], []
    n_g = n_c = 0
    for grow in "gcgggcggcggccccc":
        if grow == "g":
            a_stream += [t for c in range(n_c) for t in a_keys(n_g, c)]
            n_g += 1
        else:
            a_stream += [t for g in range(n_g) for t in a_keys(g, n_c)]
            n_c += 1
    extra += [(0, sync([cp_x[0], cp_wk[1]], [cp_wk[2], cp_wk[3]])),
              (4, sync([cp_wk[2], cp_wk[3]], [cp_x[1], cp_wk[4], cp_wk[5]])),
              (16, sync([cp_x[1]], [cp_x[2], cp_h[0], cp_tab])),
              (24, sync([cp_wk[4], cp_wk[5]], [cp_wk[6], cp_wk[7]])),
              (F0_AT, sync([cp_x[2], cp_wk[6], cp_wk[7], cp_tab, cp_h[0]], [cp_x[3], cp_kv[0], cp_x[4]])),
              (96, sync([cp_x[3], cp_x[4]]))]
    extra += [(F0_AT + 2 + 2 * k2, dft_matrix(k2)) for k2 in range(N2)]
    for g, (at, step) in {1: (0, 0.45), 2: (4, 0.45), 3: (8, 0.45), 4: (24, 0.9), 5: (32, 0.9), 6: (50, 2),
                          7: (68, 1.8)}.items():
        extra += [(at + int(step * j), t) for j, t in enumerate(a_transpose_wk(g))]
    for g in range(NT):
        at = len(a_stream)
        if g >= 5:
            for t, gg in enumerate(range(3 * (g - 5), min(3 * (g - 4), NT - 1))):
                extra += [(at + 8 * t + 8, p) for p in a_kv(gg)] + [(at + 8 * t + 16, a_mix(gg, 0)), (at + 8 * t + 16, a_mix(gg, 1))]
        a_stream += a_gram(g)
    a_stream = _spread(a_stream, extra)
    tail = []
    n_c = S // 128
    for c in range(n_c + 1):
        stream = [t for n in range(D // 256) for t in a_query(c, n)] if c < n_c else []
        stream += [t for n in range(D // 256) for t in a_out(c - 1, n)] if c > 0 else []
        at = len(a_stream)
        if c == 0:
            tail += [(at + 4, p) for p in a_kv(NT - 1)] + [(at + 8, a_mix(NT - 1, 0)), (at + 8, a_mix(NT - 1, 1))]
        if c < n_c:
            tail += [(at + 12, a_normalise(c, 0)), (at + 24, a_normalise(c, 1))]
        a_stream += stream
    a_stream = _spread(a_stream, tail)
    spread, pending = [], []
    for item in a_stream:
        spread.append(item)
        if item[0] > 0 and pending:
            spread.append(pending.pop(0))
        pending += followers.get(item[1], [])
    a_stream = spread + pending

    v_regions, m_regions = [], []
    for r in range(NB + 2):
        v = b_inverse(r - 2) if r >= 2 else []
        if r < NB:
            transposes, prep = b_prepare(r)
            v = _merge(v, transposes) + b_forward(r, prep)
        if r == NB + 1:
            v.append(sync(starts=[cp_ob[NB - 1]]))
        v_regions.append(v)
        m_regions.append(b_middle(r - 1) if 1 <= r <= NB and 'nomid' not in DBG else [])
    v_cost = [sum(c for c, _ in v) for v in v_regions]
    m_cost = [sum(c for grp in m for c, _ in grp) for m in m_regions]
    total = sum(c for c, _ in a_stream) + sum(m_cost)
    weight = [c + w for c, w in zip(v_cost, REGION_BIAS)]

    sync([cp_zero], [cp_zero, cp_wk[0], cp_x[0]])[1]()
    w_s[area("k", 0)] = jnp.zeros((HALO, CB), F32)
    for ref in (pkt_s, r_s, g_s, kv_s, pq_s, a_s, z_s, fwd_v, inv_v):
        lead = (zero(0),) + (0,) * (len(ref.shape) - 3)
        ref[(*lead, pl.ds(0, 16), slice(None))] = jnp.zeros((16, CB), ref.dtype)
    sync([cp_wk[0]], [cp_wk[1]])[1]()
    for _, run in a_transpose_wk(0):
        run()

    ai, clock, ob_sent = 0, 0, [0]
    for r in range(NB + 2):
        end = FIRST + (total - FIRST) * sum(weight[1:r + 1]) / sum(weight[1:])
        a_end, t = ai, clock + m_cost[r]
        while a_end < len(a_stream) and (t < end or a_stream[a_end][0] == 0
                                         or a_stream[a_end][1] in mid_chain or r == NB + 1):
            t += a_stream[a_end][0]
            a_end += 1
        length = sum(room.get(run, cost) for cost, run in a_stream[ai:a_end])
        v, m = v_regions[r], m_regions[r]
        lead, trail = 0, (V_TRAIL if r == NB + 1 else 0)
        if r == 0:
            first = [p for p, (cost, _) in enumerate(a_stream) if cost > 0][F0_AT + 2]
            lead = sum(room.get(run, cost) for cost, run in a_stream[:first])
        v_time, acc_cost = [], 0
        for c, _ in v:
            v_time.append(lead + (length - lead - trail) * acc_cost / v_cost[r])
            acc_cost += c

        def region(ai, a_end, length, v, m, v_time):
            now, pa, pm, pv = 0, ai, 0, 0
            while pa < a_end or pm < len(m):
                if pm < len(m) and ((length - M_TRAIL) * pm / len(m) <= now or pa == a_end):
                    todo = m[pm]
                    pm += 1
                else:
                    todo = [a_stream[pa]]
                    pa += 1
                for cost, run in todo:
                    run()
                    now += 0 if len(todo) > 1 else room.get(run, cost)
                while pv < len(v) and v_time[pv] <= now:
                    v[pv][1]()
                    pv += 1
            for _, run in v[pv:]:
                run()
            if lead_chain[0] is not None:
                fence(lead_chain[0])
                lead_chain[0] = None

        if r in BLOCKS:
            nxt = min([b for b in BLOCKS if b > r] + [NB + 2])
            far = min([b for b in BLOCKS if b > nxt] + [NB + 2])

            def needs(lo, hi):
                return ([g for i in range(max(lo, 1), min(hi, NB)) for g in (cp_h[i], cp_kv[i])]
                        + [cp_q[i - 2] for i in range(max(lo, 2), hi)])
            waits, starts = needs(r, nxt), (needs(nxt, far) if r > 0 else [])
            while ob_sent[0] + 3 <= r:
                starts.append(cp_ob[ob_sent[0]])
                ob_sent[0] += 1
            pieces = sum(c > 0 for c, _ in a_stream[:ai])
            if r == 1:
                assert F0_AT + 2 * N2 + 2 < pieces <= 160 and nxt == 2
                waits, starts = waits + cp_x[5:], starts + [cp_wvo]
            if r == 2:
                starts = starts + [cp_wq]
            if r == 3:
                assert pieces <= 256 + 5 * 32 + 8
                waits = waits + [cp_wvo, cp_wq]
            sync(waits, starts)[1]()
            todo_regions = []
        todo_regions.append(functools.partial(region, ai, a_end, length, v, m, v_time))
        if r + 1 in BLOCKS or r == NB + 1:
            with jax.named_scope(f"region{r}"):
                pl.when(zero(r) == 0)(lambda: [run() for run in todo_regions] and None)
        ai, clock = a_end, t

    sync()[1]()
    with jax.named_scope("drain"):
        for g in [cp_oa(t) for t in range(len(oa_spans))] + cp_ob:
            wait(g)


@jax.jit
def pallas_concat_heads__linear_attn_block__ssm_conv_h3__prompt_kernel(
    A_x: jax.Array,
    A_wqkv: jax.Array,
    A_wo: jax.Array,
    B_q: jax.Array,
    B_k: jax.Array,
    B_v: jax.Array,
    B_shift_k: jax.Array,
    B_ssm_k: jax.Array,
    B_ssm_D: jax.Array,
):
    hbm = pl.BlockSpec(memory_space=pl.ANY)
    scratch = [
        pltpu.VMEM((NT, S, 128), BF),
        pltpu.VMEM((NT, D, 128), BF),
        pltpu.VMEM((NT, D, 128), BF),
        pltpu.VMEM((NT, D, 128), BF),
        pltpu.VMEM((NT, D, 128), BF),
        pltpu.VMEM((NB, S, CB), BF),
        pltpu.VMEM((NB, S, CB), BF),
        pltpu.VMEM((NB, S, CB), BF),
        pltpu.VMEM((NB, CB, S), BF),
        pltpu.VMEM(_TABLES.shape, F32),
        pltpu.VMEM((N2, 128, 128), BF),
        pltpu.VMEM((N2, 128, 128), BF),
        pltpu.VMEM((NT, NT, 128, 128), BF),
        pltpu.VMEM((NT, S // 128, 128, 128), BF),
        pltpu.VMEM((NT, NT, 128, 128), BF),
        pltpu.VMEM((NT, 128, 128), BF),
        pltpu.VMEM((NT, D, 128), BF),
        pltpu.VMEM((NT, 128, 128), BF),
        pltpu.VMEM((S // 128, NT, 128, 128), BF),
        pltpu.VMEM((S // 128, NT, 128, 128), BF),
        pltpu.VMEM((S, D), BF),
        pltpu.VMEM((NB, S, CB), BF),
        pltpu.VMEM((2, 2, N2, 128, CB), BF),
        pltpu.VMEM((N2 + 1, 128, CB), BF),
        pltpu.VMEM((NT, S // 256, 128, 128), F32),
        pltpu.VMEM((W_ROWS, 128), F32),
        pltpu.SMEM((NZ,), jnp.int32),
        pltpu.VMEM((4, D), BF),
        pltpu.VMEM((1, D), BF),
        pltpu.SemaphoreType.DMA((64,)),
    ]
    out = pl.pallas_call(
        _kernel,
        out_shape=jax.ShapeDtypeStruct((S, 2 * D), BF),
        in_specs=[hbm] * 11,
        out_specs=hbm,
        scratch_shapes=scratch,
        compiler_params=pltpu.CompilerParams(vmem_limit_bytes=100 * 1024 * 1024, flags=FLAGS),
    )(np.zeros((NZ,), np.int32), A_x.reshape(S, D), A_wqkv, A_wo, B_q.reshape(S, D), B_k.reshape(S, D), B_v.reshape(S, D),
      B_shift_k.T, B_ssm_k, B_ssm_D.reshape(1, D), _TABLES)
    return out.reshape(1, S, 2 * D)
```

```python
import numpy as np
import jax
import jax.numpy as jnp
import jax.experimental.pallas as pl
import jax.experimental.pallas.tpu as pltpu

S = 2048
D = 1024
DH = 32
N1, N2 = 64, 32
CB = 128
NB = D // CB
NT = D // 128
HALO = 8
_AREAS = (("k", HALO + S), ("u", S), ("h", S), ("tf", 4 * S), ("b", 2 * N2 * 128), ("ti", 2 * S),
          ("acc", 4 * 256), ("fence", 8))
AT = {name: sum(n for _, n in _AREAS[:i]) for i, (name, _) in enumerate(_AREAS)}
W_ROWS = sum(n for _, n in _AREAS)
NZ = 32
F0_AT = 48
V_TRAIL, M_TRAIL = 1500, 1200
ROOM = (128, 0, 0)
FIRST = 150 * 128
REGION_BIAS = [0] * NB + [1500, 1500]
WIDE = "ko"
URGENT_STEPS = 9
BF = jnp.bfloat16
F32 = jnp.float32


def _dft_tables():
    idx = np.arange(N1)
    col = 16 * (idx // 8) + (idx % 8)
    e = np.exp(-2j * np.pi * np.outer(idx, idx) / N1)
    t = np.exp(-2j * np.pi * np.outer(np.arange(N2) + 0.25, idx) / S)
    tab = np.zeros((2 * 128 + 2 * N2, 128), np.float64)
    p, q, tr, ti = tab[:128], tab[128:256], tab[256:256 + N2], tab[256 + N2:]
    p[:N1, col], p[:N1, col + 8], p[N1:, col], p[N1:, col + 8] = e.real, -e.imag, e.imag, e.real
    q[:N1, col], q[:N1, col + 8], q[N1:, col], q[N1:, col + 8] = -e.imag, -e.real, e.real, -e.imag
    tr[:, col], tr[:, col + 8], ti[:, col], ti[:, col + 8] = t.real, t.real, t.imag, t.imag
    return tab.astype(np.float32)


_TABLES = _dft_tables()


def _add(a, b):
    (sa, xa), (sb, xb) = a, b
    if sa == sb:
        return (sa, xa + xb)
    return (1, xa - xb) if sa > 0 else (1, xb - xa)


def _neg(a):
    return (-a[0], a[1])


def _sub(a, b):
    return _add(a, _neg(b))


def _scale(a, c):
    return (1, a[1] * np.float32(a[0] * c))


def _val(a):
    return a[1] if a[0] > 0 else -a[1]


def _cadd(a, b):
    return (_add(a[0], b[0]), _add(a[1], b[1]))


def _csub(a, b):
    return (_sub(a[0], b[0]), _sub(a[1], b[1]))


def _cmul_i(a, s):
    return (_neg(a[1]), a[0]) if s > 0 else (a[1], _neg(a[0]))


def _cmul_const(a, w):
    c, s = float(np.real(w)), float(np.imag(w))
    return (_add(_scale(a[0], c), _scale(a[1], -s)), _add(_scale(a[0], s), _scale(a[1], c)))


def _fft4(x, s):
    a0, a1 = _cadd(x[0], x[2]), _cadd(x[1], x[3])
    b0, b1 = _csub(x[0], x[2]), _cmul_i(_csub(x[1], x[3]), s)
    return [_cadd(a0, a1), _cadd(b0, b1), _csub(a0, a1), _csub(b0, b1)]


def _fft8(x, s):
    r = np.sqrt(0.5)
    a = [_cadd(x[n], x[n + 4]) for n in range(4)]
    b = [_csub(x[n], x[n + 4]) for n in range(4)]
    t = _cadd(b[1], _cmul_i(b[1], s))
    b[1] = (_scale(t[0], r), _scale(t[1], r))
    b[2] = _cmul_i(b[2], s)
    t = _csub(_cmul_i(b[3], s), b[3])
    b[3] = (_scale(t[0], r), _scale(t[1], r))
    ev, od = _fft4(a, s), _fft4(b, s)
    return [ev[0], od[0], ev[1], od[1], ev[2], od[2], ev[3], od[3]]


_C1, _S1, _R2 = np.cos(np.pi / 8), np.sin(np.pi / 8), np.sqrt(0.5)


def _tw(n, j, s):
    return np.exp(s * 2j * np.pi * n * (4 * j + 1) / 128)


def _fwd_stage1(n, u0, u1, u2, u3):
    u0, u1, u2, u3 = (1, u0), (1, u1), (1, u2), (1, u3)
    t = _scale(u2, _R2)
    p, m_ = _add(u0, t), _sub(u0, t)
    c1u1, s1u1, c1u3, s1u3 = _scale(u1, _C1), _scale(u1, _S1), _scale(u3, _C1), _scale(u3, _S1)
    a, b = _add(c1u1, s1u3), _add(s1u1, c1u3)
    d, e = _sub(c1u1, s1u3), _sub(s1u1, c1u3)
    sj = [(_add(p, a), _neg(_add(t, b))), (_sub(m_, e), _sub(t, d)),
          (_sub(p, a), _sub(b, t)), (_add(m_, e), _add(t, d))]
    out = [sj[j] if n == 0 else _cmul_const(sj[j], _tw(n, j, -1)) for j in range(4)]
    return [(_val(re), _val(im)) for re, im in out]


def _fwd_stage2(t):
    out = _fft8([((1, re), (1, im)) for re, im in t], -1)
    return [(_val(re), _val(im)) for re, im in out]


def _inv_stage1(j, b):
    out = _fft8([((1, re), (1, im)) for re, im in b], 1)
    out = [out[n] if n == 0 else _cmul_const(out[n], _tw(n, j, 1)) for n in range(8)]
    return [(_val(re), _val(im)) for re, im in out]


def _inv_stage2(s):
    (x0, y0), (x1, y1), (x2, y2), (x3, y3) = [((1, re), (1, im)) for re, im in s]
    p, a, b = _add(x0, x2), _sub(x0, x2), _sub(y2, y0)
    m_, e, d = _add(x1, x3), _sub(x3, x1), _sub(y3, y1)
    t = _add(_sub(_add(y1, y3), _add(y0, y2)), _sub(p, m_))
    return [_val(_add(p, m_)),
            _val(_add(_scale(_add(a, d), _C1), _scale(_add(b, e), _S1))),
            _val(_scale(t, _R2)),
            _val(_add(_scale(_sub(a, d), _S1), _scale(_sub(b, e), _C1)))]


def _phi(t):
    return jnp.where(t > 0, t + 1.0, jnp.exp(t)) + 1e-6


def _dot(a, b):
    return jnp.dot(a, b, preferred_element_type=F32)


def _dot_nt(a, b):
    return jax.lax.dot_general(a, b, (((1,), (1,)), ((), ())), preferred_element_type=F32)


def _ld(ref, lead, r0, n):
    lead = lead if isinstance(lead, tuple) else (lead,)
    return pltpu.bitcast(ref.bitcast(jnp.uint32)[(*lead, pl.ds(r0 // 2, n // 2), slice(None))], BF)


def _cat(parts, axis):
    return parts[0] if len(parts) == 1 else jnp.concatenate(parts, axis=axis)


def _spread(stream, extra):
    out = []
    extra = sorted(extra, key=lambda e: e[0])
    e = 0
    for pos, item in enumerate(stream):
        while e < len(extra) and extra[e][0] <= pos:
            out.append(extra[e][1])
            e += 1
        out.append(item)
    return out + [t for _, t in extra[e:]]


def _merge(a, b):
    keyed = [((t + 0.5) / len(x), s, item) for s, x in enumerate((a, b)) for t, item in enumerate(x)]
    return [item for _, _, item in sorted(keyed, key=lambda e: e[:2])]


def _kernel(zero_hbm, x_hbm, wqkv_hbm, wo_hbm, q_hbm, k_hbm, v_hbm, sk_hbm, h_hbm, d_hbm, tab_hbm,
            out_hbm,
            x_v, wq_v, wk_v, wv_v, wo_v, q_v, k_v, v_v, h_v, tab_v, fwd_v, inv_v,
            wkt_s, pkt_s, g_s, kv_s, m_s, zb_s, pq_s, r_s, oa_s, ob_s,
            a_s, yf_s, z_s, w_s, zero_ref, sk_ref, d_ref, skip_s, sems):
    n_sem = [0]

    def zero(i):
        return zero_ref[i % NZ]

    def group(pairs):
        sem = sems.at[n_sem[0]]
        n_sem[0] += 1
        return [pltpu.make_async_copy(src, dst, sem) for src, dst in pairs]

    def start(g):
        for c in g:
            c.start()

    def wait(g):
        for c in g:
            c.wait()

    def col(ref, j):
        return ref.at[:, pl.ds(j * 128, 128)]

    def split(src, dst, n):
        step = src.shape[0] // n
        return [(src.at[pl.ds(t * step, step), :], dst.at[pl.ds(t * step, step), :]) for t in range(n)]

    cp_x = [group([(x_hbm.at[pl.ds(r0, 256), pl.ds(j * 128, 128)], x_v.at[j, pl.ds(r0, 256), :])
                   for j in range(NT)]) for r0 in range(0, S, 256)]
    cp_wq = group([(col(wqkv_hbm, j), wq_v.at[j]) for j in range(NT)])
    cp_wk = [group(split(col(wqkv_hbm, NT + g), wk_v.at[g], 4)) for g in range(NT)]
    cp_wvo = group([(col(wqkv_hbm, 2 * NT + g), wv_v.at[g]) for g in range(NT)]
                   + [(col(wo_hbm, j), wo_v.at[j]) for j in range(NT)])
    parts = [8, 8] + [2] * (NB - 2)
    cp_q = [group(split(col(q_hbm, i), q_v.at[i], 2)) for i in range(NB)]
    cp_kv = [group(split(col(k_hbm, i), k_v.at[i], parts[i]) + split(col(v_hbm, i), v_v.at[i], parts[i]))
             for i in range(NB)]
    cp_h = [group(split(h_hbm.at[pl.ds(i * CB, CB), :], h_v.at[i], parts[i])) for i in range(NB)]
    cp_tab = group([(tab_hbm, tab_v), (sk_hbm, sk_ref), (d_hbm, d_ref)])
    cp_zero = group([(zero_hbm, zero_ref)])
    cp_ob = [group(split(ob_s.at[i], col(out_hbm, NT + i), 8 if i == NB - 1 else 2)) for i in range(NB)]
    oa_spans = []

    def cp_oa(t):
        r0, n = oa_spans[t]
        pairs = split(oa_s.at[pl.ds(r0, n), :], out_hbm.at[pl.ds(r0, n), pl.ds(0, D)], 8)
        return [pltpu.make_async_copy(src, dst, sems.at[n_sem[0] + t]) for src, dst in pairs]

    rows_done = [0, 0]

    def sync(waits=(), starts=()):
        def run():
            for g in starts:
                start(g)
            done, sent = rows_done
            if done > sent:
                oa_spans.append((sent, done - sent))
                start(cp_oa(len(oa_spans) - 1))
                rows_done[1] = done
            for g in waits:
                wait(g)
        return 0, run

    RP = 64

    def area(name, r0, n=8):
        return pl.ds(AT[name] + r0, n), slice(None)

    def b_prepare(i):
        def widen(p):
            def run():
                w_s[area("k", HALO + p * RP, RP)] = _ld(k_v, i, p * RP, RP).astype(F32)
            return 30, run

        def gate(p):
            def run():
                taps = sk_ref[:, pl.ds(i * CB, CB)].astype(F32)
                acc = w_s[area("k", HALO + p * RP, RP)] * taps[0:1]
                for j in range(1, 4):
                    acc = acc + w_s[area("k", HALO + p * RP - j, RP)] * taps[j:j + 1]
                w_s[area("u", p * RP, RP)] = acc * _ld(v_v, i, p * RP, RP).astype(F32)
            return 80, run

        def transpose(p):
            def run():
                ht = h_v[i, :, pl.ds(p * 128, 128)].astype(F32).T
                if p == 0:
                    if i == 0:
                        skip_s[...] = d_ref[...].astype(F32).reshape(1, D)
                    skip = skip_s[:, pl.ds(i * CB, CB)]
                    lag = jax.lax.broadcasted_iota(jnp.int32, (128, CB), 0)
                    ht = ht + jnp.where(lag == 0, skip, 0.0)
                w_s[area("h", p * 128, 128)] = ht
            return 70, run

        prep = ([sync([cp_kv[0]], cp_x[5:] + [cp_h[1], cp_kv[1]])] if i == 0 else []) + [widen(0)]
        for p in range(S // RP):
            prep += ([widen(p + 1)] if p + 1 < S // RP else []) + [gate(p)]
        return [transpose(p) for p in range(S // 128)], prep

    def b_forward(i, prep):
        def stage1(h, j, n):
            def run():
                out = _fwd_stage1(n, *[w_s[area("uh"[h], N1 * (n + 8 * m) + 8 * j)] for m in range(4)])
                for r in range(4):
                    for part in range(2):
                        w_s[area("tf", 512 * (8 * h + j) + 16 * (8 * r + n) + 8 * part)] = out[r][part]
            return (46 if n else 32), run

        def stage2(h, j, r):
            def run():
                out = _fwd_stage2([[w_s[area("tf", 512 * (8 * h + j) + 16 * (8 * r + n) + 8 * part)]
                                    for part in range(2)] for n in range(8)])
                for l in range(8):
                    a_s[i % 2, h, r + 4 * l, pl.ds(16 * j, 16), :] = _cat(out[l], 0).astype(BF)
            return 64, run

        tasks = []
        cols = [(h, j) for h in (1, 0) for j in range(N1 // 8)]
        for c, (h, j) in enumerate(cols):
            now = [stage1(h, j, n) for n in range(8)]
            now += [stage2(*cols[c - 1], r) for r in range(4)] if c > 0 else []
            lo = 4 if i == 0 else 0
            if lo <= c < 8:
                share = prep[len(prep) * (c - lo) // (8 - lo):len(prep) * (c + 1 - lo) // (8 - lo)]
                now = _merge(now, share)
            tasks += now
        return tasks + [stage2(*cols[-1], r) for r in range(4)]

    def b_inverse(i):
        def stage1(j, r):
            def run():
                out = _inv_stage1(r, [[w_s[area("b", 128 * (N2 * (i % 2) + r + 4 * l) + 16 * j + 8 * part)]
                                       for part in range(2)] for l in range(8)])
                for n in range(8):
                    for part in range(2):
                        w_s[area("ti", 512 * j + 16 * (4 * n + r) + 8 * part)] = out[n][part]
            return 100, run

        def stage2(jp, n):
            def run():
                ys = [_inv_stage2([[w_s[area("ti", 512 * j + 16 * (4 * n + r) + 8 * part)] for part in range(2)]
                                   for r in range(4)]) for j in (2 * jp, 2 * jp + 1)]
                for m in range(4):
                    r0 = N1 * (n + 8 * m) + 16 * jp
                    y = _cat([ys[0][m], ys[1][m]], 0)
                    ob_s[i, pl.ds(r0, 16), :] = (_ld(q_v, i, r0, 16).astype(F32) * y).astype(BF)
            return 66, run

        tasks = []
        for jp in range(N1 // 16 + 1):
            first = [stage1(j, r) for j in (2 * jp, 2 * jp + 1) for r in range(4)] if jp < N1 // 16 else []
            tasks += _merge(first, [stage2(jp - 1, n) for n in range(8)] if jp > 0 else [])
        return tasks

    def dft_matrix(k2):
        def run():
            f = (tab_v[pl.ds(0, 128), :] * tab_v[pl.ds(256 + k2, 1), :]
                 + tab_v[pl.ds(128, 128), :] * tab_v[pl.ds(256 + N2 + k2, 1), :])
            fwd_v[k2] = f.astype(BF)
            inv_v[k2] = (f.T * (1.0 / S)).astype(BF)
        return 0, run

    def b_middle(i):
        def forward(k2):
            def run():
                rhs = _cat([_ld(a_s, (i % 2, h, k2), 0, 128) for h in range(2)], 1)
                xf = _dot(_ld(fwd_v, k2 + zero(i), 0, 128), rhs)
                ur, ui, hr, hi = xf[:N1, :CB], xf[N1:, :CB], xf[:N1, CB:], xf[N1:, CB:]
                if k2 % 2 == 0:
                    urgent(xf)
                yf_s[k2] = _cat([ur * hr - ui * hi, ur * hi + ui * hr], 0).astype(BF)
            return 64, run

        def inverse(k2):
            def run():
                b = _dot(_ld(inv_v, k2 + zero(i), 0, 128), _ld(yf_s, k2, 0, 128))
                if k2 % 4 == 0:
                    urgent(b)
                w_s[area("b", 128 * (N2 * (i % 2) + k2), 128)] = b
            return 32, run

        tasks = []
        for k4 in range(N2 // 4 + 1):
            if k4 < N2 // 4:
                tasks += [[forward(4 * k4), forward(4 * k4 + 1)], [forward(4 * k4 + 2), forward(4 * k4 + 3)]]
            if k4 > 0:
                tasks += [[inverse(4 * k4 - 4 + r) for r in range(4)]]
        return tasks

    def head_mask():
        r = jax.lax.broadcasted_iota(jnp.int32, (128, 128), 0) // DH
        c = jax.lax.broadcasted_iota(jnp.int32, (128, 128), 1) // DH
        return r == c

    room = {}
    mid_chain = set()

    lead_chain = [None]

    def urgent(value):
        c = value[:8, :128] if lead_chain[0] is None else lead_chain[0] + value[:8, :128]
        for _ in range(URGENT_STEPS):
            c = jnp.exp(c)
        lead_chain[0] = c

    def fence(value):
        w_s[pl.ds(pl.multiple_of(zero(0) + AT["fence"], 8), 8), :] = value
        yf_s.bitcast(jnp.uint32)[zero(0) + N2, pl.ds(0, 8), :] = pltpu.bitcast(value, jnp.uint32)

    def chain(kind, n_tiles, n_cols, operands, dot, finish):
        wide = n_cols if kind in WIDE else 1
        deep = 4 // wide
        acc = [None]

        def piece(j0, k0):
            def run():
                d = dot(*operands(range(k0, k0 + deep), range(j0, j0 + wide)))
                acc[0] = d if k0 == 0 else acc[0] + d
                fence(d[:8, :128])
                urgent(d)
                if k0 + deep == n_tiles:
                    for t in range(wide):
                        finish(j0 + t, acc[0][:, 128 * t:128 * t + 128])
            if j0 + k0 > 0:
                mid_chain.add(run)
            if k0 + deep == n_tiles:
                room[run] = ROOM[0]
            return 128, run
        return [piece(j0, k0) for j0 in range(0, n_cols, wide) for k0 in range(0, n_tiles, deep)]

    followers = {}

    def chain_then(kind, operands, dot, part):
        slot = len(followers) % 4

        def park(j, acc):
            w_s[area("acc", 256 * slot + 128 * j, 128)] = acc

        def quarter(t):
            def run():
                part(pl.ds(32 * t, 32), 32 * t, *[w_s[area("acc", 256 * slot + 128 * half + 32 * t, 32)] for half in range(2)])
            room[run] = ROOM[1]
            return 0, run
        pieces = chain(kind, NT, 2, operands, dot, park)
        followers[pieces[-1][1]] = [quarter(t) for t in range(4)]
        return pieces

    def a_transpose_wk(g):
        def tile(j):
            def run():
                wkt_s[g, j] = _ld(wk_v, g, j * 128, 128).astype(F32).T.astype(BF)
            return 0, run
        return [tile(j) for j in range(NT)]

    def a_keys(g, c):
        def operands(ks, js):
            return (_cat([_ld(wkt_s, (g + zero(c), k), 0, 128) for k in ks], 1),
                    _cat([_ld(x_v, k + zero(g), c * 256 + 128 * js[0], 128 * len(js)) for k in ks], 1))

        def part(rows, r0, lo, hi):
            lo, hi = _phi(lo), _phi(hi)
            pkt_s[g, 2 * c, rows, :] = lo.astype(BF)
            pkt_s[g, 2 * c + 1, rows, :] = hi.astype(BF)
            total = lo + hi
            if c < S // 256 - 1:
                z_s[g, c, rows, :] = total
            else:
                for b in range(c):
                    total = total + z_s[g, b, rows, :]
                z = jnp.broadcast_to(jnp.sum(total, axis=1, keepdims=True), (32, 128))
                head = jax.lax.broadcasted_iota(jnp.int32, (32, 128), 1) // DH
                zb_s[g, rows, :] = jnp.where(head == r0 // DH, z, 0.0).astype(BF)
        return chain_then("k", operands, _dot_nt, part)

    def a_gram(g):
        def block(n):
            def operands(ks, js):
                return (_cat([_ld(pkt_s, (g, k), 0, 128) for k in ks], 1),
                        _cat([_ld(x_v, 2 * n + j + zero(NT + g), 128 * ks[0], 128 * len(ks)) for j in js], 1))

            def finish(j, acc):
                g_s[g, 2 * n + j] = acc.astype(BF)
            return chain("g", S // 128, 2, operands, _dot, finish)
        return [t for n in range(D // 256) for t in block(n)]

    def a_kv(g):
        acc = [None]

        def piece(kk):
            def run():
                d = _dot(_cat([_ld(g_s, (g, j), 0, 128) for j in range(4 * kk, 4 * kk + 4)], 1),
                         _ld(wv_v, g, kk * 512, 512))
                fence(d[:8, :])
                urgent(d)
                if kk == 0:
                    acc[0] = d
                else:
                    kv_s[g] = jnp.where(head_mask(), acc[0] + d, 0.0).astype(BF)
            if kk > 0:
                mid_chain.add(run)
            return 128, run
        return [piece(0), piece(1)]

    def a_mix(g, half):
        def run():
            js = range(4 * half, 4 * half + 4)
            m = _dot(_ld(kv_s, g, 0, 128), _cat([_ld(wo_v, j, g * 128, 128) for j in js], 1))
            for t, j in enumerate(js):
                m_s[j, pl.ds(g * 128, 128), :] = m[:, t * 128:(t + 1) * 128].astype(BF)
        return 128, run

    def a_query(c, n):
        def operands(ks, js):
            return (_cat([_ld(x_v, k + zero(2 * NT + 2 * n + js[0]), c * 128, 128) for k in ks], 1),
                    _cat([_ld(wq_v, 2 * n + j + zero(c), 128 * ks[0], 128 * len(ks)) for j in js], 1))

        def part(rows, r0, lo, hi):
            pq_s[c, 2 * n, rows, :] = _phi(lo).astype(BF)
            pq_s[c, 2 * n + 1, rows, :] = _phi(hi).astype(BF)
        return chain_then("q", operands, _dot, part)

    def a_normalise(c, half):
        def run():
            for g in range(4 * half, 4 * half + 4):
                pq = _ld(pq_s, (c, g), 0, 128)
                den = _dot(pq, _ld(zb_s, g + zero(c), 0, 128)) + 1e-6
                if g % 4 == 0:
                    urgent(den)
                inv = pl.reciprocal(den, approx=True)
                inv = inv * (2.0 - den * inv)
                r_s[c, g] = (pq.astype(F32) * inv).astype(BF)
        room[run] = ROOM[2]
        return 128, run

    def a_out(c, n):
        def operands(ks, js):
            return (_cat([_ld(r_s, (c, k), 0, 128) for k in ks], 1),
                    _cat([_ld(m_s, 2 * n + j + zero(c), 128 * ks[0], 128 * len(ks)) for j in js], 1))

        def finish(j, acc):
            oa_s[pl.ds(c * 128, 128), pl.ds(n * 256 + j * 128, 128)] = acc.astype(BF)
            if n == D // 256 - 1 and j == 1:
                rows_done[0] = (c + 1) * 128
        return chain("o", NT, 2, operands, _dot, finish)

    def starter(*groups):
        def run():
            for g in groups:
                start(g)
        return 0, run

    a_stream, extra = [], []
    n_g = n_c = 0
    for grow in "gcgggcggcggccccc":
        if grow == "g":
            a_stream += [t for c in range(n_c) for t in a_keys(n_g, c)]
            n_g += 1
        else:
            a_stream += [t for g in range(n_g) for t in a_keys(g, n_c)]
            n_c += 1
    extra += [(0, sync([cp_x[0], cp_wk[1]], [cp_wk[2], cp_wk[3]])),
              (4, sync([cp_wk[2], cp_wk[3]], [cp_x[1], cp_wk[4], cp_wk[5]])),
              (16, sync([cp_x[1]], [cp_x[2], cp_h[0], cp_tab])),
              (24, sync([cp_wk[4], cp_wk[5]], [cp_wk[6], cp_wk[7]])),
              (F0_AT, sync([cp_x[2], cp_wk[6], cp_wk[7], cp_tab, cp_h[0]], [cp_x[3], cp_kv[0], cp_x[4]])),
              (96, sync([cp_x[3], cp_x[4]]))]
    extra += [(F0_AT + 2 + 2 * k2, dft_matrix(k2)) for k2 in range(N2)]
    for g, (at, step) in {1: (0, 0.45), 2: (4, 0.45), 3: (8, 0.45), 4: (24, 0.9), 5: (32, 0.9), 6: (50, 2),
                          7: (68, 1.8)}.items():
        extra += [(at + int(step * j), t) for j, t in enumerate(a_transpose_wk(g))]
    for g in range(NT):
        at = len(a_stream)
        if g >= 5:
            for t, gg in enumerate(range(3 * (g - 5), min(3 * (g - 4), NT - 1))):
                extra += [(at + 8 * t + 8, p) for p in a_kv(gg)] + [(at + 8 * t + 16, a_mix(gg, 0)), (at + 8 * t + 16, a_mix(gg, 1))]
        a_stream += a_gram(g)
    a_stream = _spread(a_stream, extra)
    tail = []
    n_c = S // 128
    for c in range(n_c + 1):
        stream = [t for n in range(D // 256) for t in a_query(c, n)] if c < n_c else []
        stream += [t for n in range(D // 256) for t in a_out(c - 1, n)] if c > 0 else []
        at = len(a_stream)
        if c == 0:
            tail += [(at + 4, p) for p in a_kv(NT - 1)] + [(at + 8, a_mix(NT - 1, 0)), (at + 8, a_mix(NT - 1, 1))]
        if c < n_c:
            tail += [(at + 12, a_normalise(c, 0)), (at + 24, a_normalise(c, 1))]
        a_stream += stream
    a_stream = _spread(a_stream, tail)
    spread, pending = [], []
    for item in a_stream:
        spread.append(item)
        if item[0] > 0 and pending:
            spread.append(pending.pop(0))
        pending += followers.get(item[1], [])
    a_stream = spread + pending

    v_regions, m_regions = [], []
    for r in range(NB + 2):
        v = b_inverse(r - 2) if r >= 2 else []
        if r < NB:
            transposes, prep = b_prepare(r)
            v = _merge(v, transposes) + b_forward(r, prep)
        if r == NB + 1:
            v.append(sync(starts=[cp_ob[NB - 1]]))
        v_regions.append(v)
        m_regions.append(b_middle(r - 1) if 1 <= r <= NB else [])
    v_cost = [sum(c for c, _ in v) for v in v_regions]
    m_cost = [sum(c for grp in m for c, _ in grp) for m in m_regions]
    total = sum(c for c, _ in a_stream) + sum(m_cost)
    weight = [c + w for c, w in zip(v_cost, REGION_BIAS)]

    sync([cp_zero], [cp_zero, cp_wk[0], cp_x[0]])[1]()
    w_s[area("k", 0)] = jnp.zeros((HALO, CB), F32)
    for ref in (pkt_s, r_s, g_s, kv_s, pq_s, a_s, z_s, fwd_v, inv_v):
        lead = (zero(0),) + (0,) * (len(ref.shape) - 3)
        ref[(*lead, pl.ds(0, 16), slice(None))] = jnp.zeros((16, CB), ref.dtype)
    sync([cp_wk[0]], [cp_wk[1]])[1]()
    for _, run in a_transpose_wk(0):
        run()

    ai, clock = 0, 0
    for r in range(NB + 2):
        end = FIRST + (total - FIRST) * sum(weight[1:r + 1]) / sum(weight[1:])
        a_end, t = ai, clock + m_cost[r]
        while a_end < len(a_stream) and (t < end or a_stream[a_end][0] == 0
                                         or a_stream[a_end][1] in mid_chain or r == NB + 1):
            t += a_stream[a_end][0]
            a_end += 1
        length = sum(room.get(run, cost) for cost, run in a_stream[ai:a_end])
        v, m = v_regions[r], m_regions[r]
        lead, trail = 0, (V_TRAIL if r == NB + 1 else 0)
        if r == 0:
            first = [p for p, (cost, _) in enumerate(a_stream) if cost > 0][F0_AT + 2]
            lead = sum(room.get(run, cost) for cost, run in a_stream[:first])
        v_time, acc_cost = [], 0
        for c, _ in v:
            v_time.append(lead + (length - lead - trail) * acc_cost / v_cost[r])
            acc_cost += c

        def region():
            now, pa, pm, pv = 0, ai, 0, 0
            while pa < a_end or pm < len(m):
                if pm < len(m) and ((length - M_TRAIL) * pm / len(m) <= now or pa == a_end):
                    todo = m[pm]
                    pm += 1
                else:
                    todo = [a_stream[pa]]
                    pa += 1
                for cost, run in todo:
                    run()
                    now += 0 if len(todo) > 1 else room.get(run, cost)
                while pv < len(v) and v_time[pv] <= now:
                    v[pv][1]()
                    pv += 1
            for _, run in v[pv:]:
                run()
            if lead_chain[0] is not None:
                fence(lead_chain[0])
                lead_chain[0] = None

        waits = ([cp_h[r], cp_kv[r]] if 1 <= r < NB else []) + ([cp_q[r - 2]] if r >= 2 else [])
        starts = (([cp_h[r + 1], cp_kv[r + 1]] if 1 <= r < NB - 1 else []) + ([cp_q[r - 1]] if 1 <= r <= NB else [])
                  + ([cp_ob[r - 3]] if r >= 3 else []))
        pieces = sum(c > 0 for c, _ in a_stream[:ai])
        if r == 1:
            assert F0_AT + 2 * N2 + 2 < pieces <= 160
            waits, starts = waits + cp_x[5:], starts + [cp_wvo]
        if r == 2:
            starts = starts + [cp_wq]
        if r == 3:
            assert pieces <= 256 + 5 * 32 + 8
            waits = waits + [cp_wvo, cp_wq]
        sync(waits, starts)[1]()
        pl.when(zero(r) == 0)(region)
        ai, clock = a_end, t

    sync()[1]()
    assert rows_done == [S, S] and n_sem[0] + len(oa_spans) <= sems.shape[0]
    for g in [cp_oa(t) for t in range(len(oa_spans))] + cp_ob:
        wait(g)


@jax.jit
def pallas_concat_heads__linear_attn_block__ssm_conv_h3__prompt_kernel(
    A_x: jax.Array,
    A_wqkv: jax.Array,
    A_wo: jax.Array,
    B_q: jax.Array,
    B_k: jax.Array,
    B_v: jax.Array,
    B_shift_k: jax.Array,
    B_ssm_k: jax.Array,
    B_ssm_D: jax.Array,
):
    hbm = pl.BlockSpec(memory_space=pl.ANY)
    scratch = [
        pltpu.VMEM((NT, S, 128), BF),
        pltpu.VMEM((NT, D, 128), BF),
        pltpu.VMEM((NT, D, 128), BF),
        pltpu.VMEM((NT, D, 128), BF),
        pltpu.VMEM((NT, D, 128), BF),
        pltpu.VMEM((NB, S, CB), BF),
        pltpu.VMEM((NB, S, CB), BF),
        pltpu.VMEM((NB, S, CB), BF),
        pltpu.VMEM((NB, CB, S), BF),
        pltpu.VMEM(_TABLES.shape, F32),
        pltpu.VMEM((N2, 128, 128), BF),
        pltpu.VMEM((N2, 128, 128), BF),
        pltpu.VMEM((NT, NT, 128, 128), BF),
        pltpu.VMEM((NT, S // 128, 128, 128), BF),
        pltpu.VMEM((NT, NT, 128, 128), BF),
        pltpu.VMEM((NT, 128, 128), BF),
        pltpu.VMEM((NT, D, 128), BF),
        pltpu.VMEM((NT, 128, 128), BF),
        pltpu.VMEM((S // 128, NT, 128, 128), BF),
        pltpu.VMEM((S // 128, NT, 128, 128), BF),
        pltpu.VMEM((S, D), BF),
        pltpu.VMEM((NB, S, CB), BF),
        pltpu.VMEM((2, 2, N2, 128, CB), BF),
        pltpu.VMEM((N2 + 1, 128, CB), BF),
        pltpu.VMEM((NT, S // 256, 128, 128), F32),
        pltpu.VMEM((W_ROWS, 128), F32),
        pltpu.SMEM((NZ,), jnp.int32),
        pltpu.VMEM((4, D), BF),
        pltpu.VMEM((D,), BF),
        pltpu.VMEM((1, D), F32),
        pltpu.SemaphoreType.DMA((64,)),
    ]
    out = pl.pallas_call(
        _kernel,
        out_shape=jax.ShapeDtypeStruct((S, 2 * D), BF),
        in_specs=[hbm] * 11,
        out_specs=hbm,
        scratch_shapes=scratch,
        compiler_params=pltpu.CompilerParams(vmem_limit_bytes=100 * 1024 * 1024),
    )(np.zeros((NZ,), np.int32), A_x.reshape(S, D), A_wqkv, A_wo, B_q.reshape(S, D), B_k.reshape(S, D), B_v.reshape(S, D),
      B_shift_k.T, B_ssm_k, B_ssm_D, _TABLES)
    return out.reshape(1, S, 2 * D)
```

```python
import numpy as np
import jax
import jax.numpy as jnp
import jax.experimental.pallas as pl
import jax.experimental.pallas.tpu as pltpu

S = 2048
D = 1024
DH = 32
N1, N2 = 64, 32
CB = 128
NB = D // CB
NT = D // 128
HALO = 8
_AREAS = (("k", HALO + S), ("u", S), ("h", S), ("tf", 4 * S), ("b", 2 * N2 * 128), ("ti", 2 * S),
          ("acc", 4 * 256), ("fence", 8))
AT = {name: sum(n for _, n in _AREAS[:i]) for i, (name, _) in enumerate(_AREAS)}
W_ROWS = sum(n for _, n in _AREAS)
NZ = 32
F0_AT = 48
V_TRAIL, M_TRAIL = 1500, 1200
ROOM = (128, 0, 0)
FIRST = 150 * 128
REGION_BIAS = [0] * NB + [1500, 1500]
WIDE = "ko"
URGENT_STEPS = 8
RP = 64
SYNCS = list(range(NB + 2))
BF = jnp.bfloat16
F32 = jnp.float32


def _dft_tables():
    idx = np.arange(N1)
    col = 16 * (idx // 8) + (idx % 8)
    e = np.exp(-2j * np.pi * np.outer(idx, idx) / N1)
    t = np.exp(-2j * np.pi * np.outer(np.arange(N2) + 0.25, idx) / S)
    tab = np.zeros((2 * 128 + 2 * N2, 128), np.float64)
    p, q, tr, ti = tab[:128], tab[128:256], tab[256:256 + N2], tab[256 + N2:]
    p[:N1, col], p[:N1, col + 8], p[N1:, col], p[N1:, col + 8] = e.real, -e.imag, e.imag, e.real
    q[:N1, col], q[:N1, col + 8], q[N1:, col], q[N1:, col + 8] = -e.imag, -e.real, e.real, -e.imag
    tr[:, col], tr[:, col + 8], ti[:, col], ti[:, col + 8] = t.real, t.real, t.imag, t.imag
    return tab.astype(np.float32)


_TABLES = _dft_tables()


def _add(a, b):
    (sa, xa), (sb, xb) = a, b
    if sa == sb:
        return (sa, xa + xb)
    return (1, xa - xb) if sa > 0 else (1, xb - xa)


def _neg(a):
    return (-a[0], a[1])


def _sub(a, b):
    return _add(a, _neg(b))


def _scale(a, c):
    return (1, a[1] * np.float32(a[0] * c))


def _val(a):
    return a[1] if a[0] > 0 else -a[1]


def _cadd(a, b):
    return (_add(a[0], b[0]), _add(a[1], b[1]))


def _csub(a, b):
    return (_sub(a[0], b[0]), _sub(a[1], b[1]))


def _cmul_i(a, s):
    return (_neg(a[1]), a[0]) if s > 0 else (a[1], _neg(a[0]))


def _cmul_const(a, w):
    c, s = float(np.real(w)), float(np.imag(w))
    return (_add(_scale(a[0], c), _scale(a[1], -s)), _add(_scale(a[0], s), _scale(a[1], c)))


def _fft4(x, s):
    a0, a1 = _cadd(x[0], x[2]), _cadd(x[1], x[3])
    b0, b1 = _csub(x[0], x[2]), _cmul_i(_csub(x[1], x[3]), s)
    return [_cadd(a0, a1), _cadd(b0, b1), _csub(a0, a1), _csub(b0, b1)]


def _fft8(x, s):
    r = np.sqrt(0.5)
    a = [_cadd(x[n], x[n + 4]) for n in range(4)]
    b = [_csub(x[n], x[n + 4]) for n in range(4)]
    t = _cadd(b[1], _cmul_i(b[1], s))
    b[1] = (_scale(t[0], r), _scale(t[1], r))
    b[2] = _cmul_i(b[2], s)
    t = _csub(_cmul_i(b[3], s), b[3])
    b[3] = (_scale(t[0], r), _scale(t[1], r))
    ev, od = _fft4(a, s), _fft4(b, s)
    return [ev[0], od[0], ev[1], od[1], ev[2], od[2], ev[3], od[3]]


_C1, _S1, _R2 = np.cos(np.pi / 8), np.sin(np.pi / 8), np.sqrt(0.5)


def _tw(n, j, s):
    return np.exp(s * 2j * np.pi * n * (4 * j + 1) / 128)


def _fwd_stage1(n, u0, u1, u2, u3):
    u0, u1, u2, u3 = (1, u0), (1, u1), (1, u2), (1, u3)
    t = _scale(u2, _R2)
    p, m_ = _add(u0, t), _sub(u0, t)
    c1u1, s1u1, c1u3, s1u3 = _scale(u1, _C1), _scale(u1, _S1), _scale(u3, _C1), _scale(u3, _S1)
    a, b = _add(c1u1, s1u3), _add(s1u1, c1u3)
    d, e = _sub(c1u1, s1u3), _sub(s1u1, c1u3)
    sj = [(_add(p, a), _neg(_add(t, b))), (_sub(m_, e), _sub(t, d)),
          (_sub(p, a), _sub(b, t)), (_add(m_, e), _add(t, d))]
    out = [sj[j] if n == 0 else _cmul_const(sj[j], _tw(n, j, -1)) for j in range(4)]
    return [(_val(re), _val(im)) for re, im in out]


def _fwd_stage2(t):
    out = _fft8([((1, re), (1, im)) for re, im in t], -1)
    return [(_val(re), _val(im)) for re, im in out]


def _inv_stage1(j, b):
    out = _fft8([((1, re), (1, im)) for re, im in b], 1)
    out = [out[n] if n == 0 else _cmul_const(out[n], _tw(n, j, 1)) for n in range(8)]
    return [(_val(re), _val(im)) for re, im in out]


def _inv_stage2(s):
    (x0, y0), (x1, y1), (x2, y2), (x3, y3) = [((1, re), (1, im)) for re, im in s]
    p, a, b = _add(x0, x2), _sub(x0, x2), _sub(y2, y0)
    m_, e, d = _add(x1, x3), _sub(x3, x1), _sub(y3, y1)
    t = _add(_sub(_add(y1, y3), _add(y0, y2)), _sub(p, m_))
    return [_val(_add(p, m_)),
            _val(_add(_scale(_add(a, d), _C1), _scale(_add(b, e), _S1))),
            _val(_scale(t, _R2)),
            _val(_add(_scale(_sub(a, d), _S1), _scale(_sub(b, e), _C1)))]


def _phi(t):
    return jnp.where(t > 0, t + 1.0, jnp.exp(t)) + 1e-6


def _dot(a, b):
    return jnp.dot(a, b, preferred_element_type=F32)


def _dot_nt(a, b):
    return jax.lax.dot_general(a, b, (((1,), (1,)), ((), ())), preferred_element_type=F32)


def _ld(ref, lead, r0, n):
    lead = lead if isinstance(lead, tuple) else (lead,)
    return pltpu.bitcast(ref.bitcast(jnp.uint32)[(*lead, pl.ds(r0 // 2, n // 2), slice(None))], BF)


def _cat(parts, axis):
    return parts[0] if len(parts) == 1 else jnp.concatenate(parts, axis=axis)


def _spread(stream, extra):
    out = []
    extra = sorted(extra, key=lambda e: e[0])
    e = 0
    for pos, item in enumerate(stream):
        while e < len(extra) and extra[e][0] <= pos:
            out.append(extra[e][1])
            e += 1
        out.append(item)
    return out + [t for _, t in extra[e:]]


def _merge(a, b):
    keyed = [((t + 0.5) / len(x), s, item) for s, x in enumerate((a, b)) for t, item in enumerate(x)]
    return [item for _, _, item in sorted(keyed, key=lambda e: e[:2])]


def _kernel(zero_hbm, x_hbm, wqkv_hbm, wo_hbm, q_hbm, k_hbm, v_hbm, sk_hbm, h_hbm, d_hbm, tab_hbm,
            out_hbm,
            x_v, wq_v, wk_v, wv_v, wo_v, q_v, k_v, v_v, h_v, tab_v, fwd_v, inv_v,
            wkt_s, pkt_s, g_s, kv_s, m_s, zb_s, pq_s, r_s, oa_s, ob_s,
            a_s, yf_s, z_s, w_s, zero_ref, sk_ref, d_ref, skip_s, sems):
    n_sem = [0]

    def zero(i):
        return zero_ref[i % NZ]

    def group(pairs):
        sem = sems.at[n_sem[0]]
        n_sem[0] += 1
        return [pltpu.make_async_copy(src, dst, sem) for src, dst in pairs]

    def start(g):
        for c in g:
            c.start()

    def wait(g):
        for c in g:
            c.wait()

    def col(ref, j):
        return ref.at[:, pl.ds(j * 128, 128)]

    def split(src, dst, n):
        step = src.shape[0] // n
        return [(src.at[pl.ds(t * step, step), :], dst.at[pl.ds(t * step, step), :]) for t in range(n)]

    cp_x = [group([(x_hbm.at[pl.ds(r0, 256), pl.ds(j * 128, 128)], x_v.at[j, pl.ds(r0, 256), :])
                   for j in range(NT)]) for r0 in range(0, S, 256)]
    cp_wq = group([(col(wqkv_hbm, j), wq_v.at[j]) for j in range(NT)])
    cp_wk = [group(split(col(wqkv_hbm, NT + g), wk_v.at[g], 4)) for g in range(NT)]
    cp_wvo = group([(col(wqkv_hbm, 2 * NT + g), wv_v.at[g]) for g in range(NT)]
                   + [(col(wo_hbm, j), wo_v.at[j]) for j in range(NT)])
    parts = [8, 8] + [2] * (NB - 2)
    cp_q = [group(split(col(q_hbm, i), q_v.at[i], 2)) for i in range(NB)]
    cp_kv = [group(split(col(k_hbm, i), k_v.at[i], parts[i]) + split(col(v_hbm, i), v_v.at[i], parts[i]))
             for i in range(NB)]
    cp_h = [group(split(h_hbm.at[pl.ds(i * CB, CB), :], h_v.at[i], parts[i])) for i in range(NB)]
    cp_tab = group([(tab_hbm, tab_v), (sk_hbm, sk_ref), (d_hbm, d_ref)])
    cp_zero = group([(zero_hbm, zero_ref)])
    cp_ob = [group(split(ob_s.at[i], col(out_hbm, NT + i), 8 if i == NB - 1 else 2)) for i in range(NB)]
    oa_spans = []

    def cp_oa(t):
        r0, n = oa_spans[t]
        pairs = split(oa_s.at[pl.ds(r0, n), :], out_hbm.at[pl.ds(r0, n), pl.ds(0, D)], 8)
        return [pltpu.make_async_copy(src, dst, sems.at[n_sem[0] + t]) for src, dst in pairs]

    rows_done = [0, 0]

    def sync(waits=(), starts=()):
        def run():
            for g in starts:
                start(g)
            done, sent = rows_done
            if done > sent:
                oa_spans.append((sent, done - sent))
                start(cp_oa(len(oa_spans) - 1))
                rows_done[1] = done
            for g in waits:
                wait(g)
        return 0, run


    def area(name, r0, n=8):
        return pl.ds(AT[name] + r0, n), slice(None)

    def b_prepare(i):
        def widen(p):
            def run():
                w_s[area("k", HALO + p * RP, RP)] = _ld(k_v, i, p * RP, RP).astype(F32)
            return 30, run

        def gate(p):
            def run():
                taps = sk_ref[:, pl.ds(i * CB, CB)].astype(F32)
                acc = w_s[area("k", HALO + p * RP, RP)] * taps[0:1]
                for j in range(1, 4):
                    acc = acc + w_s[area("k", HALO + p * RP - j, RP)] * taps[j:j + 1]
                w_s[area("u", p * RP, RP)] = acc * _ld(v_v, i, p * RP, RP).astype(F32)
            return 80, run

        def transpose(p):
            def run():
                ht = h_v[i, :, pl.ds(p * 128, 128)].astype(F32).T
                if p == 0:
                    if i == 0:
                        skip_s[...] = d_ref[...].astype(F32).reshape(1, D)
                    skip = skip_s[:, pl.ds(i * CB, CB)]
                    lag = jax.lax.broadcasted_iota(jnp.int32, (128, CB), 0)
                    ht = ht + jnp.where(lag == 0, skip, 0.0)
                w_s[area("h", p * 128, 128)] = ht
            return 70, run

        prep = ([sync([cp_kv[0]], cp_x[5:] + [cp_h[1], cp_kv[1]])] if i == 0 else []) + [widen(0)]
        for p in range(S // RP):
            prep += ([widen(p + 1)] if p + 1 < S // RP else []) + [gate(p)]
        return [transpose(p) for p in range(S // 128)], prep

    def b_forward(i, prep):
        def stage1(h, j, n):
            def run():
                out = _fwd_stage1(n, *[w_s[area("uh"[h], N1 * (n + 8 * m) + 8 * j)] for m in range(4)])
                for r in range(4):
                    for part in range(2):
                        w_s[area("tf", 512 * (8 * h + j) + 16 * (8 * r + n) + 8 * part)] = out[r][part]
            return (46 if n else 32), run

        def stage2(h, j, r):
            def run():
                out = _fwd_stage2([[w_s[area("tf", 512 * (8 * h + j) + 16 * (8 * r + n) + 8 * part)]
                                    for part in range(2)] for n in range(8)])
                for l in range(8):
                    a_s[i % 2, h, r + 4 * l, pl.ds(16 * j, 16), :] = _cat(out[l], 0).astype(BF)
            return 64, run

        tasks = []
        cols = [(h, j) for h in (1, 0) for j in range(N1 // 8)]
        for c, (h, j) in enumerate(cols):
            now = [stage1(h, j, n) for n in range(8)]
            now += [stage2(*cols[c - 1], r) for r in range(4)] if c > 0 else []
            lo = 4 if i == 0 else 0
            if lo <= c < 8:
                share = prep[len(prep) * (c - lo) // (8 - lo):len(prep) * (c + 1 - lo) // (8 - lo)]
                now = _merge(now, share)
            tasks += now
        return tasks + [stage2(*cols[-1], r) for r in range(4)]

    def b_inverse(i):
        def stage1(j, r):
            def run():
                out = _inv_stage1(r, [[w_s[area("b", 128 * (N2 * (i % 2) + r + 4 * l) + 16 * j + 8 * part)]
                                       for part in range(2)] for l in range(8)])
                for n in range(8):
                    for part in range(2):
                        w_s[area("ti", 512 * j + 16 * (4 * n + r) + 8 * part)] = out[n][part]
            return 100, run

        def stage2(jp, n):
            def run():
                ys = [_inv_stage2([[w_s[area("ti", 512 * j + 16 * (4 * n + r) + 8 * part)] for part in range(2)]
                                   for r in range(4)]) for j in (2 * jp, 2 * jp + 1)]
                for m in range(4):
                    r0 = N1 * (n + 8 * m) + 16 * jp
                    y = _cat([ys[0][m], ys[1][m]], 0)
                    ob_s[i, pl.ds(r0, 16), :] = (_ld(q_v, i, r0, 16).astype(F32) * y).astype(BF)
            return 66, run

        tasks = []
        for jp in range(N1 // 16 + 1):
            first = [stage1(j, r) for j in (2 * jp, 2 * jp + 1) for r in range(4)] if jp < N1 // 16 else []
            tasks += _merge(first, [stage2(jp - 1, n) for n in range(8)] if jp > 0 else [])
        return tasks

    def dft_matrix(k2):
        def run():
            f = (tab_v[pl.ds(0, 128), :] * tab_v[pl.ds(256 + k2, 1), :]
                 + tab_v[pl.ds(128, 128), :] * tab_v[pl.ds(256 + N2 + k2, 1), :])
            fwd_v[k2] = f.astype(BF)
            inv_v[k2] = (f.T * (1.0 / S)).astype(BF)
        return 0, run

    def b_middle(i):
        def forward(k2):
            def run():
                rhs = _cat([_ld(a_s, (i % 2, h, k2), 0, 128) for h in range(2)], 1)
                xf = _dot(_ld(fwd_v, k2 + zero(i), 0, 128), rhs)
                ur, ui, hr, hi = xf[:N1, :CB], xf[N1:, :CB], xf[:N1, CB:], xf[N1:, CB:]
                if k2 % 2 == 0:
                    urgent(xf)
                yf_s[k2] = _cat([ur * hr - ui * hi, ur * hi + ui * hr], 0).astype(BF)
            return 64, run

        def inverse(k2):
            def run():
                b = _dot(_ld(inv_v, k2 + zero(i), 0, 128), _ld(yf_s, k2, 0, 128))
                if k2 % 4 == 0:
                    urgent(b)
                w_s[area("b", 128 * (N2 * (i % 2) + k2), 128)] = b
            return 32, run

        tasks = []
        for k4 in range(N2 // 4 + 1):
            if k4 < N2 // 4:
                tasks += [[forward(4 * k4), forward(4 * k4 + 1)], [forward(4 * k4 + 2), forward(4 * k4 + 3)]]
            if k4 > 0:
                tasks += [[inverse(4 * k4 - 4 + r) for r in range(4)]]
        return tasks

    def head_mask():
        r = jax.lax.broadcasted_iota(jnp.int32, (128, 128), 0) // DH
        c = jax.lax.broadcasted_iota(jnp.int32, (128, 128), 1) // DH
        return r == c

    room = {}
    mid_chain = set()

    lead_chain = [None]

    def urgent(value):
        c = value[:8, :128] if lead_chain[0] is None else lead_chain[0] + value[:8, :128]
        for _ in range(URGENT_STEPS):
            c = jnp.exp(c)
        lead_chain[0] = c

    def fence(value):
        w_s[pl.ds(pl.multiple_of(zero(0) + AT["fence"], 8), 8), :] = value
        yf_s.bitcast(jnp.uint32)[zero(0) + N2, pl.ds(0, 8), :] = pltpu.bitcast(value, jnp.uint32)

    def chain(kind, n_tiles, n_cols, operands, dot, finish):
        wide = n_cols if kind in WIDE else 1
        deep = 4 // wide
        acc = [None]

        def piece(j0, k0):
            def run():
                d = dot(*operands(range(k0, k0 + deep), range(j0, j0 + wide)))
                acc[0] = d if k0 == 0 else acc[0] + d
                fence(d[:8, :128])
                urgent(d)
                if k0 + deep == n_tiles:
                    for t in range(wide):
                        finish(j0 + t, acc[0][:, 128 * t:128 * t + 128])
            if j0 + k0 > 0:
                mid_chain.add(run)
            if k0 + deep == n_tiles:
                room[run] = ROOM[0]
            return 128, run
        return [piece(j0, k0) for j0 in range(0, n_cols, wide) for k0 in range(0, n_tiles, deep)]

    followers = {}

    def chain_then(kind, operands, dot, part):
        slot = len(followers) % 4

        def park(j, acc):
            w_s[area("acc", 256 * slot + 128 * j, 128)] = acc

        def quarter(t):
            def run():
                part(pl.ds(32 * t, 32), 32 * t, *[w_s[area("acc", 256 * slot + 128 * half + 32 * t, 32)] for half in range(2)])
            room[run] = ROOM[1]
            return 0, run
        pieces = chain(kind, NT, 2, operands, dot, park)
        followers[pieces[-1][1]] = [quarter(t) for t in range(4)]
        return pieces

    def a_transpose_wk(g):
        def tile(j):
            def run():
                wkt_s[g, j] = _ld(wk_v, g, j * 128, 128).astype(F32).T.astype(BF)
            return 0, run
        return [tile(j) for j in range(NT)]

    def a_keys(g, c):
        def operands(ks, js):
            return (_cat([_ld(wkt_s, (g + zero(c), k), 0, 128) for k in ks], 1),
                    _cat([_ld(x_v, k + zero(g), c * 256 + 128 * js[0], 128 * len(js)) for k in ks], 1))

        def part(rows, r0, lo, hi):
            lo, hi = _phi(lo), _phi(hi)
            pkt_s[g, 2 * c, rows, :] = lo.astype(BF)
            pkt_s[g, 2 * c + 1, rows, :] = hi.astype(BF)
            total = lo + hi
            if c < S // 256 - 1:
                z_s[g, c, rows, :] = total
            else:
                for b in range(c):
                    total = total + z_s[g, b, rows, :]
                z = jnp.broadcast_to(jnp.sum(total, axis=1, keepdims=True), (32, 128))
                head = jax.lax.broadcasted_iota(jnp.int32, (32, 128), 1) // DH
                zb_s[g, rows, :] = jnp.where(head == r0 // DH, z, 0.0).astype(BF)
        return chain_then("k", operands, _dot_nt, part)

    def a_gram(g):
        def block(n):
            def operands(ks, js):
                return (_cat([_ld(pkt_s, (g, k), 0, 128) for k in ks], 1),
                        _cat([_ld(x_v, 2 * n + j + zero(NT + g), 128 * ks[0], 128 * len(ks)) for j in js], 1))

            def finish(j, acc):
                g_s[g, 2 * n + j] = acc.astype(BF)
            return chain("g", S // 128, 2, operands, _dot, finish)
        return [t for n in range(D // 256) for t in block(n)]

    def a_kv(g):
        acc = [None]

        def piece(kk):
            def run():
                d = _dot(_cat([_ld(g_s, (g, j), 0, 128) for j in range(4 * kk, 4 * kk + 4)], 1),
                         _ld(wv_v, g, kk * 512, 512))
                fence(d[:8, :])
                urgent(d)
                if kk == 0:
                    acc[0] = d
                else:
                    kv_s[g] = jnp.where(head_mask(), acc[0] + d, 0.0).astype(BF)
            if kk > 0:
                mid_chain.add(run)
            return 128, run
        return [piece(0), piece(1)]

    def a_mix(g, half):
        def run():
            js = range(4 * half, 4 * half + 4)
            m = _dot(_ld(kv_s, g, 0, 128), _cat([_ld(wo_v, j, g * 128, 128) for j in js], 1))
            for t, j in enumerate(js):
                m_s[j, pl.ds(g * 128, 128), :] = m[:, t * 128:(t + 1) * 128].astype(BF)
        return 128, run

    def a_query(c, n):
        def operands(ks, js):
            return (_cat([_ld(x_v, k + zero(2 * NT + 2 * n + js[0]), c * 128, 128) for k in ks], 1),
                    _cat([_ld(wq_v, 2 * n + j + zero(c), 128 * ks[0], 128 * len(ks)) for j in js], 1))

        def part(rows, r0, lo, hi):
            pq_s[c, 2 * n, rows, :] = _phi(lo).astype(BF)
            pq_s[c, 2 * n + 1, rows, :] = _phi(hi).astype(BF)
        return chain_then("q", operands, _dot, part)

    def a_normalise(c, half):
        def run():
            for g in range(4 * half, 4 * half + 4):
                pq = _ld(pq_s, (c, g), 0, 128)
                den = _dot(pq, _ld(zb_s, g + zero(c), 0, 128)) + 1e-6
                if g % 4 == 0:
                    urgent(den)
                inv = pl.reciprocal(den, approx=True)
                inv = inv * (2.0 - den * inv)
                r_s[c, g] = (pq.astype(F32) * inv).astype(BF)
        room[run] = ROOM[2]
        return 128, run

    def a_out(c, n):
        def operands(ks, js):
            return (_cat([_ld(r_s, (c, k), 0, 128) for k in ks], 1),
                    _cat([_ld(m_s, 2 * n + j + zero(c), 128 * ks[0], 128 * len(ks)) for j in js], 1))

        def finish(j, acc):
            oa_s[pl.ds(c * 128, 128), pl.ds(n * 256 + j * 128, 128)] = acc.astype(BF)
            if n == D // 256 - 1 and j == 1:
                rows_done[0] = (c + 1) * 128
        return chain("o", NT, 2, operands, _dot, finish)

    def starter(*groups):
        def run():
            for g in groups:
                start(g)
        return 0, run

    a_stream, extra = [], []
    n_g = n_c = 0
    for grow in "gcgggcggcggccccc":
        if grow == "g":
            a_stream += [t for c in range(n_c) for t in a_keys(n_g, c)]
            n_g += 1
        else:
            a_stream += [t for g in range(n_g) for t in a_keys(g, n_c)]
            n_c += 1
    extra += [(0, sync([cp_x[0], cp_wk[1]], [cp_wk[2], cp_wk[3]])),
              (4, sync([cp_wk[2], cp_wk[3]], [cp_x[1], cp_wk[4], cp_wk[5]])),
              (16, sync([cp_x[1]], [cp_x[2], cp_h[0], cp_tab])),
              (24, sync([cp_wk[4], cp_wk[5]], [cp_wk[6], cp_wk[7]])),
              (F0_AT, sync([cp_x[2], cp_wk[6], cp_wk[7], cp_tab, cp_h[0]], [cp_x[3], cp_kv[0], cp_x[4]])),
              (96, sync([cp_x[3], cp_x[4]]))]
    extra += [(F0_AT + 2 + 2 * k2, dft_matrix(k2)) for k2 in range(N2)]
    for g, (at, step) in {1: (0, 0.45), 2: (4, 0.45), 3: (8, 0.45), 4: (24, 0.9), 5: (32, 0.9), 6: (50, 2),
                          7: (68, 1.8)}.items():
        extra += [(at + int(step * j), t) for j, t in enumerate(a_transpose_wk(g))]
    for g in range(NT):
        at = len(a_stream)
        if g >= 5:
            for t, gg in enumerate(range(3 * (g - 5), min(3 * (g - 4), NT - 1))):
                extra += [(at + 8 * t + 8, p) for p in a_kv(gg)] + [(at + 8 * t + 16, a_mix(gg, 0)), (at + 8 * t + 16, a_mix(gg, 1))]
        a_stream += a_gram(g)
    a_stream = _spread(a_stream, extra)
    tail = []
    n_c = S // 128
    for c in range(n_c + 1):
        stream = [t for n in range(D // 256) for t in a_query(c, n)] if c < n_c else []
        stream += [t for n in range(D // 256) for t in a_out(c - 1, n)] if c > 0 else []
        at = len(a_stream)
        if c == 0:
            tail += [(at + 4, p) for p in a_kv(NT - 1)] + [(at + 8, a_mix(NT - 1, 0)), (at + 8, a_mix(NT - 1, 1))]
        if c < n_c:
            tail += [(at + 12, a_normalise(c, 0)), (at + 24, a_normalise(c, 1))]
        a_stream += stream
    a_stream = _spread(a_stream, tail)
    spread, pending = [], []
    for item in a_stream:
        spread.append(item)
        if item[0] > 0 and pending:
            spread.append(pending.pop(0))
        pending += followers.get(item[1], [])
    a_stream = spread + pending

    v_regions, m_regions = [], []
    for r in range(NB + 2):
        v = b_inverse(r - 2) if r >= 2 else []
        if r < NB:
            transposes, prep = b_prepare(r)
            early = len(prep) // 2 if r > 0 else 0
            v = _merge(v, _merge(transposes, prep[:early])) + b_forward(r, prep[early:])
        if r == NB + 1:
            v.append(sync(starts=[cp_ob[NB - 1]]))
        v_regions.append(v)
        m_regions.append(b_middle(r - 1) if 1 <= r <= NB else [])
    v_cost = [sum(c for c, _ in v) for v in v_regions]
    m_cost = [sum(c for grp in m for c, _ in grp) for m in m_regions]
    total = sum(c for c, _ in a_stream) + sum(m_cost)
    weight = [c + w for c, w in zip(v_cost, REGION_BIAS)]

    sync([cp_zero], [cp_zero, cp_wk[0], cp_x[0]])[1]()
    w_s[area("k", 0)] = jnp.zeros((HALO, CB), F32)
    for ref in (pkt_s, r_s, g_s, kv_s, pq_s, a_s, z_s, fwd_v, inv_v):
        lead = (zero(0),) + (0,) * (len(ref.shape) - 3)
        ref[(*lead, pl.ds(0, 16), slice(None))] = jnp.zeros((16, CB), ref.dtype)
    sync([cp_wk[0]], [cp_wk[1]])[1]()
    for _, run in a_transpose_wk(0):
        run()

    def needs(lo, hi):
        return ([g for i in range(max(lo, 1), min(hi, NB)) for g in (cp_h[i], cp_kv[i])]
                + [cp_q[i - 2] for i in range(max(lo, 2), hi)])

    assert SYNCS[:4] == [0, 1, 2, 3] and SYNCS[-1] == NB + 1
    ai, clock, ob_sent = 0, 0, 0
    for r in range(NB + 2):
        end = FIRST + (total - FIRST) * sum(weight[1:r + 1]) / sum(weight[1:])
        a_end, t = ai, clock + m_cost[r]
        while a_end < len(a_stream) and (t < end or a_stream[a_end][0] == 0
                                         or a_stream[a_end][1] in mid_chain or r == NB + 1):
            t += a_stream[a_end][0]
            a_end += 1
        length = sum(room.get(run, cost) for cost, run in a_stream[ai:a_end])
        v, m = v_regions[r], m_regions[r]
        lead, trail = 0, (V_TRAIL if r == NB + 1 else 0)
        if r == 0:
            first = [p for p, (cost, _) in enumerate(a_stream) if cost > 0][F0_AT + 2]
            lead = sum(room.get(run, cost) for cost, run in a_stream[:first])
        v_time, acc_cost = [], 0
        for c, _ in v:
            v_time.append(lead + (length - lead - trail) * acc_cost / v_cost[r])
            acc_cost += c

        def region():
            now, pa, pm, pv = 0, ai, 0, 0
            while pa < a_end or pm < len(m):
                if pm < len(m) and ((length - M_TRAIL) * pm / len(m) <= now or pa == a_end):
                    todo = m[pm]
                    pm += 1
                else:
                    todo = [a_stream[pa]]
                    pa += 1
                for cost, run in todo:
                    run()
                    now += 0 if len(todo) > 1 else room.get(run, cost)
                while pv < len(v) and v_time[pv] <= now:
                    v[pv][1]()
                    pv += 1
            for _, run in v[pv:]:
                run()
            if lead_chain[0] is not None:
                fence(lead_chain[0])
                lead_chain[0] = None

        if r in SYNCS:
            nxt = min([b for b in SYNCS if b > r] + [NB + 2])
            far = min([b for b in SYNCS if b > nxt] + [NB + 2])
            waits, starts = needs(r, nxt), (needs(nxt, far) if r > 0 else [])
            while ob_sent + 3 <= r:
                starts.append(cp_ob[ob_sent])
                ob_sent += 1
            pieces = sum(c > 0 for c, _ in a_stream[:ai])
            if r == 1:
                assert F0_AT + 2 * N2 + 2 < pieces <= 160 and nxt == 2
                waits, starts = waits + cp_x[5:], starts + [cp_wvo]
            if r == 2:
                starts = starts + [cp_wq]
            if r == 3:
                assert pieces <= 256 + 5 * 32 + 8
                waits = waits + [cp_wvo, cp_wq]
            sync(waits, starts)[1]()
        region()
        ai, clock = a_end, t

    sync()[1]()
    assert rows_done == [S, S] and n_sem[0] + len(oa_spans) <= sems.shape[0]
    for g in [cp_oa(t) for t in range(len(oa_spans))] + cp_ob:
        wait(g)


@jax.jit
def pallas_concat_heads__linear_attn_block__ssm_conv_h3__prompt_kernel(
    A_x: jax.Array,
    A_wqkv: jax.Array,
    A_wo: jax.Array,
    B_q: jax.Array,
    B_k: jax.Array,
    B_v: jax.Array,
    B_shift_k: jax.Array,
    B_ssm_k: jax.Array,
    B_ssm_D: jax.Array,
):
    hbm = pl.BlockSpec(memory_space=pl.ANY)
    scratch = [
        pltpu.VMEM((NT, S, 128), BF),
        pltpu.VMEM((NT, D, 128), BF),
        pltpu.VMEM((NT, D, 128), BF),
        pltpu.VMEM((NT, D, 128), BF),
        pltpu.VMEM((NT, D, 128), BF),
        pltpu.VMEM((NB, S, CB), BF),
        pltpu.VMEM((NB, S, CB), BF),
        pltpu.VMEM((NB, S, CB), BF),
        pltpu.VMEM((NB, CB, S), BF),
        pltpu.VMEM(_TABLES.shape, F32),
        pltpu.VMEM((N2, 128, 128), BF),
        pltpu.VMEM((N2, 128, 128), BF),
        pltpu.VMEM((NT, NT, 128, 128), BF),
        pltpu.VMEM((NT, S // 128, 128, 128), BF),
        pltpu.VMEM((NT, NT, 128, 128), BF),
        pltpu.VMEM((NT, 128, 128), BF),
        pltpu.VMEM((NT, D, 128), BF),
        pltpu.VMEM((NT, 128, 128), BF),
        pltpu.VMEM((S // 128, NT, 128, 128), BF),
        pltpu.VMEM((S // 128, NT, 128, 128), BF),
        pltpu.VMEM((S, D), BF),
        pltpu.VMEM((NB, S, CB), BF),
        pltpu.VMEM((2, 2, N2, 128, CB), BF),
        pltpu.VMEM((N2 + 1, 128, CB), BF),
        pltpu.VMEM((NT, S // 256, 128, 128), F32),
        pltpu.VMEM((W_ROWS, 128), F32),
        pltpu.SMEM((NZ,), jnp.int32),
        pltpu.VMEM((4, D), BF),
        pltpu.VMEM((D,), BF),
        pltpu.VMEM((1, D), F32),
        pltpu.SemaphoreType.DMA((64,)),
    ]
    out = pl.pallas_call(
        _kernel,
        out_shape=jax.ShapeDtypeStruct((S, 2 * D), BF),
        in_specs=[hbm] * 11,
        out_specs=hbm,
        scratch_shapes=scratch,
        compiler_params=pltpu.CompilerParams(vmem_limit_bytes=100 * 1024 * 1024),
    )(np.zeros((NZ,), np.int32), A_x.reshape(S, D), A_wqkv, A_wo, B_q.reshape(S, D), B_k.reshape(S, D), B_v.reshape(S, D),
      B_shift_k.T, B_ssm_k, B_ssm_D, _TABLES)
    return out.reshape(1, S, 2 * D)
```

```python
import numpy as np
import jax
import jax.numpy as jnp
import jax.experimental.pallas as pl
import jax.experimental.pallas.tpu as pltpu

S = 2048
D = 1024
DH = 32
N1, N2 = 64, 32
CB = 128
NB = D // CB
NT = D // 128
HALO = 8
_AREAS = (("k", HALO + S), ("u", S), ("h", S), ("tf", 4 * S), ("b", 2 * N2 * 128), ("ti", 2 * S),
          ("acc", 4 * 256), ("fence", 8))
AT = {name: sum(n for _, n in _AREAS[:i]) for i, (name, _) in enumerate(_AREAS)}
W_ROWS = sum(n for _, n in _AREAS)
NZ = 32
F0_AT = 48
V_TRAIL, M_TRAIL = 1500, 1200
ROOM = (128, 0, 0)
FIRST = 150 * 128
REGION_BIAS = [0] * NB + [1500, 1500]
WIDE = "ko"
URGENT_STEPS = 8
RP = 64
SYNCS = list(range(NB + 2))
BF = jnp.bfloat16
F32 = jnp.float32


def _dft_tables():
    idx = np.arange(N1)
    col = 16 * (idx // 8) + (idx % 8)
    e = np.exp(-2j * np.pi * np.outer(idx, idx) / N1)
    t = np.exp(-2j * np.pi * np.outer(np.arange(N2) + 0.25, idx) / S)
    tab = np.zeros((2 * 128 + 2 * N2, 128), np.float64)
    p, q, tr, ti = tab[:128], tab[128:256], tab[256:256 + N2], tab[256 + N2:]
    p[:N1, col], p[:N1, col + 8], p[N1:, col], p[N1:, col + 8] = e.real, -e.imag, e.imag, e.real
    q[:N1, col], q[:N1, col + 8], q[N1:, col], q[N1:, col + 8] = -e.imag, -e.real, e.real, -e.imag
    tr[:, col], tr[:, col + 8], ti[:, col], ti[:, col + 8] = t.real, t.real, t.imag, t.imag
    return tab.astype(np.float32)


_TABLES = _dft_tables()


def _add(a, b):
    (sa, xa), (sb, xb) = a, b
    if sa == sb:
        return (sa, xa + xb)
    return (1, xa - xb) if sa > 0 else (1, xb - xa)


def _neg(a):
    return (-a[0], a[1])


def _sub(a, b):
    return _add(a, _neg(b))


def _scale(a, c):
    return (1, a[1] * np.float32(a[0] * c))


def _val(a):
    return a[1] if a[0] > 0 else -a[1]


def _cadd(a, b):
    return (_add(a[0], b[0]), _add(a[1], b[1]))


def _csub(a, b):
    return (_sub(a[0], b[0]), _sub(a[1], b[1]))


def _cmul_i(a, s):
    return (_neg(a[1]), a[0]) if s > 0 else (a[1], _neg(a[0]))


def _cmul_const(a, w):
    c, s = float(np.real(w)), float(np.imag(w))
    return (_add(_scale(a[0], c), _scale(a[1], -s)), _add(_scale(a[0], s), _scale(a[1], c)))


def _fft4(x, s):
    a0, a1 = _cadd(x[0], x[2]), _cadd(x[1], x[3])
    b0, b1 = _csub(x[0], x[2]), _cmul_i(_csub(x[1], x[3]), s)
    return [_cadd(a0, a1), _cadd(b0, b1), _csub(a0, a1), _csub(b0, b1)]


def _fft8(x, s):
    r = np.sqrt(0.5)
    a = [_cadd(x[n], x[n + 4]) for n in range(4)]
    b = [_csub(x[n], x[n + 4]) for n in range(4)]
    t = _cadd(b[1], _cmul_i(b[1], s))
    b[1] = (_scale(t[0], r), _scale(t[1], r))
    b[2] = _cmul_i(b[2], s)
    t = _csub(_cmul_i(b[3], s), b[3])
    b[3] = (_scale(t[0], r), _scale(t[1], r))
    ev, od = _fft4(a, s), _fft4(b, s)
    return [ev[0], od[0], ev[1], od[1], ev[2], od[2], ev[3], od[3]]


_C1, _S1, _R2 = np.cos(np.pi / 8), np.sin(np.pi / 8), np.sqrt(0.5)


def _tw(n, j, s):
    return np.exp(s * 2j * np.pi * n * (4 * j + 1) / 128)


def _fwd_stage1(n, u0, u1, u2, u3):
    u0, u1, u2, u3 = (1, u0), (1, u1), (1, u2), (1, u3)
    t = _scale(u2, _R2)
    p, m_ = _add(u0, t), _sub(u0, t)
    c1u1, s1u1, c1u3, s1u3 = _scale(u1, _C1), _scale(u1, _S1), _scale(u3, _C1), _scale(u3, _S1)
    a, b = _add(c1u1, s1u3), _add(s1u1, c1u3)
    d, e = _sub(c1u1, s1u3), _sub(s1u1, c1u3)
    sj = [(_add(p, a), _neg(_add(t, b))), (_sub(m_, e), _sub(t, d)),
          (_sub(p, a), _sub(b, t)), (_add(m_, e), _add(t, d))]
    out = [sj[j] if n == 0 else _cmul_const(sj[j], _tw(n, j, -1)) for j in range(4)]
    return [(_val(re), _val(im)) for re, im in out]


def _fwd_stage2(t):
    out = _fft8([((1, re), (1, im)) for re, im in t], -1)
    return [(_val(re), _val(im)) for re, im in out]


def _inv_stage1(j, b):
    out = _fft8([((1, re), (1, im)) for re, im in b], 1)
    out = [out[n] if n == 0 else _cmul_const(out[n], _tw(n, j, 1)) for n in range(8)]
    return [(_val(re), _val(im)) for re, im in out]


def _inv_stage2(s):
    (x0, y0), (x1, y1), (x2, y2), (x3, y3) = [((1, re), (1, im)) for re, im in s]
    p, a, b = _add(x0, x2), _sub(x0, x2), _sub(y2, y0)
    m_, e, d = _add(x1, x3), _sub(x3, x1), _sub(y3, y1)
    t = _add(_sub(_add(y1, y3), _add(y0, y2)), _sub(p, m_))
    return [_val(_add(p, m_)),
            _val(_add(_scale(_add(a, d), _C1), _scale(_add(b, e), _S1))),
            _val(_scale(t, _R2)),
            _val(_add(_scale(_sub(a, d), _S1), _scale(_sub(b, e), _C1)))]


def _phi(t):
    return jnp.where(t > 0, t + 1.0, jnp.exp(t)) + 1e-6


def _dot(a, b):
    return jnp.dot(a, b, preferred_element_type=F32)


def _dot_nt(a, b):
    return jax.lax.dot_general(a, b, (((1,), (1,)), ((), ())), preferred_element_type=F32)


def _ld(ref, lead, r0, n):
    lead = lead if isinstance(lead, tuple) else (lead,)
    return pltpu.bitcast(ref.bitcast(jnp.uint32)[(*lead, pl.ds(r0 // 2, n // 2), slice(None))], BF)


def _cat(parts, axis):
    return parts[0] if len(parts) == 1 else jnp.concatenate(parts, axis=axis)


def _spread(stream, extra):
    out = []
    extra = sorted(extra, key=lambda e: e[0])
    e = 0
    for pos, item in enumerate(stream):
        while e < len(extra) and extra[e][0] <= pos:
            out.append(extra[e][1])
            e += 1
        out.append(item)
    return out + [t for _, t in extra[e:]]


def _merge(a, b):
    keyed = [((t + 0.5) / len(x), s, item) for s, x in enumerate((a, b)) for t, item in enumerate(x)]
    return [item for _, _, item in sorted(keyed, key=lambda e: e[:2])]


def _kernel(zero_hbm, x_hbm, wqkv_hbm, wo_hbm, q_hbm, k_hbm, v_hbm, sk_hbm, h_hbm, d_hbm, tab_hbm,
            out_hbm,
            x_v, wq_v, wk_v, wv_v, wo_v, q_v, k_v, v_v, h_v, tab_v, fwd_v, inv_v,
            wkt_s, pkt_s, g_s, kv_s, m_s, zb_s, pq_s, r_s, oa_s, ob_s,
            a_s, yf_s, z_s, w_s, zero_ref, sk_ref, d_ref, skip_s, sems):
    n_sem = [0]

    def zero(i):
        return zero_ref[i % NZ]

    def group(pairs):
        sem = sems.at[n_sem[0]]
        n_sem[0] += 1
        return [pltpu.make_async_copy(src, dst, sem) for src, dst in pairs]

    def start(g):
        for c in g:
            c.start()

    def wait(g):
        for c in g:
            c.wait()

    def col(ref, j):
        return ref.at[:, pl.ds(j * 128, 128)]

    def split(src, dst, n):
        step = src.shape[0] // n
        return [(src.at[pl.ds(t * step, step), :], dst.at[pl.ds(t * step, step), :]) for t in range(n)]

    cp_x = [group([(x_hbm.at[pl.ds(r0, 256), pl.ds(j * 128, 128)], x_v.at[j, pl.ds(r0, 256), :])
                   for j in range(NT)]) for r0 in range(0, S, 256)]
    cp_wq = group([(col(wqkv_hbm, j), wq_v.at[j]) for j in range(NT)])
    cp_wk = [group(split(col(wqkv_hbm, NT + g), wk_v.at[g], 4)) for g in range(NT)]
    cp_wvo = group([(col(wqkv_hbm, 2 * NT + g), wv_v.at[g]) for g in range(NT)]
                   + [(col(wo_hbm, j), wo_v.at[j]) for j in range(NT)])
    parts = [8, 8] + [2] * (NB - 2)
    cp_q = [group(split(col(q_hbm, i), q_v.at[i], 2)) for i in range(NB)]
    cp_kv = [group(split(col(k_hbm, i), k_v.at[i], parts[i]) + split(col(v_hbm, i), v_v.at[i], parts[i]))
             for i in range(NB)]
    cp_h = [group(split(h_hbm.at[pl.ds(i * CB, CB), :], h_v.at[i], parts[i])) for i in range(NB)]
    cp_tab = group([(tab_hbm, tab_v), (sk_hbm, sk_ref), (d_hbm, d_ref)])
    cp_zero = group([(zero_hbm, zero_ref)])
    cp_ob = [group(split(ob_s.at[i], col(out_hbm, NT + i), 8 if i == NB - 1 else 2)) for i in range(NB)]
    oa_spans = []

    def cp_oa(t):
        r0, n = oa_spans[t]
        pairs = split(oa_s.at[pl.ds(r0, n), :], out_hbm.at[pl.ds(r0, n), pl.ds(0, D)], 8)
        return [pltpu.make_async_copy(src, dst, sems.at[n_sem[0] + t]) for src, dst in pairs]

    rows_done = [0, 0]

    def sync(waits=(), starts=()):
        def run():
            for g in starts:
                start(g)
            done, sent = rows_done
            if done > sent:
                oa_spans.append((sent, done - sent))
                start(cp_oa(len(oa_spans) - 1))
                rows_done[1] = done
            for g in waits:
                wait(g)
        return 0, run


    def area(name, r0, n=8):
        return pl.ds(AT[name] + r0, n), slice(None)

    def b_prepare(i):
        def widen(p):
            def run():
                w_s[area("k", HALO + p * RP, RP)] = _ld(k_v, i, p * RP, RP).astype(F32)
            return 30, run

        def gate(p):
            def run():
                taps = sk_ref[:, pl.ds(i * CB, CB)].astype(F32)
                acc = w_s[area("k", HALO + p * RP, RP)] * taps[0:1]
                for j in range(1, 4):
                    acc = acc + w_s[area("k", HALO + p * RP - j, RP)] * taps[j:j + 1]
                w_s[area("u", p * RP, RP)] = acc * _ld(v_v, i, p * RP, RP).astype(F32)
            return 80, run

        def transpose(p):
            def run():
                ht = h_v[i, :, pl.ds(p * 128, 128)].astype(F32).T
                if p == 0:
                    if i == 0:
                        skip_s[...] = d_ref[...].astype(F32).reshape(1, D)
                    skip = skip_s[:, pl.ds(i * CB, CB)]
                    lag = jax.lax.broadcasted_iota(jnp.int32, (128, CB), 0)
                    ht = ht + jnp.where(lag == 0, skip, 0.0)
                w_s[area("h", p * 128, 128)] = ht
            return 70, run

        prep = ([sync([cp_kv[0]], cp_x[5:] + [cp_h[1], cp_kv[1]])] if i == 0 else []) + [widen(0)]
        for p in range(S // RP):
            prep += ([widen(p + 1)] if p + 1 < S // RP else []) + [gate(p)]
        return [transpose(p) for p in range(S // 128)], prep

    def b_forward(i, prep):
        def stage1(h, j, n):
            def run():
                out = _fwd_stage1(n, *[w_s[area("uh"[h], N1 * (n + 8 * m) + 8 * j)] for m in range(4)])
                for r in range(4):
                    for part in range(2):
                        w_s[area("tf", 512 * (8 * h + j) + 16 * (8 * r + n) + 8 * part)] = out[r][part]
            return (46 if n else 32), run

        def stage2(h, j, r):
            def run():
                out = _fwd_stage2([[w_s[area("tf", 512 * (8 * h + j) + 16 * (8 * r + n) + 8 * part)]
                                    for part in range(2)] for n in range(8)])
                for l in range(8):
                    a_s[i % 2, h, r + 4 * l, pl.ds(16 * j, 16), :] = _cat(out[l], 0).astype(BF)
            return 64, run

        tasks = []
        cols = [(h, j) for h in (1, 0) for j in range(N1 // 8)]
        for c, (h, j) in enumerate(cols):
            now = [stage1(h, j, n) for n in range(8)]
            now += [stage2(*cols[c - 1], r) for r in range(4)] if c > 0 else []
            lo = 4 if i == 0 else 0
            if lo <= c < 8:
                share = prep[len(prep) * (c - lo) // (8 - lo):len(prep) * (c + 1 - lo) // (8 - lo)]
                now = _merge(now, share)
            tasks += now
        return tasks + [stage2(*cols[-1], r) for r in range(4)]

    def b_inverse(i):
        def stage1(j, r):
            def run():
                out = _inv_stage1(r, [[w_s[area("b", 128 * (N2 * (i % 2) + r + 4 * l) + 16 * j + 8 * part)]
                                       for part in range(2)] for l in range(8)])
                for n in range(8):
                    for part in range(2):
                        w_s[area("ti", 512 * j + 16 * (4 * n + r) + 8 * part)] = out[n][part]
            return 100, run

        def stage2(jp, n):
            def run():
                ys = [_inv_stage2([[w_s[area("ti", 512 * j + 16 * (4 * n + r) + 8 * part)] for part in range(2)]
                                   for r in range(4)]) for j in (2 * jp, 2 * jp + 1)]
                for m in range(4):
                    r0 = N1 * (n + 8 * m) + 16 * jp
                    y = _cat([ys[0][m], ys[1][m]], 0)
                    ob_s[i, pl.ds(r0, 16), :] = (_ld(q_v, i, r0, 16).astype(F32) * y).astype(BF)
            return 66, run

        tasks = []
        for jp in range(N1 // 16 + 1):
            first = [stage1(j, r) for j in (2 * jp, 2 * jp + 1) for r in range(4)] if jp < N1 // 16 else []
            tasks += _merge(first, [stage2(jp - 1, n) for n in range(8)] if jp > 0 else [])
        return tasks

    def dft_matrix(k2):
        def run():
            f = (tab_v[pl.ds(0, 128), :] * tab_v[pl.ds(256 + k2, 1), :]
                 + tab_v[pl.ds(128, 128), :] * tab_v[pl.ds(256 + N2 + k2, 1), :])
            fwd_v[k2] = f.astype(BF)
            inv_v[k2] = (f.T * (1.0 / S)).astype(BF)
        return 0, run

    def b_middle(i):
        def forward(k2):
            def run():
                rhs = _cat([_ld(a_s, (i % 2, h, k2), 0, 128) for h in range(2)], 1)
                xf = _dot(_ld(fwd_v, k2 + zero(i), 0, 128), rhs)
                ur, ui, hr, hi = xf[:N1, :CB], xf[N1:, :CB], xf[:N1, CB:], xf[N1:, CB:]
                if k2 % 2 == 0:
                    urgent(xf)
                yf_s[k2] = _cat([ur * hr - ui * hi, ur * hi + ui * hr], 0).astype(BF)
            return 64, run

        def inverse(k2):
            def run():
                b = _dot(_ld(inv_v, k2 + zero(i), 0, 128), _ld(yf_s, k2, 0, 128))
                if k2 % 4 == 0:
                    urgent(b)
                w_s[area("b", 128 * (N2 * (i % 2) + k2), 128)] = b
            return 32, run

        tasks = []
        for k4 in range(N2 // 4 + 1):
            if k4 < N2 // 4:
                tasks += [[forward(4 * k4), forward(4 * k4 + 1)], [forward(4 * k4 + 2), forward(4 * k4 + 3)]]
            if k4 > 0:
                tasks += [[inverse(4 * k4 - 4 + r) for r in range(4)]]
        return tasks

    def head_mask():
        r = jax.lax.broadcasted_iota(jnp.int32, (128, 128), 0) // DH
        c = jax.lax.broadcasted_iota(jnp.int32, (128, 128), 1) // DH
        return r == c

    room = {}
    mid_chain = set()

    lead_chain = [None]

    def urgent(value):
        c = value[:8, :128] if lead_chain[0] is None else lead_chain[0] + value[:8, :128]
        for _ in range(URGENT_STEPS):
            c = jnp.exp(c)
        lead_chain[0] = c

    fenced = [inv_v]

    def fence(value):
        w_s[pl.ds(pl.multiple_of(zero(0) + AT["fence"], 8), 8), :] = value
        fenced[0].bitcast(jnp.uint32)[zero(0) + N2, pl.ds(0, 8), :] = pltpu.bitcast(value, jnp.uint32)

    def chain(kind, n_tiles, n_cols, operands, dot, finish):
        wide = n_cols if kind in WIDE else 1
        deep = 4 // wide
        acc = [None]

        def piece(j0, k0):
            def run():
                d = dot(*operands(range(k0, k0 + deep), range(j0, j0 + wide)))
                acc[0] = d if k0 == 0 else acc[0] + d
                fence(d[:8, :128])
                urgent(d)
                if k0 + deep == n_tiles:
                    for t in range(wide):
                        finish(j0 + t, acc[0][:, 128 * t:128 * t + 128])
            if j0 + k0 > 0:
                mid_chain.add(run)
            if k0 + deep == n_tiles:
                room[run] = ROOM[0]
            return 128, run
        return [piece(j0, k0) for j0 in range(0, n_cols, wide) for k0 in range(0, n_tiles, deep)]

    followers = {}

    def chain_then(kind, operands, dot, part):
        slot = len(followers) % 4

        def park(j, acc):
            w_s[area("acc", 256 * slot + 128 * j, 128)] = acc

        def quarter(t):
            def run():
                part(pl.ds(32 * t, 32), 32 * t, *[w_s[area("acc", 256 * slot + 128 * half + 32 * t, 32)] for half in range(2)])
            room[run] = ROOM[1]
            return 0, run
        pieces = chain(kind, NT, 2, operands, dot, park)
        followers[pieces[-1][1]] = [quarter(t) for t in range(4)]
        return pieces

    def a_transpose_wk(g):
        def tile(j):
            def run():
                wkt_s[g, j] = _ld(wk_v, g, j * 128, 128).astype(F32).T.astype(BF)
            return 0, run
        return [tile(j) for j in range(NT)]

    def a_keys(g, c):
        def operands(ks, js):
            return (_cat([_ld(wkt_s, (g + zero(c), k), 0, 128) for k in ks], 1),
                    _cat([_ld(x_v, k + zero(g), c * 256 + 128 * js[0], 128 * len(js)) for k in ks], 1))

        def part(rows, r0, lo, hi):
            lo, hi = _phi(lo), _phi(hi)
            pkt_s[g, 2 * c, rows, :] = lo.astype(BF)
            pkt_s[g, 2 * c + 1, rows, :] = hi.astype(BF)
            total = lo + hi
            if c < S // 256 - 1:
                z_s[g, c, rows, :] = total
            else:
                for b in range(c):
                    total = total + z_s[g, b, rows, :]
                z = jnp.broadcast_to(jnp.sum(total, axis=1, keepdims=True), (32, 128))
                head = jax.lax.broadcasted_iota(jnp.int32, (32, 128), 1) // DH
                zb_s[g, rows, :] = jnp.where(head == r0 // DH, z, 0.0).astype(BF)
        return chain_then("k", operands, _dot_nt, part)

    def a_gram(g):
        def block(n):
            def operands(ks, js):
                return (_cat([_ld(pkt_s, (g, k), 0, 128) for k in ks], 1),
                        _cat([_ld(x_v, 2 * n + j + zero(NT + g), 128 * ks[0], 128 * len(ks)) for j in js], 1))

            def finish(j, acc):
                g_s[g, 2 * n + j] = acc.astype(BF)
            return chain("g", S // 128, 2, operands, _dot, finish)
        return [t for n in range(D // 256) for t in block(n)]

    def a_kv(g):
        acc = [None]

        def piece(kk):
            def run():
                d = _dot(_cat([_ld(g_s, (g, j), 0, 128) for j in range(4 * kk, 4 * kk + 4)], 1),
                         _ld(wv_v, g, kk * 512, 512))
                fence(d[:8, :])
                urgent(d)
                if kk == 0:
                    acc[0] = d
                else:
                    kv_s[g] = jnp.where(head_mask(), acc[0] + d, 0.0).astype(BF)
            if kk > 0:
                mid_chain.add(run)
            return 128, run
        return [piece(0), piece(1)]

    def a_mix(g, half):
        def run():
            js = range(4 * half, 4 * half + 4)
            m = _dot(_ld(kv_s, g, 0, 128), _cat([_ld(wo_v, j, g * 128, 128) for j in js], 1))
            urgent(m)
            for t, j in enumerate(js):
                m_s[j, pl.ds(g * 128, 128), :] = m[:, t * 128:(t + 1) * 128].astype(BF)
        return 128, run

    def a_query(c, n):
        def operands(ks, js):
            return (_cat([_ld(x_v, k + zero(2 * NT + 2 * n + js[0]), c * 128, 128) for k in ks], 1),
                    _cat([_ld(wq_v, 2 * n + j + zero(c), 128 * ks[0], 128 * len(ks)) for j in js], 1))

        def part(rows, r0, lo, hi):
            pq_s[c, 2 * n, rows, :] = _phi(lo).astype(BF)
            pq_s[c, 2 * n + 1, rows, :] = _phi(hi).astype(BF)
        return chain_then("q", operands, _dot, part)

    def a_normalise(c, half):
        def run():
            for g in range(4 * half, 4 * half + 4):
                pq = _ld(pq_s, (c, g), 0, 128)
                den = _dot(pq, _ld(zb_s, g + zero(c), 0, 128)) + 1e-6
                if g % 4 == 0:
                    urgent(den)
                inv = pl.reciprocal(den, approx=True)
                inv = inv * (2.0 - den * inv)
                r_s[c, g] = (pq.astype(F32) * inv).astype(BF)
        room[run] = ROOM[2]
        return 128, run

    def a_out(c, n):
        def operands(ks, js):
            return (_cat([_ld(r_s, (c, k), 0, 128) for k in ks], 1),
                    _cat([_ld(m_s, 2 * n + j + zero(c), 128 * ks[0], 128 * len(ks)) for j in js], 1))

        def finish(j, acc):
            oa_s[pl.ds(c * 128, 128), pl.ds(n * 256 + j * 128, 128)] = acc.astype(BF)
            if n == D // 256 - 1 and j == 1:
                rows_done[0] = (c + 1) * 128
        return chain("o", NT, 2, operands, _dot, finish)

    def starter(*groups):
        def run():
            for g in groups:
                start(g)
        return 0, run

    a_stream, extra = [], []
    n_g = n_c = 0
    for grow in "gcgggcggcggccccc":
        if grow == "g":
            a_stream += [t for c in range(n_c) for t in a_keys(n_g, c)]
            n_g += 1
        else:
            a_stream += [t for g in range(n_g) for t in a_keys(g, n_c)]
            n_c += 1
    extra += [(0, sync([cp_x[0], cp_wk[1]], [cp_wk[2], cp_wk[3]])),
              (4, sync([cp_wk[2], cp_wk[3]], [cp_x[1], cp_wk[4], cp_wk[5]])),
              (16, sync([cp_x[1]], [cp_x[2], cp_h[0], cp_tab])),
              (24, sync([cp_wk[4], cp_wk[5]], [cp_wk[6], cp_wk[7]])),
              (F0_AT, sync([cp_x[2], cp_wk[6], cp_wk[7], cp_tab, cp_h[0]], [cp_x[3], cp_kv[0], cp_x[4]])),
              (96, sync([cp_x[3], cp_x[4]]))]
    extra += [(F0_AT + 2 + 2 * k2, dft_matrix(k2)) for k2 in range(N2)]
    for g, (at, step) in {1: (0, 0.45), 2: (4, 0.45), 3: (8, 0.45), 4: (24, 0.9), 5: (32, 0.9), 6: (50, 2),
                          7: (68, 1.8)}.items():
        extra += [(at + int(step * j), t) for j, t in enumerate(a_transpose_wk(g))]
    for g in range(NT):
        at = len(a_stream)
        if g >= 5:
            for t, gg in enumerate(range(3 * (g - 5), min(3 * (g - 4), NT - 1))):
                extra += [(at + 8 * t + 8, p) for p in a_kv(gg)] + [(at + 8 * t + 16, a_mix(gg, 0)), (at + 8 * t + 16, a_mix(gg, 1))]
        a_stream += a_gram(g)
    a_stream = _spread(a_stream, extra)
    tail = []
    n_c = S // 128
    for c in range(n_c + 1):
        stream = [t for n in range(D // 256) for t in a_query(c, n)] if c < n_c else []
        stream += [t for n in range(D // 256) for t in a_out(c - 1, n)] if c > 0 else []
        at = len(a_stream)
        if c == 0:
            tail += [(at + 4, p) for p in a_kv(NT - 1)] + [(at + 8, a_mix(NT - 1, 0)), (at + 8, a_mix(NT - 1, 1))]
        if c < n_c:
            tail += [(at + 12, a_normalise(c, 0)), (at + 24, a_normalise(c, 1))]
        a_stream += stream
    a_stream = _spread(a_stream, tail)
    spread, pending = [], []
    for item in a_stream:
        spread.append(item)
        if item[0] > 0 and pending:
            spread.append(pending.pop(0))
        pending += followers.get(item[1], [])
    a_stream = spread + pending

    v_regions, m_regions = [], []
    for r in range(NB + 2):
        v = b_inverse(r - 2) if r >= 2 else []
        if r < NB:
            transposes, prep = b_prepare(r)
            early = len(prep) // 2 if r > 0 else 0
            v = _merge(v, _merge(transposes, prep[:early])) + b_forward(r, prep[early:])
        if r == NB + 1:
            v.append(sync(starts=[cp_ob[NB - 1]]))
        v_regions.append(v)
        m_regions.append(b_middle(r - 1) if 1 <= r <= NB else [])
    v_cost = [sum(c for c, _ in v) for v in v_regions]
    m_cost = [sum(c for grp in m for c, _ in grp) for m in m_regions]
    total = sum(c for c, _ in a_stream) + sum(m_cost)
    weight = [c + w for c, w in zip(v_cost, REGION_BIAS)]

    sync([cp_zero], [cp_zero, cp_wk[0], cp_x[0]])[1]()
    w_s[area("k", 0)] = jnp.zeros((HALO, CB), F32)
    for ref in (pkt_s, r_s, g_s, kv_s, pq_s, a_s, z_s, fwd_v, inv_v):
        lead = (zero(0),) + (0,) * (len(ref.shape) - 3)
        ref[(*lead, pl.ds(0, 16), slice(None))] = jnp.zeros((16, CB), ref.dtype)
    sync([cp_wk[0]], [cp_wk[1]])[1]()
    for _, run in a_transpose_wk(0):
        run()

    def needs(lo, hi):
        return ([g for i in range(max(lo, 1), min(hi, NB)) for g in (cp_h[i], cp_kv[i])]
                + [cp_q[i - 2] for i in range(max(lo, 2), hi)])

    assert SYNCS[:4] == [0, 1, 2, 3] and SYNCS[-1] == NB + 1
    ai, clock, ob_sent = 0, 0, 0
    for r in range(NB + 2):
        end = FIRST + (total - FIRST) * sum(weight[1:r + 1]) / sum(weight[1:])
        a_end, t = ai, clock + m_cost[r]
        while a_end < len(a_stream) and (t < end or a_stream[a_end][0] == 0
                                         or a_stream[a_end][1] in mid_chain or r == NB + 1):
            t += a_stream[a_end][0]
            a_end += 1
        length = sum(room.get(run, cost) for cost, run in a_stream[ai:a_end])
        v, m = v_regions[r], m_regions[r]
        lead, trail = 0, (V_TRAIL if r == NB + 1 else 0)
        if r == 0:
            first = [p for p, (cost, _) in enumerate(a_stream) if cost > 0][F0_AT + 2]
            lead = sum(room.get(run, cost) for cost, run in a_stream[:first])
        v_time, acc_cost = [], 0
        for c, _ in v:
            v_time.append(lead + (length - lead - trail) * acc_cost / v_cost[r])
            acc_cost += c

        def region():
            now, pa, pm, pv = 0, ai, 0, 0
            while pa < a_end or pm < len(m):
                if pm < len(m) and ((length - M_TRAIL) * pm / len(m) <= now or pa == a_end):
                    todo = m[pm]
                    pm += 1
                else:
                    todo = [a_stream[pa]]
                    pa += 1
                for cost, run in todo:
                    run()
                    now += 0 if len(todo) > 1 else room.get(run, cost)
                while pv < len(v) and v_time[pv] <= now:
                    v[pv][1]()
                    pv += 1
            for _, run in v[pv:]:
                run()
            if lead_chain[0] is not None:
                fence(lead_chain[0])
                lead_chain[0] = None

        if r in SYNCS:
            nxt = min([b for b in SYNCS if b > r] + [NB + 2])
            far = min([b for b in SYNCS if b > nxt] + [NB + 2])
            waits, starts = needs(r, nxt), (needs(nxt, far) if r > 0 else [])
            while ob_sent + 3 <= r:
                starts.append(cp_ob[ob_sent])
                ob_sent += 1
            pieces = sum(c > 0 for c, _ in a_stream[:ai])
            if r == 1:
                assert F0_AT + 2 * N2 + 2 < pieces <= 160 and nxt == 2
                waits, starts = waits + cp_x[5:], starts + [cp_wvo]
            if r == 2:
                starts = starts + [cp_wq]
            if r == 3:
                assert pieces <= 256 + 5 * 32 + 8
                waits = waits + [cp_wvo, cp_wq]
            sync(waits, starts)[1]()
        fenced[0] = inv_v if r == 0 else yf_s
        region()
        ai, clock = a_end, t

    sync()[1]()
    assert rows_done == [S, S] and n_sem[0] + len(oa_spans) <= sems.shape[0]
    for g in [cp_oa(t) for t in range(len(oa_spans))] + cp_ob:
        wait(g)


@jax.jit
def pallas_concat_heads__linear_attn_block__ssm_conv_h3__prompt_kernel(
    A_x: jax.Array,
    A_wqkv: jax.Array,
    A_wo: jax.Array,
    B_q: jax.Array,
    B_k: jax.Array,
    B_v: jax.Array,
    B_shift_k: jax.Array,
    B_ssm_k: jax.Array,
    B_ssm_D: jax.Array,
):
    hbm = pl.BlockSpec(memory_space=pl.ANY)
    scratch = [
        pltpu.VMEM((NT, S, 128), BF),
        pltpu.VMEM((NT, D, 128), BF),
        pltpu.VMEM((NT, D, 128), BF),
        pltpu.VMEM((NT, D, 128), BF),
        pltpu.VMEM((NT, D, 128), BF),
        pltpu.VMEM((NB, S, CB), BF),
        pltpu.VMEM((NB, S, CB), BF),
        pltpu.VMEM((NB, S, CB), BF),
        pltpu.VMEM((NB, CB, S), BF),
        pltpu.VMEM(_TABLES.shape, F32),
        pltpu.VMEM((N2, 128, 128), BF),
        pltpu.VMEM((N2 + 1, 128, 128), BF),
        pltpu.VMEM((NT, NT, 128, 128), BF),
        pltpu.VMEM((NT, S // 128, 128, 128), BF),
        pltpu.VMEM((NT, NT, 128, 128), BF),
        pltpu.VMEM((NT, 128, 128), BF),
        pltpu.VMEM((NT, D, 128), BF),
        pltpu.VMEM((NT, 128, 128), BF),
        pltpu.VMEM((S // 128, NT, 128, 128), BF),
        pltpu.VMEM((S // 128, NT, 128, 128), BF),
        pltpu.VMEM((S, D), BF),
        pltpu.VMEM((NB, S, CB), BF),
        pltpu.VMEM((2, 2, N2, 128, CB), BF),
        pltpu.VMEM((N2 + 1, 128, CB), BF),
        pltpu.VMEM((NT, S // 256, 128, 128), F32),
        pltpu.VMEM((W_ROWS, 128), F32),
        pltpu.SMEM((NZ,), jnp.int32),
        pltpu.VMEM((4, D), BF),
        pltpu.VMEM((D,), BF),
        pltpu.VMEM((1, D), F32),
        pltpu.SemaphoreType.DMA((64,)),
    ]
    out = pl.pallas_call(
        _kernel,
        out_shape=jax.ShapeDtypeStruct((S, 2 * D), BF),
        in_specs=[hbm] * 11,
        out_specs=hbm,
        scratch_shapes=scratch,
        compiler_params=pltpu.CompilerParams(vmem_limit_bytes=100 * 1024 * 1024),
    )(np.zeros((NZ,), np.int32), A_x.reshape(S, D), A_wqkv, A_wo, B_q.reshape(S, D), B_k.reshape(S, D), B_v.reshape(S, D),
      B_shift_k.T, B_ssm_k, B_ssm_D, _TABLES)
    return out.reshape(1, S, 2 * D)
```
